```python
import jax
import jax.numpy as jnp

def _softmax(x, axis=-1):
    return jax.nn.softmax(x, axis=axis)
def _gelu(x):
    return jax.nn.gelu(x, approximate=True)
def _silu(x):
    return jax.nn.silu(x)
def _sigmoid(x):
    return jax.nn.sigmoid(x)
def _layernorm(x, axis=-1, eps=1e-5):
    m = jnp.mean(x, axis=axis, keepdims=True)
    v = jnp.var(x, axis=axis, keepdims=True)
    return (x - m) / jnp.sqrt(v + eps)
def _scatter_add(tgt, idx, src, axis=0):
    return tgt.at[idx].add(src)
def _segment_sum(src, seg, n):
    return jax.ops.segment_sum(src, seg, n)
class _Rng:
    def __init__(self, key):
        self._k = key
    def _next(self):
        self._k, sub = jax.random.split(self._k)
        return sub
    def normal(self, shape):
        return jax.random.normal(self._next(), shape, dtype=jnp.bfloat16)
    def randint(self, lo, hi, shape):
        return jax.random.randint(self._next(), shape, lo, hi, dtype=jnp.int32)
    def uniform(self, shape, lo=0.0, hi=1.0):
        return jax.random.uniform(self._next(), shape, jnp.bfloat16, lo, hi)
    def permutation(self, n):
        return jax.random.permutation(self._next(), n)


kernel_name = 'recurrent_scan__gqa_block_cached__moe_arch_mod__prompt'

def setup_inputs():
    _rng = _Rng(jax.random.key(int.from_bytes(__import__("os").urandom(4), "little")))
    _w = (lambda a: (lambda t: t.astype(jnp.bfloat16) if jnp.issubdtype(t.dtype, jnp.floating) else t)(jnp.asarray(a)))
    def _A_setup():
        B, Sq, D = 1, 2048, 576
        Hq, Hkv, Sk, Dh = 32, 16, 2048, 128
        assert Hq % Hkv == 0, (Hq, Hkv)
        return {
            "x": _w((lambda *s: _rng.normal(s) * 0.05)(B, Sq, D)),
            "k_cache": _w((lambda *s: _rng.normal(s) * 0.05)(B, Hkv, Sk, Dh)),
            "v_cache": _w((lambda *s: _rng.normal(s) * 0.05)(B, Hkv, Sk, Dh)),
            "wq": _w((lambda *s: _rng.normal(s) * 0.05)(D, Hq * Dh) * (D ** -0.5)),
            "wo": _w((lambda *s: _rng.normal(s) * 0.05)(Hq * Dh, D) * ((Hq * Dh) ** -0.5)),
        }
    _A_in = _A_setup()

    def _B_setup():
        B, S, D, F, C = 1, 2048, 576, 4608, 8
        return {
            "x": _w((lambda *s: _rng.normal(s) * 0.05)(B, S, D)),
            "w_r": _w((lambda *s: _rng.normal(s) * 0.05)(D)),
            "w_gate": _w((lambda *s: _rng.normal(s) * 0.05)(D, F)),
            "w_up": _w((lambda *s: _rng.normal(s) * 0.05)(D, F)),
            "w_down": _w((lambda *s: _rng.normal(s) * 0.05)(F, D)),
        }
    _B_in = _B_setup()

    return {
        "A_x": _A_in["x"],
        "A_k_cache": _A_in["k_cache"],
        "A_v_cache": _A_in["v_cache"],
        "A_wq": _A_in["wq"],
        "A_wo": _A_in["wo"],
        "B_x": _B_in["x"],
        "B_w_r": _B_in["w_r"],
        "B_w_gate": _B_in["w_gate"],
        "B_w_up": _B_in["w_up"],
        "B_w_down": _B_in["w_down"],
    }

def reference(A_x, A_k_cache, A_v_cache, A_wq, A_wo, B_x, B_w_r, B_w_gate, B_w_up, B_w_down):
    def _A_ref(x, k_cache, v_cache, wq, wo):
        B, Sq, D = x.shape
        Hq, Dh = 32, 128
        Hkv = k_cache.shape[1]
        rep = Hq // Hkv
        q = (lambda x, *d: x.transpose(*d))((x @ wq).reshape(B, Sq, Hq, Dh), 0, 2, 1, 3)
        k = jnp.repeat(k_cache, rep, axis=1)
        v = jnp.repeat(v_cache, rep, axis=1)
        scores = jnp.einsum("bhqd,bhkd->bhqk", q, k) * (Dh ** -0.5)
        p = _softmax(scores, axis=-1)
        o = jnp.einsum("bhqk,bhkd->bhqd", p, v)
        return (lambda x, *d: x.transpose(*d))(o, 0, 2, 1, 3).reshape(B, Sq, Hq * Dh) @ wo

    def _B_ref(x, w_r, w_gate, w_up, w_down):
        B, S, D = x.shape
        C = 8
        r = x @ w_r
        idx = jnp.argsort(-r, axis=-1)[:, :C]
        idx_e = jnp.repeat(idx.reshape(B, C, 1), D, axis=2)
        x_sel = jnp.take_along_axis(x, idx_e, axis=1)
        g = _silu(x_sel @ w_gate)
        u = x_sel @ w_up
        y = (g * u) @ w_down
        r_sel = _sigmoid(jnp.take_along_axis(r, idx, axis=1))
        y = y * r_sel.reshape(B, C, 1)
        b_off = (jnp.arange(B) * S).reshape(B, 1)
        flat_idx = (idx + b_off).reshape(B * C)
        zero = (x * 0.0).reshape(B * S, D)
        upd = _scatter_add(zero, flat_idx, y.reshape(B * C, D), axis=0)
        return x + upd.reshape(B, S, D)

    x = A_x
    xn = _layernorm(x, axis=-1)
    s = _A_ref(xn, A_k_cache, A_v_cache, A_wq, A_wo)
    g = _silu(_B_ref(xn, B_w_r, B_w_gate, B_w_up, B_w_down))
    return x + s * g
```

```python
import functools
import math

import jax
import jax.numpy as jnp
from jax import lax
import jax.experimental.pallas as pl
import jax.experimental.pallas.tpu as pltpu

S = 2048
D = 576
DP = 640
HQ = 32
HKV = 16
DH = 128
F = 4608
C = 8
EPS_BF16 = 1.0013580322265625e-05

TQ = 128
UN = 4
CH = 512
TPH = S // TQ
IPH = TPH // UN
NIT = HKV * IPH
XC = 8
XR = S // XC

BF = jnp.bfloat16
F32 = jnp.float32
U32 = jnp.uint32
QSCALE = (DH ** -0.5) * math.log2(math.e)


def _rb(v):
    return v.astype(BF).astype(F32)


def _pack(v_bf16):
    return pltpu.bitcast(v_bf16, U32)


def _unpack(v_u32):
    return pltpu.bitcast(v_u32, BF)


def _fold(x, op):
    r = x[:, 0:128]
    for j in range(1, x.shape[1] // 128):
        r = op(r, x[:, j * 128:(j + 1) * 128])
    return r


def _sigmoid(v):
    return 1.0 / (1.0 + jnp.exp(-v))


def _kernel(x_hbm, k_hbm, v_hbm, wq_hbm, wo_hbm, wr_ref, wg_hbm, wu_hbm, wd_hbm,
            out_hbm,
            x_v, xn_p, z_v, acc_v, k_v, v_v, wq_v, wo_v, wg_v, wu_v, wd_v,
            q_buf, o_buf, xs_v, out_v,
            sem_x, sem_h, sem_m, sem_o):

    def x_copy(c):
        return pltpu.make_async_copy(
            x_hbm.at[pl.ds(c * XR, XR), :], x_v.at[pl.ds(c * XR, XR), :], sem_x.at[c])

    def head_copies(j):
        col = pl.multiple_of(j * (2 * DH), 2 * DH)
        return [
            pltpu.make_async_copy(wq_hbm.at[:, pl.ds(col, 2 * DH)],
                                  wq_v.at[pl.ds(0, D), pl.ds(col, 2 * DH)], sem_h.at[4 * j]),
            pltpu.make_async_copy(k_hbm.at[j], k_v.at[j], sem_h.at[4 * j + 1]),
            pltpu.make_async_copy(v_hbm.at[j], v_v.at[j], sem_h.at[4 * j + 2]),
            pltpu.make_async_copy(wo_hbm.at[pl.ds(col, 2 * DH), :],
                                  wo_v.at[pl.ds(col, 2 * DH), :], sem_h.at[4 * j + 3]),
        ]

    def moe_copies():
        return [pltpu.make_async_copy(wg_hbm, wg_v, sem_m.at[0]),
                pltpu.make_async_copy(wu_hbm, wu_v, sem_m.at[1]),
                pltpu.make_async_copy(wd_hbm, wd_v, sem_m.at[2])]

    def out_copy(c):
        return pltpu.make_async_copy(
            out_v.at[pl.ds(c * XR, XR), :], out_hbm.at[pl.ds(c * XR, XR), :], sem_o.at[c])

    for c in range(XC):
        x_copy(c).start()
    for cp in head_copies(0):
        cp.start()
    for cp in head_copies(1):
        cp.start()

    acc_v[...] = jnp.zeros(acc_v.shape, F32)
    o_buf[...] = jnp.zeros(o_buf.shape, U32)
    xn_p[:, 512:DP] = jnp.zeros((S // 2, DP - 512), U32)
    wq_v[D:DP, :] = jnp.zeros((DP - D, HQ * DH), BF)
    xs_v[...] = jnp.zeros(xs_v.shape, F32)

    eps_b = EPS_BF16
    for c in range(XC):
        x_copy(c).wait()
        xf = x_v[c * XR:(c + 1) * XR, :].astype(F32)
        mean = jnp.sum(xf, axis=1, keepdims=True) / D
        cen = xf - mean
        var = jnp.sum(cen * cen, axis=1, keepdims=True) / D
        dlt = _rb(xf - _rb(mean))
        sd = _rb(jnp.sqrt(_rb(_rb(var) + eps_b)))
        xn = (dlt / sd).astype(BF)
        z_v[c * XR:(c + 1) * XR, :] = xn.astype(F32)
        xn_p[c * XR // 2:(c + 1) * XR // 2, 0:D] = _pack(xn)

    def qproj(j, row0, a):
        col = pl.multiple_of(j * (2 * DH), 2 * DH)
        r2 = pl.multiple_of(row0 // 2, UN * TQ // 2)
        xb = _unpack(xn_p[pl.ds(r2 + a * (TQ // 2), TQ // 2), :])
        q2 = jnp.dot(xb, wq_v[:, pl.ds(col, 2 * DH)], preferred_element_type=F32)
        q2 = (q2 * QSCALE).astype(BF)
        q_buf[a, 0:TQ // 2, :] = _pack(q2[:, 0:DH])
        q_buf[a, TQ // 2:TQ, :] = _pack(q2[:, DH:2 * DH])

    def oproj(j, row0, a):
        col = pl.multiple_of(j * (2 * DH), 2 * DH)
        r = pl.multiple_of(row0, UN * TQ) + a * TQ
        o2 = _unpack(o_buf[a])
        upd = jnp.dot(o2, wo_v[pl.ds(col, 2 * DH), :], preferred_element_type=F32)
        acc_v[pl.ds(r, TQ), :] = acc_v[pl.ds(r, TQ), :] + upd

    def attention(j, a):
        q = _unpack(q_buf[a])
        m = l = acc = None
        for c in range(S // CH):
            kc = k_v[j, c * CH:(c + 1) * CH, :]
            s = lax.dot_general(q, kc, (((1,), (1,)), ((), ())),
                                preferred_element_type=F32)
            mc = jnp.broadcast_to(jnp.max(_fold(s, jnp.maximum), axis=1, keepdims=True),
                                  (2 * TQ, 128))
            m_new = mc if m is None else jnp.maximum(m, mc)
            p = jnp.exp2(s - jnp.tile(m_new, (1, CH // 128)))
            lc = _fold(p, jnp.add)
            pv = jnp.dot(p.astype(BF), v_v[j, c * CH:(c + 1) * CH, :],
                         preferred_element_type=F32)
            if m is None:
                l, acc = lc, pv
            else:
                alpha = jnp.exp2(m - m_new)
                l = l * alpha + lc
                acc = acc * alpha + pv
            m = m_new
        ls = jnp.sum(l, axis=1, keepdims=True)
        o = (acc * (1.0 / ls)).astype(BF)
        o_buf[a, :, 0:DH] = _pack(o[0:TQ])
        o_buf[a, :, DH:2 * DH] = _pack(o[TQ:2 * TQ])

    for cp in head_copies(0):
        cp.wait()
    for a in range(UN):
        qproj(0, 0, a)

    def body(u, carry):
        j = u // IPH
        un = jnp.minimum(u + 1, NIT - 1)
        jn = un // IPH
        up = jnp.maximum(u - 1, 0)
        jp = up // IPH

        @pl.when(jnp.logical_and((u + 1) % IPH == 0, u + 1 < NIT))
        def _():
            for cp in head_copies(jn):
                cp.wait()

            @pl.when(jn + 1 < HKV)
            def _():
                for cp in head_copies(jn + 1):
                    cp.start()

        @pl.when(u == IPH)
        def _():
            for cp in moe_copies():
                cp.start()

        rown = (un % IPH) * (UN * TQ)
        rowp = (up % IPH) * (UN * TQ)
        for a in range(UN):
            oproj(jp, rowp, a)
            attention(j, a)
            qproj(jn, rown, a)
        return carry

    lax.fori_loop(0, NIT, body, 0)
    for a in range(UN):
        oproj(HKV - 1, S - UN * TQ, a)

    for cp in moe_copies():
        cp.wait()
    xn_all = _unpack(xn_p[:, 0:D])
    wr = jnp.broadcast_to(wr_ref[...], (16, D))
    r = lax.dot_general(wr, xn_all, (((1,), (1,)), ((), ())),
                        preferred_element_type=F32)
    r = _rb(r[0:8, :])
    col = lax.broadcasted_iota(jnp.int32, (8, S), 1).astype(F32)
    sel = []
    for c in range(C):
        mx = jnp.max(r)
        idx_f = jnp.min(jnp.where(r == mx, col, float(S)))
        idx = jnp.minimum(idx_f.astype(jnp.int32), S - 1)
        r = jnp.where(col == idx_f, -jnp.inf, r)
        sel.append((idx, mx))
        xs_v[c:c + 1, :] = z_v[pl.ds(idx, 1), :]
    xs = xs_v[...].astype(BF)
    g = _rb(jnp.dot(xs, wg_v[...], preferred_element_type=F32))
    uu = _rb(jnp.dot(xs, wu_v[...], preferred_element_type=F32))
    h = (_rb(g * _rb(_sigmoid(g))) * uu).astype(BF)
    y = _rb(jnp.dot(h, wd_v[...], preferred_element_type=F32))
    for c in range(C):
        idx, mx = sel[c]
        gate = _rb(_sigmoid(jnp.full((1, D), mx, F32)))
        row = z_v[pl.ds(idx, 1), :]
        z_v[pl.ds(idx, 1), :] = _rb(row + _rb(y[c:c + 1, :] * gate))

    for c in range(XC):
        rows = slice(c * XR, (c + 1) * XR)
        z = z_v[rows, :]
        gt = _rb(z * _rb(_sigmoid(z)))
        sg = _rb(_rb(acc_v[rows, :]) * gt)
        out_v[rows, :] = (x_v[rows, :].astype(F32) + sg).astype(BF)
        out_copy(c).start()
    for c in range(XC):
        out_copy(c).wait()


@jax.jit
def pallas_recurrent_scan__gqa_block_cached__moe_arch_mod__prompt_kernel(
    A_x: jax.Array,
    A_k_cache: jax.Array,
    A_v_cache: jax.Array,
    A_wq: jax.Array,
    A_wo: jax.Array,
    B_x: jax.Array,
    B_w_r: jax.Array,
    B_w_gate: jax.Array,
    B_w_up: jax.Array,
    B_w_down: jax.Array,
):
    del B_x
    x = A_x.reshape(S, D)
    k = A_k_cache.reshape(HKV, S, DH)
    v = A_v_cache.reshape(HKV, S, DH)
    wr = B_w_r.reshape(1, D)

    hbm = pl.BlockSpec(memory_space=pl.ANY)
    vmem = pl.BlockSpec(memory_space=pltpu.VMEM)
    out = pl.pallas_call(
        _kernel,
        out_shape=jax.ShapeDtypeStruct((S, D), BF),
        in_specs=[hbm, hbm, hbm, hbm, hbm, vmem, hbm, hbm, hbm],
        out_specs=hbm,
        scratch_shapes=[
            pltpu.VMEM((S, D), BF),
            pltpu.VMEM((S // 2, DP), U32),
            pltpu.VMEM((S, D), F32),
            pltpu.VMEM((S, D), F32),
            pltpu.VMEM((HKV, S, DH), BF),
            pltpu.VMEM((HKV, S, DH), BF),
            pltpu.VMEM((DP, HQ * DH), BF),
            pltpu.VMEM((HQ * DH, D), BF),
            pltpu.VMEM((D, F), BF),
            pltpu.VMEM((D, F), BF),
            pltpu.VMEM((F, D), BF),
            pltpu.VMEM((UN, TQ, DH), U32),
            pltpu.VMEM((UN, TQ // 2, 2 * DH), U32),
            pltpu.VMEM((16, D), F32),
            pltpu.VMEM((S, D), BF),
            pltpu.SemaphoreType.DMA((XC,)),
            pltpu.SemaphoreType.DMA((4 * HKV,)),
            pltpu.SemaphoreType.DMA((3,)),
            pltpu.SemaphoreType.DMA((XC,)),
        ],
        compiler_params=pltpu.CompilerParams(vmem_limit_bytes=100 * 1024 * 1024),
        name="fused_attn_moe",
    )(x, k, v, A_wq, A_wo, wr, B_w_gate, B_w_up, B_w_down)
    return out.reshape(1, S, D)
```

```python
import functools
import math

import jax
import jax.numpy as jnp
from jax import lax
import jax.experimental.pallas as pl
import jax.experimental.pallas.tpu as pltpu

S = 2048
D = 576
DP = 640
HQ = 32
HKV = 16
DH = 128
F = 4608
C = 8
EPS_BF16 = 1.0013580322265625e-05

TQ = 128
UN = 4
CH = 512
TPH = S // TQ
IPH = TPH // UN
NIT = HKV * IPH
XC = 8
XR = S // XC

BF = jnp.bfloat16
F32 = jnp.float32
U32 = jnp.uint32
QSCALE = (DH ** -0.5) * math.log2(math.e)


def _rb(v):
    return v.astype(BF).astype(F32)


def _pack(v_bf16):
    return pltpu.bitcast(v_bf16, U32)


def _unpack(v_u32):
    return pltpu.bitcast(v_u32, BF)


def _fold(x, op):
    r = x[:, 0:128]
    for j in range(1, x.shape[1] // 128):
        r = op(r, x[:, j * 128:(j + 1) * 128])
    return r


def _sigmoid(v):
    return 0.5 * jnp.tanh(0.5 * v) + 0.5


def _recip(v):
    r = pl.reciprocal(v, approx=True)
    return r * (2.0 - v * r)


def _kernel(xT_hbm, k_hbm, v_hbm, wq_hbm, woT_hbm, wr_ref, wg_hbm, wu_hbm, wdT_hbm,
            outT_hbm,
            xT_v, xnT_p, xn_p, accT, k_v, v_v, wq_v, woT_v, wg_v, wu_v, wdT_v,
            q_buf, o_buf, xs_v, outT_v,
            sem_x, sem_h, sem_m, sem_o):

    def x_copy(c):
        return pltpu.make_async_copy(
            xT_hbm.at[:, pl.ds(c * XR, XR)], xT_v.at[:, pl.ds(c * XR, XR)], sem_x.at[c])

    def head_copies(j):
        col = pl.multiple_of(j * (2 * DH), 2 * DH)
        return [
            pltpu.make_async_copy(wq_hbm.at[:, pl.ds(col, 2 * DH)],
                                  wq_v.at[pl.ds(0, D), pl.ds(col, 2 * DH)], sem_h.at[4 * j]),
            pltpu.make_async_copy(k_hbm.at[j], k_v.at[j], sem_h.at[4 * j + 1]),
            pltpu.make_async_copy(v_hbm.at[j], v_v.at[j], sem_h.at[4 * j + 2]),
            pltpu.make_async_copy(woT_hbm.at[:, pl.ds(col, 2 * DH)],
                                  woT_v.at[:, pl.ds(col, 2 * DH)], sem_h.at[4 * j + 3]),
        ]

    def moe_copies():
        return [pltpu.make_async_copy(wg_hbm, wg_v, sem_m.at[0]),
                pltpu.make_async_copy(wu_hbm, wu_v, sem_m.at[1]),
                pltpu.make_async_copy(wdT_hbm, wdT_v, sem_m.at[2])]

    def out_copy(c):
        return pltpu.make_async_copy(
            outT_v.at[:, pl.ds(c * XR, XR)], outT_hbm.at[:, pl.ds(c * XR, XR)], sem_o.at[c])

    for c in range(XC):
        x_copy(c).start()
    for cp in head_copies(0):
        cp.start()
    for cp in head_copies(1):
        cp.start()

    accT[...] = jnp.zeros(accT.shape, F32)
    o_buf[...] = jnp.zeros(o_buf.shape, U32)
    wq_v[D:DP, :] = jnp.zeros((DP - D, HQ * DH), BF)
    xs_v[...] = jnp.zeros(xs_v.shape, F32)

    for c in range(XC):
        x_copy(c).wait()
        cols = slice(c * XR, (c + 1) * XR)
        xf = xT_v[:, cols].astype(F32)
        mean = jnp.sum(xf, axis=0, keepdims=True) / D
        cen = xf - mean
        var = jnp.sum(cen * cen, axis=0, keepdims=True) / D
        dlt = _rb(xf - _rb(mean))
        sd = _rb(jnp.sqrt(_rb(_rb(var) + EPS_BF16)))
        xnT = (dlt / sd).astype(BF)
        xnT_p[:, cols] = _pack(xnT)
        xpad = jnp.concatenate([xnT, jnp.zeros((DP - D, XR), BF)], axis=0)
        xn_p[c * XR // 2:(c + 1) * XR // 2, :] = _pack(xpad.T)

    def qproj(j, row0, a):
        col = pl.multiple_of(j * (2 * DH), 2 * DH)
        r2 = pl.multiple_of(row0 // 2, UN * TQ // 2)
        xb = _unpack(xn_p[pl.ds(r2 + a * (TQ // 2), TQ // 2), :])
        q2 = jnp.dot(xb, wq_v[:, pl.ds(col, 2 * DH)], preferred_element_type=F32)
        q2 = (q2 * QSCALE).astype(BF)
        q_buf[a, 0:TQ // 2, :] = _pack(q2[:, 0:DH])
        q_buf[a, TQ // 2:TQ, :] = _pack(q2[:, DH:2 * DH])

    def oproj(j, row0, a):
        col = pl.multiple_of(j * (2 * DH), 2 * DH)
        t = row0 // TQ + a
        o2 = _unpack(o_buf[a])
        upd = lax.dot_general(woT_v[:, pl.ds(col, 2 * DH)], o2, (((1,), (1,)), ((), ())),
                              preferred_element_type=F32)
        accT[t] = accT[t] + upd

    def attention(j, a):
        q = _unpack(q_buf[a])
        m = l = acc = None
        for c in range(S // CH):
            kc = k_v[j, c * CH:(c + 1) * CH, :]
            s = lax.dot_general(q, kc, (((1,), (1,)), ((), ())),
                                preferred_element_type=F32)
            mc = jnp.broadcast_to(jnp.max(_fold(s, jnp.maximum), axis=1, keepdims=True),
                                  (2 * TQ, 128))
            m_new = mc if m is None else jnp.maximum(m, mc)
            p = jnp.exp2(s - jnp.tile(m_new, (1, CH // 128)))
            lc = _fold(p, jnp.add)
            pv = jnp.dot(p.astype(BF), v_v[j, c * CH:(c + 1) * CH, :],
                         preferred_element_type=F32)
            if m is None:
                l, acc = lc, pv
            else:
                alpha = jnp.exp2(m - m_new)
                l = l * alpha + lc
                acc = acc * alpha + pv
            m = m_new
        ls = jnp.sum(l, axis=1, keepdims=True)
        o = (acc * _recip(ls)).astype(BF)
        o_buf[a, :, 0:DH] = _pack(o[0:TQ])
        o_buf[a, :, DH:2 * DH] = _pack(o[TQ:2 * TQ])

    for cp in head_copies(0):
        cp.wait()
    for a in range(UN):
        qproj(0, 0, a)

    def body(u, carry):
        j = u // IPH
        un = jnp.minimum(u + 1, NIT - 1)
        jn = un // IPH
        up = jnp.maximum(u - 1, 0)
        jp = up // IPH

        @pl.when(jnp.logical_and((u + 1) % IPH == 0, u + 1 < NIT))
        def _():
            for cp in head_copies(jn):
                cp.wait()

            @pl.when(jn + 1 < HKV)
            def _():
                for cp in head_copies(jn + 1):
                    cp.start()

        @pl.when(u == IPH)
        def _():
            for cp in moe_copies():
                cp.start()

        rown = (un % IPH) * (UN * TQ)
        rowp = (up % IPH) * (UN * TQ)
        for a in range(UN):
            oproj(jp, rowp, a)
            attention(j, a)
            qproj(jn, rown, a)
        return carry

    lax.fori_loop(0, NIT, body, 0)
    for a in range(UN):
        oproj(HKV - 1, S - UN * TQ, a)

    for cp in moe_copies():
        cp.wait()
    wr = jnp.broadcast_to(wr_ref[...], (16, D))
    r = jnp.dot(wr, _unpack(xnT_p[...]), preferred_element_type=F32)
    r = _rb(r[0:8, :])
    col = lax.broadcasted_iota(jnp.int32, (8, S), 1).astype(F32)
    row16 = lax.broadcasted_iota(jnp.int32, (16, S), 0)
    col16 = lax.broadcasted_iota(jnp.int32, (16, S), 1)
    rowg = lax.broadcasted_iota(jnp.int32, (16, 1), 0)
    onehot = jnp.zeros((16, S), F32)
    rsel = jnp.zeros((16, 1), F32)
    for c in range(C):
        mx = jnp.max(r)
        idx_f = jnp.min(jnp.where(r == mx, col, float(S)))
        idx = jnp.minimum(idx_f.astype(jnp.int32), S - 1)
        r = jnp.where(col == idx_f, -jnp.inf, r)
        onehot = jnp.where(jnp.logical_and(row16 == c, col16 == idx), 1.0, onehot)
        rsel = jnp.where(rowg == c, mx, rsel)
        w = xn_p[pl.ds(idx // 2, 1), :]
        w = jnp.where(idx % 2 == 0, w << 16, w & jnp.uint32(0xFFFF0000))
        xs_v[c:c + 1, :] = lax.bitcast_convert_type(w, F32)
    xs = xs_v[:, 0:D].astype(BF)
    g = _rb(jnp.dot(xs, wg_v[...], preferred_element_type=F32))
    uu = _rb(jnp.dot(xs, wu_v[...], preferred_element_type=F32))
    h = (_rb(g * _rb(_sigmoid(g))) * uu).astype(BF)
    y = _rb(lax.dot_general(h, wdT_v[...], (((1,), (1,)), ((), ())),
                            preferred_element_type=F32))
    y = _rb(y * _rb(_sigmoid(rsel)))
    ypad = jnp.concatenate([y, jnp.zeros((112, D), F32)], axis=0)
    ypad = jnp.concatenate([ypad, jnp.zeros((128, DP - D), F32)], axis=1)
    yT = ypad.T[0:D, :].astype(BF)
    oh = jnp.concatenate([onehot, jnp.zeros((112, S), F32)], axis=0).astype(BF)

    for c in range(XC):
        cols = slice(c * XR, (c + 1) * XR)
        upd = jnp.dot(yT, oh[:, cols], preferred_element_type=F32)
        z = _unpack(xnT_p[:, cols]).astype(F32) + upd
        gt = z * _sigmoid(z)
        tpc = XR // TQ
        s_att = jnp.concatenate([accT[c * tpc + i] for i in range(tpc)], axis=1)
        outT_v[:, cols] = (xT_v[:, cols].astype(F32) + s_att * gt).astype(BF)
        out_copy(c).start()
    for c in range(XC):
        out_copy(c).wait()


@jax.jit
def pallas_recurrent_scan__gqa_block_cached__moe_arch_mod__prompt_kernel(
    A_x: jax.Array,
    A_k_cache: jax.Array,
    A_v_cache: jax.Array,
    A_wq: jax.Array,
    A_wo: jax.Array,
    B_x: jax.Array,
    B_w_r: jax.Array,
    B_w_gate: jax.Array,
    B_w_up: jax.Array,
    B_w_down: jax.Array,
):
    del B_x
    xT = A_x.reshape(S, D).T
    woT = A_wo.T
    wdT = B_w_down.T
    k = A_k_cache.reshape(HKV, S, DH)
    v = A_v_cache.reshape(HKV, S, DH)
    wr = B_w_r.reshape(1, D)

    hbm = pl.BlockSpec(memory_space=pltpu.HBM)
    vmem = pl.BlockSpec(memory_space=pltpu.VMEM)
    outT = pl.pallas_call(
        _kernel,
        out_shape=jax.ShapeDtypeStruct((D, S), BF),
        in_specs=[hbm, hbm, hbm, hbm, hbm, vmem, hbm, hbm, hbm],
        out_specs=hbm,
        scratch_shapes=[
            pltpu.VMEM((D, S), BF),
            pltpu.VMEM((D // 2, S), U32),
            pltpu.VMEM((S // 2, DP), U32),
            pltpu.VMEM((S // TQ, D, TQ), F32),
            pltpu.VMEM((HKV, S, DH), BF),
            pltpu.VMEM((HKV, S, DH), BF),
            pltpu.VMEM((DP, HQ * DH), BF),
            pltpu.VMEM((D, HQ * DH), BF),
            pltpu.VMEM((D, F), BF),
            pltpu.VMEM((D, F), BF),
            pltpu.VMEM((D, F), BF),
            pltpu.VMEM((UN, TQ, DH), U32),
            pltpu.VMEM((UN, TQ // 2, 2 * DH), U32),
            pltpu.VMEM((16, DP), F32),
            pltpu.VMEM((D, S), BF),
            pltpu.SemaphoreType.DMA((XC,)),
            pltpu.SemaphoreType.DMA((4 * HKV,)),
            pltpu.SemaphoreType.DMA((3,)),
            pltpu.SemaphoreType.DMA((XC,)),
        ],
        compiler_params=pltpu.CompilerParams(vmem_limit_bytes=100 * 1024 * 1024),
        name="fused_attn_moe",
    )(xT, k, v, A_wq, woT, wr, B_w_gate, B_w_up, wdT)
    return outT.T.reshape(1, S, D)
```

```python
import functools
import math

import jax
import jax.numpy as jnp
from jax import lax
import jax.experimental.pallas as pl
import jax.experimental.pallas.tpu as pltpu

S = 2048
D = 576
DP = 640
HQ = 32
HKV = 16
DH = 128
F = 4608
C = 8
EPS_BF16 = 1.0013580322265625e-05

TQ = 128
UN = 4
CH = 512
TPH = S // TQ
IPH = TPH // UN
NIT = HKV * IPH
XC = 8
XR = S // XC

BF = jnp.bfloat16
F32 = jnp.float32
U32 = jnp.uint32
QSCALE = (DH ** -0.5) * math.log2(math.e)
LOG_IPH = IPH.bit_length() - 1
assert 1 << LOG_IPH == IPH

SCORE_BOUND = 40.0
V_HI = 2.0 ** 60
V_LO = 2.0 ** -60


def _rb(v):
    return v.astype(BF).astype(F32)


def _pack(v_bf16):
    return pltpu.bitcast(v_bf16, U32)


def _unpack(v_u32):
    return pltpu.bitcast(v_u32, BF)


def _fold(x, op):
    r = x[:, 0:128]
    for j in range(1, x.shape[1] // 128):
        r = op(r, x[:, j * 128:(j + 1) * 128])
    return r


def _sigmoid(v):
    return 0.5 * jnp.tanh(0.5 * v) + 0.5


def _recip(v):
    r = pl.reciprocal(v, approx=True)
    return r * (2.0 - v * r)


def _kernel(xT_hbm, k_hbm, v_hbm, wq_hbm, woT_hbm, wr_ref, wg_hbm, wu_hbm, wdT_hbm,
            outT_hbm,
            xT_v, xnT_p, xn_p, accT, k_v, v_v, wq_v, woT_v, wg_v, wu_v, wdT_v,
            q_buf, o_buf, xs_v, outT_v, kst, vst, wst, xnm,
            sem_x, sem_h, sem_m, sem_o):

    def x_copy(c):
        return pltpu.make_async_copy(
            xT_hbm.at[:, pl.ds(c * XR, XR)], xT_v.at[:, pl.ds(c * XR, XR)], sem_x.at[c])

    def head_copies(j):
        col = pl.multiple_of(j * (2 * DH), 2 * DH)
        return [
            pltpu.make_async_copy(wq_hbm.at[:, pl.ds(col, 2 * DH)],
                                  wq_v.at[pl.ds(0, D), pl.ds(col, 2 * DH)], sem_h.at[4 * j]),
            pltpu.make_async_copy(k_hbm.at[j], k_v.at[j], sem_h.at[4 * j + 1]),
            pltpu.make_async_copy(v_hbm.at[j], v_v.at[j], sem_h.at[4 * j + 2]),
            pltpu.make_async_copy(woT_hbm.at[:, pl.ds(col, 2 * DH)],
                                  woT_v.at[:, pl.ds(col, 2 * DH)], sem_h.at[4 * j + 3]),
        ]

    def moe_copies():
        return [pltpu.make_async_copy(wg_hbm, wg_v, sem_m.at[0]),
                pltpu.make_async_copy(wu_hbm, wu_v, sem_m.at[1]),
                pltpu.make_async_copy(wdT_hbm, wdT_v, sem_m.at[2])]

    def out_copy(c):
        return pltpu.make_async_copy(
            outT_v.at[:, pl.ds(c * XR, XR)], outT_hbm.at[:, pl.ds(c * XR, XR)], sem_o.at[c])

    for c in range(XC):
        x_copy(c).start()
    for cp in head_copies(0):
        cp.start()
    for cp in head_copies(1):
        cp.start()

    accT[...] = jnp.zeros(accT.shape, F32)
    o_buf[...] = jnp.zeros(o_buf.shape, U32)
    wq_v[D:DP, :] = jnp.zeros((DP - D, HQ * DH), BF)
    xs_v[...] = jnp.zeros(xs_v.shape, F32)

    n2max = None
    for c in range(XC):
        x_copy(c).wait()
        cols = slice(c * XR, (c + 1) * XR)
        xf = xT_v[:, cols].astype(F32)
        mean = jnp.sum(xf, axis=0, keepdims=True) / D
        cen = xf - mean
        var = jnp.sum(cen * cen, axis=0, keepdims=True) / D
        mean_b = _rb(mean)
        dlt = _rb(xf - mean_b)
        sd = _rb(jnp.sqrt(_rb(_rb(var) + EPS_BF16)))
        n2 = D * (var + (mean - mean_b) * (mean - mean_b)) / (sd * sd)
        n2max = n2 if n2max is None else jnp.maximum(n2max, n2)
        xnT = (dlt / sd).astype(BF)
        xnT_p[:, cols] = _pack(xnT)
        xpad = jnp.concatenate([xnT, jnp.zeros((DP - D, XR), BF)], axis=0)
        xn_p[c * XR // 2:(c + 1) * XR // 2, :] = _pack(xpad.T)
    xnm[...] = jnp.broadcast_to(_fold(n2max, jnp.maximum), (8, DH))

    def qproj(j, row0, a):
        col = pl.multiple_of(j * (2 * DH), 2 * DH)
        r2 = pl.multiple_of(lax.shift_right_logical(row0, 1), UN * TQ // 2)
        xb = _unpack(xn_p[pl.ds(r2 + a * (TQ // 2), TQ // 2), :])
        q2 = jnp.dot(xb, wq_v[:, pl.ds(col, 2 * DH)], preferred_element_type=F32)
        q2 = (q2 * QSCALE).astype(BF)
        q_buf[a, 0:TQ // 2, :] = _pack(q2[:, 0:DH])
        q_buf[a, TQ // 2:TQ, :] = _pack(q2[:, DH:2 * DH])

    def oproj(j, row0, a):
        col = pl.multiple_of(j * (2 * DH), 2 * DH)
        t = lax.shift_right_logical(row0, TQ.bit_length() - 1) + a
        o2 = _unpack(o_buf[a])
        upd = lax.dot_general(woT_v[:, pl.ds(col, 2 * DH)], o2, (((1,), (1,)), ((), ())),
                              preferred_element_type=F32)
        accT[t] = accT[t] + upd

    def attention(j, a, fast):
        q = _unpack(q_buf[a])
        m = l = acc = None
        for c in range(S // CH):
            kc = k_v[j, c * CH:(c + 1) * CH, :]
            s = lax.dot_general(q, kc, (((1,), (1,)), ((), ())),
                                preferred_element_type=F32)
            if fast:
                p = jnp.exp2(s)
            else:
                mc = jnp.broadcast_to(
                    jnp.max(_fold(s, jnp.maximum), axis=1, keepdims=True), (2 * TQ, 128))
                m_new = mc if m is None else jnp.maximum(m, mc)
                p = jnp.exp2(s - jnp.tile(m_new, (1, CH // 128)))
            lc = _fold(p, jnp.add)
            pv = jnp.dot(p.astype(BF), v_v[j, c * CH:(c + 1) * CH, :],
                         preferred_element_type=F32)
            if l is None:
                l, acc = lc, pv
            elif fast:
                l, acc = l + lc, acc + pv
            else:
                alpha = jnp.exp2(m - m_new)
                l, acc = l * alpha + lc, acc * alpha + pv
            if not fast:
                m = m_new
        ls = jnp.sum(l, axis=1, keepdims=True)
        o = (acc * _recip(ls)).astype(BF)
        o_buf[a, :, 0:DH] = _pack(o[0:TQ])
        o_buf[a, :, DH:2 * DH] = _pack(o[TQ:2 * TQ])

    def _absmax_packed(w):
        w = w & jnp.uint32(0x7FFF7FFF)
        hi = lax.bitcast_convert_type(w, F32)
        lo = lax.bitcast_convert_type(w << 16, F32)
        m = jnp.maximum(hi, lo)
        r = m[0:8]
        for i in range(1, m.shape[0] // 8):
            r = jnp.maximum(r, m[i * 8:(i + 1) * 8])
        return r

    def head_stats(j, i, nparts):
        first = i == 0
        kr = S // nparts
        r0 = pl.multiple_of(i * kr, kr)
        km = _absmax_packed(_pack(k_v[j, pl.ds(r0, kr), :]))
        vm = _absmax_packed(_pack(v_v[j, pl.ds(r0, kr), :]))
        km = jnp.where(first, km, jnp.maximum(km, kst[...]))
        vm = jnp.where(first, vm, jnp.maximum(vm, vst[...]))
        kst[...] = km
        vst[...] = vm
        wr_ = DP // nparts
        w0 = pl.multiple_of(i * wr_, 16)
        col = pl.multiple_of(j * (2 * DH), 2 * DH)
        wf = wq_v[pl.ds(w0, wr_), pl.ds(col, 2 * DH)].astype(F32)
        w2 = wf * wf
        ws = w2[0:8]
        for t in range(1, wr_ // 8):
            ws = ws + w2[t * 8:(t + 1) * 8]
        ws = jnp.where(first, ws, ws + wst[...])
        wst[...] = ws
        wn2 = jnp.sum(ws, axis=0, keepdims=True)
        wn = jnp.sqrt(jnp.maximum(wn2[:, 0:DH], wn2[:, DH:2 * DH]))
        kmx = jnp.max(km, axis=0, keepdims=True)
        xn = jnp.sqrt(jnp.max(xnm[0:1, :], axis=1, keepdims=True))
        bound = jnp.sum(wn * kmx, axis=1, keepdims=True) * xn * (1.05 * QSCALE)
        vmx = jnp.max(jnp.max(vm, axis=0, keepdims=True), axis=1, keepdims=True)
        ok = jnp.logical_and(bound <= SCORE_BOUND,
                             jnp.logical_and(vmx <= V_HI, vmx >= V_LO))
        return jnp.max(jnp.where(ok, 1.0, 0.0)).astype(jnp.int32)

    for cp in head_copies(0):
        cp.wait()
    safe0 = head_stats(0, 0, 1)
    for a in range(UN):
        qproj(0, 0, a)

    def body(u, safe):
        j = lax.shift_right_logical(u, LOG_IPH)
        i = u & (IPH - 1)
        un = jnp.minimum(u + 1, NIT - 1)
        jn = lax.shift_right_logical(un, LOG_IPH)
        up = jnp.maximum(u - 1, 0)
        jp = lax.shift_right_logical(up, LOG_IPH)
        js = jnp.minimum(j + 1, HKV - 1)

        @pl.when(i == 0)
        def _():
            @pl.when(j + 1 < HKV)
            def _():
                for cp in head_copies(j + 1):
                    cp.wait()

            @pl.when(j + 2 < HKV)
            def _():
                for cp in head_copies(j + 2):
                    cp.start()

        @pl.when(u == IPH)
        def _():
            for cp in moe_copies():
                cp.start()

        rown = (un & (IPH - 1)) * (UN * TQ)
        rowp = (up & (IPH - 1)) * (UN * TQ)

        def work(fast):
            for a in range(UN):
                oproj(jp, rowp, a)
                attention(j, a, fast)
                qproj(jn, rown, a)
            return head_stats(js, i, IPH)

        nxt = lax.cond(safe > 0, lambda: work(True), lambda: work(False))
        return jnp.where(i == IPH - 1, nxt, safe)

    lax.fori_loop(0, NIT, body, safe0)
    for a in range(UN):
        oproj(HKV - 1, S - UN * TQ, a)

    for cp in moe_copies():
        cp.wait()
    wr = jnp.broadcast_to(wr_ref[...], (16, D))
    r = jnp.dot(wr, _unpack(xnT_p[...]), preferred_element_type=F32)
    r = _rb(r[0:8, :])
    col = lax.broadcasted_iota(jnp.int32, (8, S), 1).astype(F32)
    row16 = lax.broadcasted_iota(jnp.int32, (16, S), 0)
    col16 = lax.broadcasted_iota(jnp.int32, (16, S), 1)
    rowg = lax.broadcasted_iota(jnp.int32, (16, 1), 0)
    onehot = jnp.zeros((16, S), F32)
    rsel = jnp.zeros((16, 1), F32)
    for c in range(C):
        mx = jnp.max(r)
        idx_f = jnp.min(jnp.where(r == mx, col, float(S)))
        idx = jnp.minimum(idx_f.astype(jnp.int32), S - 1)
        r = jnp.where(col == idx_f, -jnp.inf, r)
        onehot = jnp.where(jnp.logical_and(row16 == c, col16 == idx), 1.0, onehot)
        rsel = jnp.where(rowg == c, mx, rsel)
        w = xn_p[pl.ds(idx // 2, 1), :]
        w = jnp.where(idx % 2 == 0, w << 16, w & jnp.uint32(0xFFFF0000))
        xs_v[c:c + 1, :] = lax.bitcast_convert_type(w, F32)
    xs = xs_v[:, 0:D].astype(BF)
    g = _rb(jnp.dot(xs, wg_v[...], preferred_element_type=F32))
    uu = _rb(jnp.dot(xs, wu_v[...], preferred_element_type=F32))
    h = (_rb(g * _rb(_sigmoid(g))) * uu).astype(BF)
    y = _rb(lax.dot_general(h, wdT_v[...], (((1,), (1,)), ((), ())),
                            preferred_element_type=F32))
    y = _rb(y * _rb(_sigmoid(rsel)))
    ypad = jnp.concatenate([y, jnp.zeros((112, D), F32)], axis=0)
    ypad = jnp.concatenate([ypad, jnp.zeros((128, DP - D), F32)], axis=1)
    yT = ypad.T[0:D, :].astype(BF)
    oh = jnp.concatenate([onehot, jnp.zeros((112, S), F32)], axis=0).astype(BF)

    for c in range(XC):
        cols = slice(c * XR, (c + 1) * XR)
        upd = jnp.dot(yT, oh[:, cols], preferred_element_type=F32)
        z = _unpack(xnT_p[:, cols]).astype(F32) + upd
        gt = z * _sigmoid(z)
        tpc = XR // TQ
        s_att = jnp.concatenate([accT[c * tpc + i] for i in range(tpc)], axis=1)
        outT_v[:, cols] = (xT_v[:, cols].astype(F32) + s_att * gt).astype(BF)
        out_copy(c).start()
    for c in range(XC):
        out_copy(c).wait()


@jax.jit
def pallas_recurrent_scan__gqa_block_cached__moe_arch_mod__prompt_kernel(
    A_x: jax.Array,
    A_k_cache: jax.Array,
    A_v_cache: jax.Array,
    A_wq: jax.Array,
    A_wo: jax.Array,
    B_x: jax.Array,
    B_w_r: jax.Array,
    B_w_gate: jax.Array,
    B_w_up: jax.Array,
    B_w_down: jax.Array,
):
    del B_x
    xT = A_x.reshape(S, D).T
    woT = A_wo.T
    wdT = B_w_down.T
    k = A_k_cache.reshape(HKV, S, DH)
    v = A_v_cache.reshape(HKV, S, DH)
    wr = B_w_r.reshape(1, D)

    hbm = pl.BlockSpec(memory_space=pltpu.HBM)
    vmem = pl.BlockSpec(memory_space=pltpu.VMEM)
    outT = pl.pallas_call(
        _kernel,
        out_shape=jax.ShapeDtypeStruct((D, S), BF),
        in_specs=[hbm, hbm, hbm, hbm, hbm, vmem, hbm, hbm, hbm],
        out_specs=hbm,
        scratch_shapes=[
            pltpu.VMEM((D, S), BF),
            pltpu.VMEM((D // 2, S), U32),
            pltpu.VMEM((S // 2, DP), U32),
            pltpu.VMEM((S // TQ, D, TQ), F32),
            pltpu.VMEM((HKV, S, DH), BF),
            pltpu.VMEM((HKV, S, DH), BF),
            pltpu.VMEM((DP, HQ * DH), BF),
            pltpu.VMEM((D, HQ * DH), BF),
            pltpu.VMEM((D, F), BF),
            pltpu.VMEM((D, F), BF),
            pltpu.VMEM((D, F), BF),
            pltpu.VMEM((UN, TQ, DH), U32),
            pltpu.VMEM((UN, TQ // 2, 2 * DH), U32),
            pltpu.VMEM((16, DP), F32),
            pltpu.VMEM((D, S), BF),
            pltpu.VMEM((8, DH), F32),
            pltpu.VMEM((8, DH), F32),
            pltpu.VMEM((8, 2 * DH), F32),
            pltpu.VMEM((8, DH), F32),
            pltpu.SemaphoreType.DMA((XC,)),
            pltpu.SemaphoreType.DMA((4 * HKV,)),
            pltpu.SemaphoreType.DMA((3,)),
            pltpu.SemaphoreType.DMA((XC,)),
        ],
        compiler_params=pltpu.CompilerParams(vmem_limit_bytes=100 * 1024 * 1024,
                                             disable_bounds_checks=True),
        name="fused_attn_moe",
    )(xT, k, v, A_wq, woT, wr, B_w_gate, B_w_up, wdT)
    return outT.T.reshape(1, S, D)
```

```python
import functools
import math

import jax
import jax.numpy as jnp
from jax import lax
import jax.experimental.pallas as pl
import jax.experimental.pallas.tpu as pltpu

S = 2048
D = 576
DP = 640
HQ = 32
HKV = 16
DH = 128
F = 4608
C = 8
EPS_BF16 = 1.0013580322265625e-05

TQ = 128
UN = 4
CH = 512
TPH = S // TQ
IPH = TPH // UN
NIT = HKV * IPH
XC = 8
XR = S // XC

BF = jnp.bfloat16
F32 = jnp.float32
U32 = jnp.uint32
QSCALE = (DH ** -0.5) * math.log2(math.e)
LOG_IPH = IPH.bit_length() - 1
assert 1 << LOG_IPH == IPH

SCORE_BOUND = 40.0
V_HI = 2.0 ** 60
V_LO = 2.0 ** -60


def _rb(v):
    return v.astype(BF).astype(F32)


def _pack(v_bf16):
    return pltpu.bitcast(v_bf16, U32)


def _unpack(v_u32):
    return pltpu.bitcast(v_u32, BF)


def _fold(x, op):
    r = x[:, 0:128]
    for j in range(1, x.shape[1] // 128):
        r = op(r, x[:, j * 128:(j + 1) * 128])
    return r


def _sigmoid(v):
    return 0.5 * jnp.tanh(0.5 * v) + 0.5


def _recip(v):
    r = pl.reciprocal(v, approx=True)
    return r * (2.0 - v * r)


def _kernel(xT_hbm, k_hbm, v_hbm, wq_hbm, woT_hbm, wr_ref, wg_hbm, wu_hbm, wdT_hbm,
            outT_hbm,
            xT_v, xnT_p, xn_p, accT, k_v, v_v, wq_v, woT_v, wg_v, wu_v, wdT_v,
            q_buf, o_buf, xs_v, outT_v, kst, vst, wst, xnm,
            sem_x, sem_h, sem_m, sem_o):

    def x_copy(c):
        return pltpu.make_async_copy(
            xT_hbm.at[:, pl.ds(c * XR, XR)], xT_v.at[:, pl.ds(c * XR, XR)], sem_x.at[c])

    k_p, v_p = k_hbm.bitcast(U32), v_hbm.bitcast(U32)
    wq_p, woT_p = wq_hbm.bitcast(U32), woT_hbm.bitcast(U32)

    def head_copies(j):
        col = pl.multiple_of(j * (2 * DH), 2 * DH)
        return [
            pltpu.make_async_copy(wq_p.at[:, pl.ds(col, 2 * DH)],
                                  wq_v.at[j, pl.ds(0, D // 2), :], sem_h.at[4 * j]),
            pltpu.make_async_copy(k_p.at[j], k_v.at[j], sem_h.at[4 * j + 1]),
            pltpu.make_async_copy(v_p.at[j], v_v.at[j], sem_h.at[4 * j + 2]),
            pltpu.make_async_copy(woT_p.at[:, pl.ds(col, 2 * DH)], woT_v.at[j],
                                  sem_h.at[4 * j + 3]),
        ]

    def moe_copies():
        return [pltpu.make_async_copy(wg_hbm.bitcast(U32), wg_v, sem_m.at[0]),
                pltpu.make_async_copy(wu_hbm.bitcast(U32), wu_v, sem_m.at[1]),
                pltpu.make_async_copy(wdT_hbm.bitcast(U32), wdT_v, sem_m.at[2])]

    def out_copy(c):
        return pltpu.make_async_copy(
            outT_v.at[:, pl.ds(c * XR, XR)], outT_hbm.at[:, pl.ds(c * XR, XR)], sem_o.at[c])

    for c in range(XC):
        x_copy(c).start()
    accT[...] = jnp.zeros(accT.shape, F32)
    o_buf[...] = jnp.zeros(o_buf.shape, U32)
    wq_v[:, D // 2:DP // 2, :] = jnp.zeros((HKV, (DP - D) // 2, 2 * DH), U32)
    xs_v[...] = jnp.zeros(xs_v.shape, F32)

    n2max = None
    for c in range(XC):
        x_copy(c).wait()
        cols = slice(c * XR, (c + 1) * XR)
        xf = xT_v[:, cols].astype(F32)
        mean = jnp.sum(xf, axis=0, keepdims=True) / D
        cen = xf - mean
        var = jnp.sum(cen * cen, axis=0, keepdims=True) / D
        mean_b = _rb(mean)
        dlt = _rb(xf - mean_b)
        sd = _rb(jnp.sqrt(_rb(_rb(var) + EPS_BF16)))
        n2 = D * (var + (mean - mean_b) * (mean - mean_b)) / (sd * sd)
        n2max = n2 if n2max is None else jnp.maximum(n2max, n2)
        xnT = (dlt / sd).astype(BF)
        xnT_p[:, cols] = _pack(xnT)
        xpad = jnp.concatenate([xnT, jnp.zeros((DP - D, XR), BF)], axis=0)
        xn_p[c * XR // 2:(c + 1) * XR // 2, :] = _pack(xpad.T)
        if c == 2:
            for cp in head_copies(0):
                cp.start()
        if c == XC - 1:
            for cp in head_copies(1):
                cp.start()
    xnm[...] = jnp.broadcast_to(_fold(n2max, jnp.maximum), (8, DH))

    def qproj(j, row0, a):
        r2 = pl.multiple_of(lax.shift_right_logical(row0, 1), UN * TQ // 2)
        xb = _unpack(xn_p[pl.ds(pl.multiple_of(r2 + a * (TQ // 2), TQ // 2), TQ // 2), :])
        q2 = jnp.dot(xb, _unpack(wq_v[j]), preferred_element_type=F32)
        q2 = (q2 * QSCALE).astype(BF)
        q_buf[a, 0:TQ // 2, :] = _pack(q2[:, 0:DH])
        q_buf[a, TQ // 2:TQ, :] = _pack(q2[:, DH:2 * DH])

    def oproj(j, row0, a):
        t = lax.shift_right_logical(row0, TQ.bit_length() - 1) + a
        o2 = _unpack(o_buf[a])
        upd = lax.dot_general(_unpack(woT_v[j]), o2, (((1,), (1,)), ((), ())),
                              preferred_element_type=F32)
        accT[t] = accT[t] + upd

    def attention(j, a, fast):
        q = _unpack(q_buf[a])
        m = l = acc = None
        for c in range(S // CH):
            kc = _unpack(k_v[j, c * CH // 2:(c + 1) * CH // 2, :])
            s = lax.dot_general(q, kc, (((1,), (1,)), ((), ())),
                                preferred_element_type=F32)
            if fast:
                p = jnp.exp2(s)
            else:
                mc = jnp.broadcast_to(
                    jnp.max(_fold(s, jnp.maximum), axis=1, keepdims=True), (2 * TQ, 128))
                m_new = mc if m is None else jnp.maximum(m, mc)
                p = jnp.exp2(s - jnp.tile(m_new, (1, CH // 128)))
            lc = _fold(p, jnp.add)
            pv = jnp.dot(p.astype(BF), _unpack(v_v[j, c * CH // 2:(c + 1) * CH // 2, :]),
                         preferred_element_type=F32)
            if l is None:
                l, acc = lc, pv
            elif fast:
                l, acc = l + lc, acc + pv
            else:
                alpha = jnp.exp2(m - m_new)
                l, acc = l * alpha + lc, acc * alpha + pv
            if not fast:
                m = m_new
        ls = jnp.sum(l, axis=1, keepdims=True)
        o = (acc * _recip(ls)).astype(BF)
        o_buf[a, :, 0:DH] = _pack(o[0:TQ])
        o_buf[a, :, DH:2 * DH] = _pack(o[TQ:2 * TQ])

    def _absmax_packed(w):
        w = w & jnp.uint32(0x7FFF7FFF)
        hi = lax.bitcast_convert_type(w, F32)
        lo = lax.bitcast_convert_type(w << 16, F32)
        m = jnp.maximum(hi, lo)
        r = m[0:8]
        for i in range(1, m.shape[0] // 8):
            r = jnp.maximum(r, m[i * 8:(i + 1) * 8])
        return r

    def head_stats(j, i, nparts):
        first = i == 0
        kr = S // 2 // nparts
        r0 = pl.multiple_of(i * kr, kr)
        km = _absmax_packed(k_v[j, pl.ds(r0, kr), :])
        vm = _absmax_packed(v_v[j, pl.ds(r0, kr), :])
        km = jnp.where(first, km, jnp.maximum(km, kst[...]))
        vm = jnp.where(first, vm, jnp.maximum(vm, vst[...]))
        kst[...] = km
        vst[...] = vm
        wr_ = DP // 2 // nparts
        w0 = pl.multiple_of(i * wr_, 8)
        wf = _unpack(wq_v[j, pl.ds(w0, wr_), :]).astype(F32)
        w2 = wf * wf
        ws = w2[0:8]
        for t in range(1, 2 * wr_ // 8):
            ws = ws + w2[t * 8:(t + 1) * 8]
        ws = jnp.where(first, ws, ws + wst[...])
        wst[...] = ws
        wn2 = jnp.sum(ws, axis=0, keepdims=True)
        wn = jnp.sqrt(jnp.maximum(wn2[:, 0:DH], wn2[:, DH:2 * DH]))
        kmx = jnp.max(km, axis=0, keepdims=True)
        xn = jnp.sqrt(jnp.max(xnm[0:1, :], axis=1, keepdims=True))
        bound = jnp.sum(wn * kmx, axis=1, keepdims=True) * xn * (1.05 * QSCALE)
        vmx = jnp.max(jnp.max(vm, axis=0, keepdims=True), axis=1, keepdims=True)
        ok = jnp.logical_and(bound <= SCORE_BOUND,
                             jnp.logical_and(vmx <= V_HI, vmx >= V_LO))
        return jnp.max(jnp.where(ok, 1.0, 0.0)).astype(jnp.int32)

    for cp in head_copies(0):
        cp.wait()
    safe0 = head_stats(0, 0, 1)
    for a in range(UN):
        qproj(0, 0, a)

    def body(u, safe):
        j = lax.shift_right_logical(u, LOG_IPH)
        i = u & (IPH - 1)
        un = jnp.minimum(u + 1, NIT - 1)
        jn = lax.shift_right_logical(un, LOG_IPH)
        up = jnp.maximum(u - 1, 0)
        jp = lax.shift_right_logical(up, LOG_IPH)
        js = jnp.minimum(j + 1, HKV - 1)

        @pl.when(i == 0)
        def _():
            @pl.when(j + 1 < HKV)
            def _():
                for cp in head_copies(j + 1):
                    cp.wait()

            @pl.when(j + 2 < HKV)
            def _():
                for cp in head_copies(j + 2):
                    cp.start()

        @pl.when(u == IPH)
        def _():
            for cp in moe_copies():
                cp.start()

        rown = (un & (IPH - 1)) * (UN * TQ)
        rowp = (up & (IPH - 1)) * (UN * TQ)

        def task(a, fast):
            oproj(jp, rowp, a)
            attention(j, a, fast)
            qproj(jn, rown, a)

        def work(fast):
            if fast:
                for a in range(UN):
                    task(a, True)
            else:
                def slow_task(a, c):
                    task(a, False)
                    return c
                lax.fori_loop(0, UN, slow_task, 0)
            return head_stats(js, i, IPH)

        nxt = lax.cond(safe > 0, lambda: work(True), lambda: work(False))
        return jnp.where(i == IPH - 1, nxt, safe)

    lax.fori_loop(0, NIT, body, safe0)
    for a in range(UN):
        oproj(HKV - 1, S - UN * TQ, a)

    for cp in moe_copies():
        cp.wait()
    wr = jnp.broadcast_to(wr_ref[...], (16, D))
    r = jnp.dot(wr, _unpack(xnT_p[...]), preferred_element_type=F32)
    r = _rb(r[0:8, :])
    col = lax.broadcasted_iota(jnp.int32, (8, S), 1).astype(F32)
    row16 = lax.broadcasted_iota(jnp.int32, (16, S), 0)
    col16 = lax.broadcasted_iota(jnp.int32, (16, S), 1)
    rowg = lax.broadcasted_iota(jnp.int32, (16, 1), 0)
    onehot = jnp.zeros((16, S), F32)
    rsel = jnp.zeros((16, 1), F32)
    for c in range(C):
        mx = jnp.max(r)
        idx_f = jnp.min(jnp.where(r == mx, col, float(S)))
        idx = jnp.minimum(idx_f.astype(jnp.int32), S - 1)
        r = jnp.where(col == idx_f, -jnp.inf, r)
        onehot = jnp.where(jnp.logical_and(row16 == c, col16 == idx), 1.0, onehot)
        rsel = jnp.where(rowg == c, mx, rsel)
        w = xn_p[pl.ds(idx // 2, 1), :]
        w = jnp.where(idx % 2 == 0, w << 16, w & jnp.uint32(0xFFFF0000))
        xs_v[c:c + 1, :] = lax.bitcast_convert_type(w, F32)
    xs = xs_v[:, 0:D].astype(BF)
    g = _rb(jnp.dot(xs, _unpack(wg_v[...]), preferred_element_type=F32))
    uu = _rb(jnp.dot(xs, _unpack(wu_v[...]), preferred_element_type=F32))
    h = (_rb(g * _rb(_sigmoid(g))) * uu).astype(BF)
    y = _rb(lax.dot_general(h, _unpack(wdT_v[...]), (((1,), (1,)), ((), ())),
                            preferred_element_type=F32))
    y = _rb(y * _rb(_sigmoid(rsel)))
    ypad = jnp.concatenate([y, jnp.zeros((112, D), F32)], axis=0)
    ypad = jnp.concatenate([ypad, jnp.zeros((128, DP - D), F32)], axis=1)
    yT = ypad.T[0:D, :].astype(BF)
    oh = jnp.concatenate([onehot, jnp.zeros((112, S), F32)], axis=0).astype(BF)

    for c in range(XC):
        cols = slice(c * XR, (c + 1) * XR)
        upd = jnp.dot(yT, oh[:, cols], preferred_element_type=F32)
        z = _unpack(xnT_p[:, cols]).astype(F32) + upd
        gt = z * _sigmoid(z)
        tpc = XR // TQ
        s_att = jnp.concatenate([accT[c * tpc + i] for i in range(tpc)], axis=1)
        outT_v[:, cols] = (xT_v[:, cols].astype(F32) + s_att * gt).astype(BF)
        out_copy(c).start()
    for c in range(XC):
        out_copy(c).wait()


@jax.jit
def pallas_recurrent_scan__gqa_block_cached__moe_arch_mod__prompt_kernel(
    A_x: jax.Array,
    A_k_cache: jax.Array,
    A_v_cache: jax.Array,
    A_wq: jax.Array,
    A_wo: jax.Array,
    B_x: jax.Array,
    B_w_r: jax.Array,
    B_w_gate: jax.Array,
    B_w_up: jax.Array,
    B_w_down: jax.Array,
):
    del B_x
    xT = A_x.reshape(S, D).T
    woT = A_wo.T
    wdT = B_w_down.T
    k = A_k_cache.reshape(HKV, S, DH)
    v = A_v_cache.reshape(HKV, S, DH)
    wr = B_w_r.reshape(1, D)

    hbm = pl.BlockSpec(memory_space=pltpu.HBM)
    vmem = pl.BlockSpec(memory_space=pltpu.VMEM)
    outT = pl.pallas_call(
        _kernel,
        out_shape=jax.ShapeDtypeStruct((D, S), BF),
        in_specs=[hbm, hbm, hbm, hbm, hbm, vmem, hbm, hbm, hbm],
        out_specs=hbm,
        scratch_shapes=[
            pltpu.VMEM((D, S), BF),
            pltpu.VMEM((D // 2, S), U32),
            pltpu.VMEM((S // 2, DP), U32),
            pltpu.VMEM((S // TQ, D, TQ), F32),
            pltpu.VMEM((HKV, S // 2, DH), U32),
            pltpu.VMEM((HKV, S // 2, DH), U32),
            pltpu.VMEM((HKV, DP // 2, 2 * DH), U32),
            pltpu.VMEM((HKV, D // 2, 2 * DH), U32),
            pltpu.VMEM((D // 2, F), U32),
            pltpu.VMEM((D // 2, F), U32),
            pltpu.VMEM((D // 2, F), U32),
            pltpu.VMEM((UN, TQ, DH), U32),
            pltpu.VMEM((UN, TQ // 2, 2 * DH), U32),
            pltpu.VMEM((16, DP), F32),
            pltpu.VMEM((D, S), BF),
            pltpu.VMEM((8, DH), F32),
            pltpu.VMEM((8, DH), F32),
            pltpu.VMEM((8, 2 * DH), F32),
            pltpu.VMEM((8, DH), F32),
            pltpu.SemaphoreType.DMA((XC,)),
            pltpu.SemaphoreType.DMA((4 * HKV,)),
            pltpu.SemaphoreType.DMA((3,)),
            pltpu.SemaphoreType.DMA((XC,)),
        ],
        compiler_params=pltpu.CompilerParams(vmem_limit_bytes=100 * 1024 * 1024,
                                             disable_bounds_checks=True),
        name="fused_attn_moe",
    )(xT, k, v, A_wq, woT, wr, B_w_gate, B_w_up, wdT)
    return outT.T.reshape(1, S, D)
```

```python
import functools
import math

import jax
import jax.numpy as jnp
from jax import lax
import jax.experimental.pallas as pl
import jax.experimental.pallas.tpu as pltpu

S = 2048
D = 576
DP = 640
HQ = 32
HKV = 16
DH = 128
F = 4608
C = 8
EPS_BF16 = 1.0013580322265625e-05

TQ = 128
UN = 4
CH = 512
TPH = S // TQ
IPH = TPH // UN
XC = 8
XR = S // XC

BF = jnp.bfloat16
F32 = jnp.float32
U32 = jnp.uint32
QSCALE = (DH ** -0.5) * math.log2(math.e)

SCORE_BOUND = 40.0
V_HI = 2.0 ** 60
V_LO = 2.0 ** -60


def _rb(v):
    return v.astype(BF).astype(F32)


def _pack(v_bf16):
    return pltpu.bitcast(v_bf16, U32)


def _unpack(v_u32):
    return pltpu.bitcast(v_u32, BF)


def _fold(x, op):
    r = x[:, 0:128]
    for j in range(1, x.shape[1] // 128):
        r = op(r, x[:, j * 128:(j + 1) * 128])
    return r


def _sigmoid(v):
    return 0.5 * jnp.tanh(0.5 * v) + 0.5


def _recip(v):
    r = pl.reciprocal(v, approx=True)
    return r * (2.0 - v * r)


def _kernel(xT_hbm, k_hbm, v_hbm, wq_hbm, woT_hbm, wr_ref, wg_hbm, wu_hbm, wdT_hbm,
            outT_hbm,
            xT_v, xnT_p, xn_p, accT, k_v, v_v, wq_v, woT_v, wg_v, wu_v, wdT_v,
            q_buf, o_buf, xs_v, outT_v, kst, vst, wst, xnm,
            sem_x, sem_h, sem_m, sem_o):

    def x_copy(c):
        return pltpu.make_async_copy(
            xT_hbm.at[:, pl.ds(c * XR, XR)], xT_v.at[:, pl.ds(c * XR, XR)], sem_x.at[c])

    k_p, v_p = k_hbm.bitcast(U32), v_hbm.bitcast(U32)
    wq_p, woT_p = wq_hbm.bitcast(U32), woT_hbm.bitcast(U32)

    def head_copies(j):
        col = pl.multiple_of(j * (2 * DH), 2 * DH)
        return [
            pltpu.make_async_copy(wq_p.at[:, pl.ds(col, 2 * DH)],
                                  wq_v.at[j, pl.ds(0, D // 2), :], sem_h.at[4 * j]),
            pltpu.make_async_copy(k_p.at[j], k_v.at[j], sem_h.at[4 * j + 1]),
            pltpu.make_async_copy(v_p.at[j], v_v.at[j], sem_h.at[4 * j + 2]),
            pltpu.make_async_copy(woT_p.at[:, pl.ds(col, 2 * DH)], woT_v.at[j],
                                  sem_h.at[4 * j + 3]),
        ]

    def moe_copies():
        return [pltpu.make_async_copy(wg_hbm.bitcast(U32), wg_v, sem_m.at[0]),
                pltpu.make_async_copy(wu_hbm.bitcast(U32), wu_v, sem_m.at[1]),
                pltpu.make_async_copy(wdT_hbm.bitcast(U32), wdT_v, sem_m.at[2])]

    def out_copy(c):
        return pltpu.make_async_copy(
            outT_v.at[:, pl.ds(c * XR, XR)], outT_hbm.at[:, pl.ds(c * XR, XR)], sem_o.at[c])

    for c in range(XC):
        x_copy(c).start()
    accT[...] = jnp.zeros(accT.shape, F32)
    o_buf[...] = jnp.zeros(o_buf.shape, U32)
    wq_v[:, D // 2:DP // 2, :] = jnp.zeros((HKV, (DP - D) // 2, 2 * DH), U32)
    xs_v[...] = jnp.zeros(xs_v.shape, F32)

    n2max = None
    for c in range(XC):
        x_copy(c).wait()
        cols = slice(c * XR, (c + 1) * XR)
        xf = xT_v[:, cols].astype(F32)
        mean = jnp.sum(xf, axis=0, keepdims=True) / D
        cen = xf - mean
        var = jnp.sum(cen * cen, axis=0, keepdims=True) / D
        mean_b = _rb(mean)
        dlt = _rb(xf - mean_b)
        sd = _rb(jnp.sqrt(_rb(_rb(var) + EPS_BF16)))
        n2 = D * (var + (mean - mean_b) * (mean - mean_b)) / (sd * sd)
        n2max = n2 if n2max is None else jnp.maximum(n2max, n2)
        xnT = (dlt / sd).astype(BF)
        xnT_p[:, cols] = _pack(xnT)
        xpad = jnp.concatenate([xnT, jnp.zeros((DP - D, XR), BF)], axis=0)
        xn_p[c * XR // 2:(c + 1) * XR // 2, :] = _pack(xpad.T)
        if c == 2:
            for cp in head_copies(0):
                cp.start()
        if c == XC - 1:
            for cp in head_copies(1):
                cp.start()
    xnm[...] = jnp.broadcast_to(_fold(n2max, jnp.maximum), (8, DH))

    def qproj(j, t):
        r2 = pl.multiple_of(t * (TQ // 2), TQ // 2)
        xb = _unpack(xn_p[pl.ds(r2, TQ // 2), :])
        q2 = jnp.dot(xb, _unpack(wq_v[j]), preferred_element_type=F32)
        q2 = (q2 * QSCALE).astype(BF)
        return jnp.concatenate([_pack(q2[:, 0:DH]), _pack(q2[:, DH:2 * DH])], axis=0)

    def oproj(j, t, o2p):
        upd = lax.dot_general(_unpack(woT_v[j]), _unpack(o2p), (((1,), (1,)), ((), ())),
                              preferred_element_type=F32)
        accT[t] = accT[t] + upd

    def attention(j, qp, fast):
        q = _unpack(qp)
        m = l = acc = None
        for c in range(S // CH):
            kc = _unpack(k_v[j, c * CH // 2:(c + 1) * CH // 2, :])
            s = lax.dot_general(q, kc, (((1,), (1,)), ((), ())),
                                preferred_element_type=F32)
            if fast:
                p = jnp.exp2(s)
            else:
                mc = jnp.broadcast_to(
                    jnp.max(_fold(s, jnp.maximum), axis=1, keepdims=True), (2 * TQ, 128))
                m_new = mc if m is None else jnp.maximum(m, mc)
                p = jnp.exp2(s - jnp.tile(m_new, (1, CH // 128)))
            lc = _fold(p, jnp.add)
            pv = jnp.dot(p.astype(BF), _unpack(v_v[j, c * CH // 2:(c + 1) * CH // 2, :]),
                         preferred_element_type=F32)
            if l is None:
                l, acc = lc, pv
            elif fast:
                l, acc = l + lc, acc + pv
            else:
                alpha = jnp.exp2(m - m_new)
                l, acc = l * alpha + lc, acc * alpha + pv
            if not fast:
                m = m_new
        ls = jnp.sum(l, axis=1, keepdims=True)
        o = (acc * _recip(ls)).astype(BF)
        return jnp.concatenate([_pack(o[0:TQ]), _pack(o[TQ:2 * TQ])], axis=1)

    def _absmax_packed(w):
        w = w & jnp.uint32(0x7FFF7FFF)
        hi = lax.bitcast_convert_type(w, F32)
        lo = lax.bitcast_convert_type(w << 16, F32)
        m = jnp.maximum(hi, lo)
        r = m[0:8]
        for i in range(1, m.shape[0] // 8):
            r = jnp.maximum(r, m[i * 8:(i + 1) * 8])
        return r

    def head_stats(j, i, nparts):
        first = i == 0
        kr = S // 2 // nparts
        r0 = pl.multiple_of(i * kr, kr)
        km = _absmax_packed(k_v[j, pl.ds(r0, kr), :])
        vm = _absmax_packed(v_v[j, pl.ds(r0, kr), :])
        km = jnp.where(first, km, jnp.maximum(km, kst[...]))
        vm = jnp.where(first, vm, jnp.maximum(vm, vst[...]))
        kst[...] = km
        vst[...] = vm
        wr_ = DP // 2 // nparts
        w0 = pl.multiple_of(i * wr_, 8)
        wf = _unpack(wq_v[j, pl.ds(w0, wr_), :]).astype(F32)
        w2 = wf * wf
        ws = w2[0:8]
        for t in range(1, 2 * wr_ // 8):
            ws = ws + w2[t * 8:(t + 1) * 8]
        ws = jnp.where(first, ws, ws + wst[...])
        wst[...] = ws
        wn2 = jnp.sum(ws, axis=0, keepdims=True)
        wn = jnp.sqrt(jnp.maximum(wn2[:, 0:DH], wn2[:, DH:2 * DH]))
        kmx = jnp.max(km, axis=0, keepdims=True)
        xn = jnp.sqrt(jnp.max(xnm[0:1, :], axis=1, keepdims=True))
        bound = jnp.sum(wn * kmx, axis=1, keepdims=True) * xn * (1.05 * QSCALE)
        vmx = jnp.max(jnp.max(vm, axis=0, keepdims=True), axis=1, keepdims=True)
        ok = jnp.logical_and(bound <= SCORE_BOUND,
                             jnp.logical_and(vmx <= V_HI, vmx >= V_LO))
        return jnp.max(jnp.where(ok, 1.0, 0.0)).astype(jnp.int32)

    for cp in head_copies(0):
        cp.wait()
    safe0 = head_stats(0, 0, 1)
    for a in range(UN):
        q_buf[a] = qproj(0, a)

    def block_coords(j, i):
        first = i == 0
        last = i == IPH - 1
        jp = jnp.where(first, jnp.maximum(j - 1, 0), j)
        tp = jnp.where(first, IPH - 1, i - 1) * UN
        jn = jnp.where(last, jnp.minimum(j + 1, HKV - 1), j)
        tn = jnp.where(last, 0, i + 1) * UN
        return jp, tp, jn, tn

    def task(j, coords, a, fast):
        jp, tp, jn, tn = coords
        oproj(jp, tp + a, o_buf[a])
        o_buf[a] = attention(j, q_buf[a], fast)
        q_buf[a] = qproj(jn, tn + a)

    def head_body(j, safe):
        @pl.when(j + 1 < HKV)
        def _():
            for cp in head_copies(j + 1):
                cp.wait()

        @pl.when(j + 2 < HKV)
        def _():
            for cp in head_copies(j + 2):
                cp.start()

        @pl.when(j == 1)
        def _():
            for cp in moe_copies():
                cp.start()

        js = jnp.minimum(j + 1, HKV - 1)

        def fast_head():
            def it(i, c):
                coords = block_coords(j, i)
                for a in range(UN):
                    task(j, coords, a, True)
                return head_stats(js, i, IPH)
            return lax.fori_loop(0, IPH, it, 0)

        def slow_head():
            def it(t, c):
                task(j, block_coords(j, t // UN), t % UN, False)
                return c
            lax.fori_loop(0, TPH, it, 0)
            return head_stats(js, 0, 1)

        return lax.cond(safe > 0, fast_head, slow_head)

    lax.fori_loop(0, HKV, head_body, safe0)
    for a in range(UN):
        oproj(HKV - 1, TPH - UN + a, o_buf[a])

    for cp in moe_copies():
        cp.wait()
    wr = jnp.broadcast_to(wr_ref[...], (16, D))
    r = jnp.dot(wr, _unpack(xnT_p[...]), preferred_element_type=F32)
    r = _rb(r[0:8, :])
    col = lax.broadcasted_iota(jnp.int32, (8, S), 1).astype(F32)
    row16 = lax.broadcasted_iota(jnp.int32, (16, S), 0)
    col16 = lax.broadcasted_iota(jnp.int32, (16, S), 1)
    rowg = lax.broadcasted_iota(jnp.int32, (16, 1), 0)
    onehot = jnp.zeros((16, S), F32)
    rsel = jnp.zeros((16, 1), F32)
    for c in range(C):
        mx = jnp.max(r)
        idx_f = jnp.min(jnp.where(r == mx, col, float(S)))
        idx = jnp.minimum(idx_f.astype(jnp.int32), S - 1)
        r = jnp.where(col == idx_f, -jnp.inf, r)
        onehot = jnp.where(jnp.logical_and(row16 == c, col16 == idx), 1.0, onehot)
        rsel = jnp.where(rowg == c, mx, rsel)
        w = xn_p[pl.ds(idx // 2, 1), :]
        w = jnp.where(idx % 2 == 0, w << 16, w & jnp.uint32(0xFFFF0000))
        xs_v[c:c + 1, :] = lax.bitcast_convert_type(w, F32)
    xs = xs_v[:, 0:D].astype(BF)
    g = _rb(jnp.dot(xs, _unpack(wg_v[...]), preferred_element_type=F32))
    uu = _rb(jnp.dot(xs, _unpack(wu_v[...]), preferred_element_type=F32))
    h = (_rb(g * _rb(_sigmoid(g))) * uu).astype(BF)
    y = _rb(lax.dot_general(h, _unpack(wdT_v[...]), (((1,), (1,)), ((), ())),
                            preferred_element_type=F32))
    y = _rb(y * _rb(_sigmoid(rsel)))
    ypad = jnp.concatenate([y, jnp.zeros((112, D), F32)], axis=0)
    ypad = jnp.concatenate([ypad, jnp.zeros((128, DP - D), F32)], axis=1)
    yT = ypad.T[0:D, :].astype(BF)
    oh = jnp.concatenate([onehot, jnp.zeros((112, S), F32)], axis=0).astype(BF)

    for c in range(XC):
        cols = slice(c * XR, (c + 1) * XR)
        upd = jnp.dot(yT, oh[:, cols], preferred_element_type=F32)
        z = _unpack(xnT_p[:, cols]).astype(F32) + upd
        gt = z * _sigmoid(z)
        tpc = XR // TQ
        s_att = jnp.concatenate([accT[c * tpc + i] for i in range(tpc)], axis=1)
        outT_v[:, cols] = (xT_v[:, cols].astype(F32) + s_att * gt).astype(BF)
        out_copy(c).start()
    for c in range(XC):
        out_copy(c).wait()


@jax.jit
def pallas_recurrent_scan__gqa_block_cached__moe_arch_mod__prompt_kernel(
    A_x: jax.Array,
    A_k_cache: jax.Array,
    A_v_cache: jax.Array,
    A_wq: jax.Array,
    A_wo: jax.Array,
    B_x: jax.Array,
    B_w_r: jax.Array,
    B_w_gate: jax.Array,
    B_w_up: jax.Array,
    B_w_down: jax.Array,
):
    del B_x
    xT = A_x.reshape(S, D).T
    woT = A_wo.T
    wdT = B_w_down.T
    k = A_k_cache.reshape(HKV, S, DH)
    v = A_v_cache.reshape(HKV, S, DH)
    wr = B_w_r.reshape(1, D)

    hbm = pl.BlockSpec(memory_space=pltpu.HBM)
    vmem = pl.BlockSpec(memory_space=pltpu.VMEM)
    outT = pl.pallas_call(
        _kernel,
        out_shape=jax.ShapeDtypeStruct((D, S), BF),
        in_specs=[hbm, hbm, hbm, hbm, hbm, vmem, hbm, hbm, hbm],
        out_specs=hbm,
        scratch_shapes=[
            pltpu.VMEM((D, S), BF),
            pltpu.VMEM((D // 2, S), U32),
            pltpu.VMEM((S // 2, DP), U32),
            pltpu.VMEM((S // TQ, D, TQ), F32),
            pltpu.VMEM((HKV, S // 2, DH), U32),
            pltpu.VMEM((HKV, S // 2, DH), U32),
            pltpu.VMEM((HKV, DP // 2, 2 * DH), U32),
            pltpu.VMEM((HKV, D // 2, 2 * DH), U32),
            pltpu.VMEM((D // 2, F), U32),
            pltpu.VMEM((D // 2, F), U32),
            pltpu.VMEM((D // 2, F), U32),
            pltpu.VMEM((UN, TQ, DH), U32),
            pltpu.VMEM((UN, TQ // 2, 2 * DH), U32),
            pltpu.VMEM((16, DP), F32),
            pltpu.VMEM((D, S), BF),
            pltpu.VMEM((8, DH), F32),
            pltpu.VMEM((8, DH), F32),
            pltpu.VMEM((8, 2 * DH), F32),
            pltpu.VMEM((8, DH), F32),
            pltpu.SemaphoreType.DMA((XC,)),
            pltpu.SemaphoreType.DMA((4 * HKV,)),
            pltpu.SemaphoreType.DMA((3,)),
            pltpu.SemaphoreType.DMA((XC,)),
        ],
        compiler_params=pltpu.CompilerParams(vmem_limit_bytes=100 * 1024 * 1024,
                                             disable_bounds_checks=True),
        name="fused_attn_moe",
    )(xT, k, v, A_wq, woT, wr, B_w_gate, B_w_up, wdT)
    return outT.T.reshape(1, S, D)
```

```python
import functools
import math

import jax
import jax.numpy as jnp
from jax import lax
import jax.experimental.pallas as pl
import jax.experimental.pallas.tpu as pltpu

S = 2048
D = 576
DP = 640
HQ = 32
HKV = 16
DH = 128
F = 4608
C = 8
EPS_BF16 = 1.0013580322265625e-05

TQ = 128
UN = 8
CH = 512
TPH = S // TQ
IPH = TPH // UN
XC = 8
XR = S // XC

BF = jnp.bfloat16
F32 = jnp.float32
U32 = jnp.uint32
QSCALE = (DH ** -0.5) * math.log2(math.e)

SCORE_BOUND = 40.0
V_HI = 2.0 ** 60
V_LO = 2.0 ** -60


def _rb(v):
    return v.astype(BF).astype(F32)


def _pack(v_bf16):
    return pltpu.bitcast(v_bf16, U32)


def _unpack(v_u32):
    return pltpu.bitcast(v_u32, BF)


def _fold(x, op):
    r = x[:, 0:128]
    for j in range(1, x.shape[1] // 128):
        r = op(r, x[:, j * 128:(j + 1) * 128])
    return r


def _sigmoid(v):
    return 0.5 * jnp.tanh(0.5 * v) + 0.5


def _recip(v):
    r = pl.reciprocal(v, approx=True)
    return r * (2.0 - v * r)


def _kernel(xT_hbm, k_hbm, v_hbm, wq_hbm, woT_hbm, wr_ref, wg_hbm, wu_hbm, wdT_hbm,
            outT_hbm,
            xT_v, xnT_p, xn_p, accT, k_v, v_v, wq_v, woT_v, wg_v, wu_v, wdT_v,
            q_buf, xs_v, outT_v, kst, vst, wst, xnm, rs_v, yT_p, sel_s,
            sem_x, sem_h, sem_m, sem_o):

    def x_copy(c):
        return pltpu.make_async_copy(
            xT_hbm.at[:, pl.ds(c * XR, XR)], xT_v.at[c], sem_x.at[c])

    k_p, v_p = k_hbm.bitcast(U32), v_hbm.bitcast(U32)
    wq_p, woT_p = wq_hbm.bitcast(U32), woT_hbm.bitcast(U32)

    def head_copies(j):
        col = pl.multiple_of(j * (2 * DH), 2 * DH)
        return [
            pltpu.make_async_copy(wq_p.at[:, pl.ds(col, 2 * DH)],
                                  wq_v.at[j, pl.ds(0, D // 2), :], sem_h.at[4 * j]),
            pltpu.make_async_copy(k_p.at[j], k_v.at[j], sem_h.at[4 * j + 1]),
            pltpu.make_async_copy(v_p.at[j], v_v.at[j], sem_h.at[4 * j + 2]),
            pltpu.make_async_copy(woT_p.at[:, pl.ds(col, 2 * DH)], woT_v.at[j],
                                  sem_h.at[4 * j + 3]),
        ]

    def moe_copies():
        return [pltpu.make_async_copy(wg_hbm.bitcast(U32), wg_v, sem_m.at[0]),
                pltpu.make_async_copy(wu_hbm.bitcast(U32), wu_v, sem_m.at[1]),
                pltpu.make_async_copy(wdT_hbm.bitcast(U32), wdT_v, sem_m.at[2])]

    def out_copy(c):
        cols = pl.ds(pl.multiple_of(c * XR, XR), XR)
        return pltpu.make_async_copy(outT_v.at[c], outT_hbm.at[:, cols], sem_o.at[c])

    for c in range(XC):
        x_copy(c).start()
    accT[...] = jnp.zeros(accT.shape, F32)
    wq_v[:, D // 2:DP // 2, :] = jnp.zeros((HKV, (DP - D) // 2, 2 * DH), U32)
    xs_v[...] = jnp.zeros(xs_v.shape, F32)

    n2max = None
    for c in range(XC):
        x_copy(c).wait()
        xf = xT_v[c].astype(F32)
        mean = jnp.sum(xf, axis=0, keepdims=True) / D
        cen = xf - mean
        var = jnp.sum(cen * cen, axis=0, keepdims=True) / D
        mean_b = _rb(mean)
        dlt = _rb(xf - mean_b)
        sd = _rb(jnp.sqrt(_rb(_rb(var) + EPS_BF16)))
        n2 = D * (var + (mean - mean_b) * (mean - mean_b)) / (sd * sd)
        n2max = n2 if n2max is None else jnp.maximum(n2max, n2)
        xnT = (dlt / sd).astype(BF)
        xnT_p[c] = _pack(xnT)
        xpad = jnp.concatenate([xnT, jnp.zeros((DP - D, XR), BF)], axis=0)
        xn_p[c * XR // 2:(c + 1) * XR // 2, :] = _pack(xpad.T)
        if c == 2:
            for cp in head_copies(0):
                cp.start()
        if c == XC - 1:
            for cp in head_copies(1):
                cp.start()
    xnm[0:8] = jnp.broadcast_to(_fold(n2max, jnp.maximum), (8, DH))

    def qproj(j, t):
        r2 = pl.multiple_of(t * (TQ // 2), TQ // 2)
        xb = _unpack(xn_p[pl.ds(r2, TQ // 2), :])
        q2 = jnp.dot(xb, _unpack(wq_v[j]), preferred_element_type=F32)
        q2 = (q2 * QSCALE).astype(BF)
        return jnp.concatenate([_pack(q2[:, 0:DH]), _pack(q2[:, DH:2 * DH])], axis=0)

    def oproj(j, t, o2p):
        upd = lax.dot_general(_unpack(woT_v[j]), _unpack(o2p), (((1,), (1,)), ((), ())),
                              preferred_element_type=F32)
        accT[t] = accT[t] + upd

    def attention(j, qp, fast):
        q = _unpack(qp)
        m = l = acc = None
        for c in range(S // CH):
            kc = _unpack(k_v[j, c * CH // 2:(c + 1) * CH // 2, :])
            s = lax.dot_general(q, kc, (((1,), (1,)), ((), ())),
                                preferred_element_type=F32)
            if fast:
                p = jnp.exp2(s)
            else:
                mc = jnp.broadcast_to(
                    jnp.max(_fold(s, jnp.maximum), axis=1, keepdims=True), (2 * TQ, 128))
                m_new = mc if m is None else jnp.maximum(m, mc)
                p = jnp.exp2(s - jnp.tile(m_new, (1, CH // 128)))
            lc = _fold(p, jnp.add)
            pv = jnp.dot(p.astype(BF), _unpack(v_v[j, c * CH // 2:(c + 1) * CH // 2, :]),
                         preferred_element_type=F32)
            if l is None:
                l, acc = lc, pv
            elif fast:
                l, acc = l + lc, acc + pv
            else:
                alpha = jnp.exp2(m - m_new)
                l, acc = l * alpha + lc, acc * alpha + pv
            if not fast:
                m = m_new
        ls = jnp.sum(l, axis=1, keepdims=True)
        o = (acc * _recip(ls)).astype(BF)
        return jnp.concatenate([_pack(o[0:TQ]), _pack(o[TQ:2 * TQ])], axis=1)

    def _absmax_packed(w):
        w = w & jnp.uint32(0x7FFF7FFF)
        hi = lax.bitcast_convert_type(w, F32)
        lo = lax.bitcast_convert_type(w << 16, F32)
        m = jnp.maximum(hi, lo)
        r = m[0:8]
        for i in range(1, m.shape[0] // 8):
            r = jnp.maximum(r, m[i * 8:(i + 1) * 8])
        return r

    def head_stats(j, i, nparts):
        first = i == 0
        kr = S // 2 // nparts
        r0 = pl.multiple_of(i * kr, kr)
        km = _absmax_packed(k_v[j, pl.ds(r0, kr), :])
        vm = _absmax_packed(v_v[j, pl.ds(r0, kr), :])
        km = jnp.where(first, km, jnp.maximum(km, kst[0:8]))
        vm = jnp.where(first, vm, jnp.maximum(vm, vst[0:8]))
        kst[0:8] = km
        vst[0:8] = vm
        wr_ = DP // 2 // nparts
        w0 = pl.multiple_of(i * wr_, 8)
        wf = _unpack(wq_v[j, pl.ds(w0, wr_), :]).astype(F32)
        w2 = wf * wf
        ws = w2[0:8]
        for t in range(1, 2 * wr_ // 8):
            ws = ws + w2[t * 8:(t + 1) * 8]
        ws = jnp.where(first, ws, ws + wst[0:8])
        wst[0:8] = ws
        wn2 = jnp.sum(ws, axis=0, keepdims=True)
        wn = jnp.sqrt(jnp.maximum(wn2[:, 0:DH], wn2[:, DH:2 * DH]))
        kmx = jnp.max(km, axis=0, keepdims=True)
        xn = jnp.sqrt(jnp.max(xnm[0:1, :], axis=1, keepdims=True))
        bound = jnp.sum(wn * kmx, axis=1, keepdims=True) * xn * (1.05 * QSCALE)
        vmx = jnp.max(jnp.max(vm, axis=0, keepdims=True), axis=1, keepdims=True)
        ok = jnp.logical_and(bound <= SCORE_BOUND,
                             jnp.logical_and(vmx <= V_HI, vmx >= V_LO))
        return jnp.max(jnp.where(ok, 1.0, 0.0)).astype(jnp.int32)

    def moe_route():
        wr = jnp.broadcast_to(wr_ref[...], (16, D))
        xnT_all = jnp.concatenate([_unpack(xnT_p[c]) for c in range(XC)], axis=1)
        r = jnp.dot(wr, xnT_all, preferred_element_type=F32)
        r = _rb(r[0:8, :])
        col = lax.broadcasted_iota(jnp.int32, (8, S), 1).astype(F32)
        rowg = lax.broadcasted_iota(jnp.int32, (16, 128), 0)
        rsel = jnp.zeros((16, 128), F32)
        for c in range(C):
            mx = jnp.max(r)
            idx_f = jnp.min(jnp.where(r == mx, col, float(S)))
            idx = jnp.clip(idx_f.astype(jnp.int32), 0, S - 1)
            r = jnp.where(col == idx_f, -jnp.inf, r)
            rsel = jnp.where(rowg == c, mx, rsel)
            sel_s[c] = idx
            w = xn_p[pl.ds(lax.shift_right_logical(idx, 1), 1), :]
            w = jnp.where((idx & 1) == 0, w << 16, w & jnp.uint32(0xFFFF0000))
            xs_v[c:c + 1, :] = lax.bitcast_convert_type(w, F32)
        rs_v[0:16] = rsel

    def moe_ffn():
        for cp in moe_copies():
            cp.wait()
        xs = xs_v[0:16, 0:D].astype(BF)
        g = _rb(jnp.dot(xs, _unpack(wg_v[...]), preferred_element_type=F32))
        uu = _rb(jnp.dot(xs, _unpack(wu_v[...]), preferred_element_type=F32))
        h = (_rb(g * _rb(_sigmoid(g))) * uu).astype(BF)
        y = _rb(lax.dot_general(h, _unpack(wdT_v[...]), (((1,), (1,)), ((), ())),
                                preferred_element_type=F32))
        y = _rb(y * _rb(_sigmoid(rs_v[0:16, 0:1])))
        ypad = jnp.concatenate([y, jnp.zeros((112, D), F32)], axis=0)
        ypad = jnp.concatenate([ypad, jnp.zeros((128, DP - D), F32)], axis=1)
        yT_p[...] = _pack(ypad.T[0:D, :].astype(BF))

    def final(c):
        row = lax.broadcasted_iota(jnp.int32, (16, XR), 0)
        tok = lax.broadcasted_iota(jnp.int32, (16, XR), 1) + c * XR
        onehot = jnp.zeros((16, XR), F32)
        for k in range(C):
            onehot = jnp.where(jnp.logical_and(row == k, tok == sel_s[k]), 1.0, onehot)
        onehot = jnp.concatenate([onehot, jnp.zeros((112, XR), F32)], axis=0).astype(BF)
        upd = jnp.dot(_unpack(yT_p[...]), onehot, preferred_element_type=F32)
        z = _unpack(xnT_p[c]).astype(F32) + upd
        s_att = jnp.concatenate([accT[2 * c], accT[2 * c + 1]], axis=1)
        outT_v[c] = (xT_v[c].astype(F32) + s_att * (z * _sigmoid(z))).astype(BF)

    for cp in head_copies(0):
        cp.wait()
    moe_route()
    safe0 = head_stats(0, 0, 1)
    for a in range(UN):
        q_buf[a] = qproj(0, a)

    def block(j, i, tasks, fast):
        last = i == IPH - 1
        jn = jnp.where(last, jnp.minimum(j + 1, HKV - 1), j)
        tn = jnp.where(last, 0, i + 1) * UN
        outs = [attention(j, q_buf[a], fast) for a in tasks]
        for a in tasks:
            q_buf[a] = qproj(jn, tn + a)
        for a, op in zip(tasks, outs):
            oproj(j, i * UN + a, op)

    def finish(c0, n):
        def fin(k, carry):
            for c in (c0 + 2 * k, c0 + 2 * k + 1):
                final(c)
                out_copy(c).start()
            return carry
        lax.fori_loop(0, n // 2, fin, 0)

    def head_body(j, safe):
        @pl.when(j + 1 < HKV)
        def _():
            for cp in head_copies(j + 1):
                cp.wait()

        @pl.when(j + 2 < HKV)
        def _():
            for cp in head_copies(j + 2):
                cp.start()

        @pl.when(j == 1)
        def _():
            for cp in moe_copies():
                cp.start()

        @pl.when(j == HKV - 1)
        def _():
            moe_ffn()

        js = jnp.minimum(j + 1, HKV - 1)

        def fast_head():
            def it(i, c):
                block(j, i, range(UN), True)
                flag = head_stats(js, i, IPH)

                @pl.when(j == HKV - 1)
                def _():
                    finish(i * (UN // 2), UN // 2)
                return flag
            return lax.fori_loop(0, IPH, it, 0)

        def slow_head():
            def it(t, c):
                block(j, t // UN, [t % UN], False)
                return c
            lax.fori_loop(0, TPH, it, 0)

            @pl.when(j == HKV - 1)
            def _():
                finish(0, XC)
            return head_stats(js, 0, 1)

        return lax.cond(safe > 0, fast_head, slow_head)

    lax.fori_loop(0, HKV, head_body, safe0)
    for c in range(XC):
        out_copy(c).wait()


@jax.jit
def pallas_recurrent_scan__gqa_block_cached__moe_arch_mod__prompt_kernel(
    A_x: jax.Array,
    A_k_cache: jax.Array,
    A_v_cache: jax.Array,
    A_wq: jax.Array,
    A_wo: jax.Array,
    B_x: jax.Array,
    B_w_r: jax.Array,
    B_w_gate: jax.Array,
    B_w_up: jax.Array,
    B_w_down: jax.Array,
):
    del B_x
    xT = A_x.reshape(S, D).T
    woT = A_wo.T
    wdT = B_w_down.T
    k = A_k_cache.reshape(HKV, S, DH)
    v = A_v_cache.reshape(HKV, S, DH)
    wr = B_w_r.reshape(1, D)

    hbm = pl.BlockSpec(memory_space=pltpu.HBM)
    vmem = pl.BlockSpec(memory_space=pltpu.VMEM)
    outT = pl.pallas_call(
        _kernel,
        out_shape=jax.ShapeDtypeStruct((D, S), BF),
        in_specs=[hbm, hbm, hbm, hbm, hbm, vmem, hbm, hbm, hbm],
        out_specs=hbm,
        scratch_shapes=[
            pltpu.VMEM((XC, D, XR), BF),
            pltpu.VMEM((XC, D // 2, XR), U32),
            pltpu.VMEM((S // 2, DP), U32),
            pltpu.VMEM((S // TQ, D, TQ), F32),
            pltpu.VMEM((HKV, S // 2, DH), U32),
            pltpu.VMEM((HKV, S // 2, DH), U32),
            pltpu.VMEM((HKV, DP // 2, 2 * DH), U32),
            pltpu.VMEM((HKV, D // 2, 2 * DH), U32),
            pltpu.VMEM((D // 2, F), U32),
            pltpu.VMEM((D // 2, F), U32),
            pltpu.VMEM((D // 2, F), U32),
            pltpu.VMEM((UN, TQ, DH), U32),
            pltpu.VMEM((32, DP), F32),
            pltpu.VMEM((XC, D, XR), BF),
            pltpu.VMEM((32, DH), F32),
            pltpu.VMEM((32, DH), F32),
            pltpu.VMEM((16, 2 * DH), F32),
            pltpu.VMEM((32, DH), F32),
            pltpu.VMEM((32, 128), F32),
            pltpu.VMEM((D // 2, 128), U32),
            pltpu.SMEM((C,), jnp.int32),
            pltpu.SemaphoreType.DMA((XC,)),
            pltpu.SemaphoreType.DMA((4 * HKV,)),
            pltpu.SemaphoreType.DMA((3,)),
            pltpu.SemaphoreType.DMA((XC,)),
        ],
        compiler_params=pltpu.CompilerParams(vmem_limit_bytes=100 * 1024 * 1024,
                                             disable_bounds_checks=True),
        name="fused_attn_moe",
    )(xT, k, v, A_wq, woT, wr, B_w_gate, B_w_up, wdT)
    return outT.T.reshape(1, S, D)
```

```python
import functools
import math

import jax
import jax.numpy as jnp
from jax import lax
import jax.experimental.pallas as pl
import jax.experimental.pallas.tpu as pltpu

S = 2048
D = 576
DP = 640
HQ = 32
HKV = 16
DH = 128
F = 4608
C = 8
EPS_BF16 = 1.0013580322265625e-05

TQ = 128
UN = 8
CH = 512
TPH = S // TQ
IPH = TPH // UN
WSL = 5 if UN == 8 else 2
XC = 8
XR = S // XC

BF = jnp.bfloat16
F32 = jnp.float32
U32 = jnp.uint32
QSCALE = (DH ** -0.5) * math.log2(math.e)

SCORE_BOUND = 40.0
V_HI = 2.0 ** 60
V_LO = 2.0 ** -60


def _rb(v):
    return v.astype(BF).astype(F32)


def _pack(v_bf16):
    return pltpu.bitcast(v_bf16, U32)


def _unpack(v_u32):
    return pltpu.bitcast(v_u32, BF)


def _fold(x, op):
    r = x[:, 0:128]
    for j in range(1, x.shape[1] // 128):
        r = op(r, x[:, j * 128:(j + 1) * 128])
    return r


def _sigmoid(v):
    return 0.5 * jnp.tanh(0.5 * v) + 0.5


def _recip(v):
    r = pl.reciprocal(v, approx=True)
    return r * (2.0 - v * r)


def _kernel(xT_hbm, k_hbm, v_hbm, wq_hbm, woT_hbm, wr_ref, wg_hbm, wu_hbm, wdT_hbm,
            outT_hbm,
            xT_v, xnT_p, xn_p, accT, k_v, v_v, wq_v, woT_v, wg_v, wu_v, wdT_v,
            q_buf, xs_v, outT_v, kst, vst, wst, xnm, rs_v, yT_p, sel_s,
            sem_x, sem_h, sem_m, sem_o):

    def x_copy(c):
        return pltpu.make_async_copy(
            xT_hbm.at[:, pl.ds(c * XR, XR)], xT_v.at[c], sem_x.at[c])

    k_p, v_p = k_hbm.bitcast(U32), v_hbm.bitcast(U32)
    wq_p, woT_p = wq_hbm.bitcast(U32), woT_hbm.bitcast(U32)

    def head_copies(j, which=(0, 1, 2, 3)):
        col = pl.multiple_of(j * (2 * DH), 2 * DH)
        pairs = [
            (wq_p.at[:, pl.ds(col, 2 * DH)], wq_v.at[j, pl.ds(0, D // 2), :]),
            (k_p.at[j], k_v.at[j]),
            (v_p.at[j], v_v.at[j]),
            (woT_p.at[:, pl.ds(col, 2 * DH)], woT_v.at[j]),
        ]
        return [pltpu.make_async_copy(*pairs[w], sem_h.at[4 * j + w]) for w in which]

    def moe_copies():
        return [pltpu.make_async_copy(wg_hbm.bitcast(U32), wg_v, sem_m.at[0]),
                pltpu.make_async_copy(wu_hbm.bitcast(U32), wu_v, sem_m.at[1]),
                pltpu.make_async_copy(wdT_hbm.bitcast(U32), wdT_v, sem_m.at[2])]

    def out_copy(c):
        cols = pl.ds(pl.multiple_of(c * XR, XR), XR)
        return pltpu.make_async_copy(outT_v.at[c], outT_hbm.at[:, cols], sem_o.at[c])

    for c in range(XC // 2):
        x_copy(c).start()
    head_copies(0, (0,))[0].start()
    for c in range(XC // 2, XC):
        x_copy(c).start()

    wq_v[:, D // 2:DP // 2, :] = jnp.zeros((HKV, (DP - D) // 2, 2 * DH), U32)
    xs_v[...] = jnp.zeros(xs_v.shape, F32)

    def ln_chunk(c):
        xf = xT_v[c].astype(F32)
        mean = jnp.sum(xf, axis=0, keepdims=True) / D
        cen = xf - mean
        var = jnp.sum(cen * cen, axis=0, keepdims=True) / D
        mean_b = _rb(mean)
        dlt = _rb(xf - mean_b)
        sd = _rb(jnp.sqrt(_rb(_rb(var) + EPS_BF16)))
        xnT_p[c] = _pack((dlt / sd).astype(BF))
        return D * (var + (mean - mean_b) * (mean - mean_b)) / (sd * sd)

    def tr_chunk(c):
        xpad = jnp.concatenate([_unpack(xnT_p[c]), jnp.zeros((DP - D, XR), BF)], axis=0)
        xn_p[c * XR // 2:(c + 1) * XR // 2, :] = _pack(xpad.T)

    n2max = None
    for c in range(XC // 2):
        x_copy(c).wait()
        n2 = ln_chunk(c)
        n2max = n2 if n2max is None else jnp.maximum(n2max, n2)
        if c > 0:
            tr_chunk(c - 1)

    def qproj(j, t, scale=QSCALE):
        r2 = pl.multiple_of(t * (TQ // 2), TQ // 2)
        xb = _unpack(xn_p[pl.ds(r2, TQ // 2), :])
        q2 = jnp.dot(xb, _unpack(wq_v[j]), preferred_element_type=F32)
        q2 = (q2 * scale).astype(BF)
        return jnp.concatenate([_pack(q2[:, 0:DH]), _pack(q2[:, DH:2 * DH])], axis=0)

    def oproj(j, t, o2p):
        upd = lax.dot_general(_unpack(woT_v[j]), _unpack(o2p), (((1,), (1,)), ((), ())),
                              preferred_element_type=F32)
        accT[t] = jnp.where(j == 0, upd, accT[t] + upd)

    def attention(j, qp, fast):
        q = _unpack(qp)
        m = l = acc = None
        for c in range(S // CH):
            kc = _unpack(k_v[j, c * CH // 2:(c + 1) * CH // 2, :])
            s = lax.dot_general(q, kc, (((1,), (1,)), ((), ())),
                                preferred_element_type=F32)
            if fast:
                p = jnp.exp2(s)
            else:
                mc = jnp.broadcast_to(
                    jnp.max(_fold(s, jnp.maximum), axis=1, keepdims=True), (2 * TQ, 128))
                m_new = mc if m is None else jnp.maximum(m, mc)
                p = jnp.exp2(s - jnp.tile(m_new, (1, CH // 128)))
            lc = _fold(p, jnp.add)
            pv = jnp.dot(p.astype(BF), _unpack(v_v[j, c * CH // 2:(c + 1) * CH // 2, :]),
                         preferred_element_type=F32)
            if l is None:
                l, acc = lc, pv
            elif fast:
                l, acc = l + lc, acc + pv
            else:
                alpha = jnp.exp2(m - m_new)
                l, acc = l * alpha + lc, acc * alpha + pv
            if not fast:
                m = m_new
        ls = jnp.sum(l, axis=1, keepdims=True)
        o = (acc * _recip(ls)).astype(BF)
        return jnp.concatenate([_pack(o[0:TQ]), _pack(o[TQ:2 * TQ])], axis=1)

    def _absmax_packed(w):
        w = w & jnp.uint32(0x7FFF7FFF)
        hi = lax.bitcast_convert_type(w, F32)
        lo = lax.bitcast_convert_type(w << 16, F32)
        m = jnp.maximum(hi, lo)
        return _fold8(m, jnp.maximum)

    def _fold8(m, op):
        r = m[0:8]
        for i in range(1, m.shape[0] // 8):
            r = op(r, m[i * 8:(i + 1) * 8])
        return r

    def stats_fold(j, st, k0, nk, w0, nw):
        km, vm, ws = st
        km = jnp.maximum(km, _absmax_packed(k_v[j, pl.ds(k0, nk), :]))
        vm = jnp.maximum(vm, _absmax_packed(v_v[j, pl.ds(k0, nk), :]))
        if nw:
            wf = _unpack(wq_v[j, pl.ds(w0, nw), :]).astype(F32)
            ws = ws + _fold8(wf * wf, jnp.add)
        return km, vm, ws

    def stats_flag(st):
        km, vm, ws = st
        wn2 = jnp.sum(ws, axis=0, keepdims=True)
        wn = jnp.sqrt(jnp.maximum(wn2[:, 0:DH], wn2[:, DH:2 * DH]))
        kmx = jnp.max(km, axis=0, keepdims=True)
        xn = jnp.sqrt(jnp.max(xnm[0:1, :], axis=1, keepdims=True))
        bound = jnp.sum(wn * kmx, axis=1, keepdims=True) * xn * (1.05 * QSCALE)
        vmx = jnp.max(jnp.max(vm, axis=0, keepdims=True), axis=1, keepdims=True)
        ok = jnp.logical_and(bound <= SCORE_BOUND,
                             jnp.logical_and(vmx <= V_HI, vmx >= V_LO))
        return jnp.max(jnp.where(ok, 1.0, 0.0)).astype(jnp.int32)

    def stats_zero():
        return (jnp.zeros((8, DH), F32), jnp.zeros((8, DH), F32), jnp.zeros((8, 2 * DH), F32))

    def head_stats(j):
        return stats_flag(stats_fold(j, stats_zero(), 0, S // 2, 0, DP // 2))

    def moe_route():
        wr = jnp.broadcast_to(wr_ref[...], (16, D))
        xnT_all = jnp.concatenate([_unpack(xnT_p[c]) for c in range(XC)], axis=1)
        r = jnp.dot(wr, xnT_all, preferred_element_type=F32)
        r = _rb(r[0:8, :])
        col = lax.broadcasted_iota(jnp.int32, (8, S), 1)
        r = jnp.where(r == r, jnp.clip(r, -3e38, 3e38), -3e38)
        bits = lax.bitcast_convert_type(r, jnp.int32) & jnp.int32(-65536)
        bits = jnp.where(jnp.abs(r) < 2.0 ** -126, jnp.int32(0x00800000), bits)
        low = jnp.where(bits < 0, col, (S - 1) - col)
        key = lax.bitcast_convert_type(bits | low, F32)
        rowg = lax.broadcasted_iota(jnp.int32, (16, 128), 0)
        rsel = jnp.zeros((16, 128), F32)
        for c in range(C):
            mx = jnp.max(key, axis=1, keepdims=True)
            key = jnp.where(key == mx, -jnp.inf, key)
            mb = lax.bitcast_convert_type(mx, jnp.int32)
            lowb = mb & (S - 1)
            idx_v = jnp.where(mb < 0, lowb, (S - 1) - lowb)
            idx = jnp.max(idx_v)
            val = lax.bitcast_convert_type(mb & jnp.int32(-65536), F32)[0:1, :]
            rsel = jnp.where(rowg == c, val, rsel)
            sel_s[c] = idx
            w = xn_p[pl.ds(lax.shift_right_logical(idx, 1), 1), :]
            w = jnp.where((idx & 1) == 0, w << 16, w & jnp.uint32(0xFFFF0000))
            xs_v[c:c + 1, :] = lax.bitcast_convert_type(w, F32)
        rs_v[0:16] = rsel

    def moe_ffn():
        for cp in moe_copies():
            cp.wait()
        xs = xs_v[0:16, 0:D].astype(BF)
        g = _rb(jnp.dot(xs, _unpack(wg_v[...]), preferred_element_type=F32))
        uu = _rb(jnp.dot(xs, _unpack(wu_v[...]), preferred_element_type=F32))
        h = (_rb(g * _rb(_sigmoid(g))) * uu).astype(BF)
        y = _rb(lax.dot_general(h, _unpack(wdT_v[...]), (((1,), (1,)), ((), ())),
                                preferred_element_type=F32))
        y = _rb(y * _rb(_sigmoid(rs_v[0:16, 0:1])))
        ypad = jnp.concatenate([y, jnp.zeros((112, D), F32)], axis=0)
        ypad = jnp.concatenate([ypad, jnp.zeros((128, DP - D), F32)], axis=1)
        yT_p[...] = _pack(ypad.T[0:D, :].astype(BF))

    def final(c):
        row = lax.broadcasted_iota(jnp.int32, (16, XR), 0)
        tok = lax.broadcasted_iota(jnp.int32, (16, XR), 1) + c * XR
        onehot = jnp.zeros((16, XR), F32)
        for k in range(C):
            onehot = jnp.where(jnp.logical_and(row == k, tok == sel_s[k]), 1.0, onehot)
        onehot = jnp.concatenate([onehot, jnp.zeros((112, XR), F32)], axis=0).astype(BF)
        upd = jnp.dot(_unpack(yT_p[...]), onehot, preferred_element_type=F32)
        z = _unpack(xnT_p[c]).astype(F32) + upd
        s_att = jnp.concatenate([accT[2 * c], accT[2 * c + 1]], axis=1)
        outT_v[c] = (xT_v[c].astype(F32) + s_att * (z * _sigmoid(z))).astype(BF)

    head_copies(0, (0,))[0].wait()
    for cp in head_copies(0, (1, 2, 3)):
        cp.start()
    tr_chunk(XC // 2 - 1)
    for a in range(UN):
        q_buf[a] = qproj(0, a)
    for c in range(XC // 2, XC):
        x_copy(c).wait()
    for cp in head_copies(1):
        cp.start()
    for c in range(XC // 2, XC):
        n2max = jnp.maximum(n2max, ln_chunk(c))
        tr_chunk(c)
    xnm[0:8] = jnp.broadcast_to(_fold(n2max, jnp.maximum), (8, DH))
    moe_route()
    for cp in head_copies(0, (1, 2, 3)):
        cp.wait()
    safe0 = head_stats(0)

    def block(j, i, tasks, fast):
        last = i == IPH - 1
        jn = jnp.where(last, jnp.minimum(j + 1, HKV - 1), j)
        tn = jnp.where(last, 0, i + 1) * UN
        outs = [attention(j, q_buf[a], fast) for a in tasks]
        if not fast:
            for a in tasks:
                q_buf[a] = qproj(jn, tn + a)
            for a, op in zip(tasks, outs):
                oproj(j, i * UN + a, op)
            return None
        js = jnp.minimum(j + 1, HKV - 1)
        first = i == 0
        st = tuple(jnp.where(first, z, old)
                   for z, old in zip(stats_zero(), (kst[0:8], vst[0:8], wst[0:8])))
        nk = S // 2 // TPH
        nw = DP // 2 // IPH // WSL
        for a in tasks:
            k0 = pl.multiple_of((i * UN + a) * nk, nk)
            w0 = pl.multiple_of((i * WSL + a) * nw, 8)
            st = stats_fold(js, st, k0, nk, w0, nw if a < WSL else 0)
            zero = jnp.minimum(jnp.minimum(st[0][0:1, :], st[1][0:1, :]), 0.0)
            scale = QSCALE + jnp.minimum(jnp.concatenate([zero, zero], axis=1), st[2][0:1, :])
            q_buf[a] = qproj(jn, tn + a, scale)
        kst[0:8], vst[0:8], wst[0:8] = st
        for a, op in zip(tasks, outs):
            oproj(j, i * UN + a, op)
        return stats_flag(st)

    def finish(c0, n):
        def fin(k, carry):
            for c in (c0 + 2 * k, c0 + 2 * k + 1):
                final(c)
                out_copy(c).start()
            return carry
        lax.fori_loop(0, n // 2, fin, 0)

    def head_body(j, safe):
        @pl.when(j + 1 < HKV)
        def _():
            for cp in head_copies(j + 1):
                cp.wait()

        @pl.when(j + 2 < HKV)
        def _():
            for cp in head_copies(j + 2):
                cp.start()

        @pl.when(j == 1)
        def _():
            for cp in moe_copies():
                cp.start()

        @pl.when(j == HKV - 1)
        def _():
            moe_ffn()

        js = jnp.minimum(j + 1, HKV - 1)

        def fast_head():
            def it(i, c):
                flag = block(j, i, range(UN), True)

                @pl.when(j == HKV - 1)
                def _():
                    finish(i * (UN // 2), UN // 2)
                return flag
            return lax.fori_loop(0, IPH, it, 0)

        def slow_head():
            def it(t, c):
                block(j, t // UN, [t % UN], False)
                return c
            lax.fori_loop(0, TPH, it, 0)

            @pl.when(j == HKV - 1)
            def _():
                finish(0, XC)
            return head_stats(js)

        return lax.cond(safe > 0, fast_head, slow_head)

    lax.fori_loop(0, HKV, head_body, safe0)
    for c in range(XC):
        out_copy(c).wait()


@jax.jit
def pallas_recurrent_scan__gqa_block_cached__moe_arch_mod__prompt_kernel(
    A_x: jax.Array,
    A_k_cache: jax.Array,
    A_v_cache: jax.Array,
    A_wq: jax.Array,
    A_wo: jax.Array,
    B_x: jax.Array,
    B_w_r: jax.Array,
    B_w_gate: jax.Array,
    B_w_up: jax.Array,
    B_w_down: jax.Array,
):
    del B_x
    xT = A_x.reshape(S, D).T
    woT = A_wo.T
    wdT = B_w_down.T
    k = A_k_cache.reshape(HKV, S, DH)
    v = A_v_cache.reshape(HKV, S, DH)
    wr = B_w_r.reshape(1, D)

    hbm = pl.BlockSpec(memory_space=pltpu.HBM)
    vmem = pl.BlockSpec(memory_space=pltpu.VMEM)
    outT = pl.pallas_call(
        _kernel,
        out_shape=jax.ShapeDtypeStruct((D, S), BF),
        in_specs=[hbm, hbm, hbm, hbm, hbm, vmem, hbm, hbm, hbm],
        out_specs=hbm,
        scratch_shapes=[
            pltpu.VMEM((XC, D, XR), BF),
            pltpu.VMEM((XC, D // 2, XR), U32),
            pltpu.VMEM((S // 2, DP), U32),
            pltpu.VMEM((S // TQ, D, TQ), F32),
            pltpu.VMEM((HKV, S // 2, DH), U32),
            pltpu.VMEM((HKV, S // 2, DH), U32),
            pltpu.VMEM((HKV, DP // 2, 2 * DH), U32),
            pltpu.VMEM((HKV, D // 2, 2 * DH), U32),
            pltpu.VMEM((D // 2, F), U32),
            pltpu.VMEM((D // 2, F), U32),
            pltpu.VMEM((D // 2, F), U32),
            pltpu.VMEM((UN, TQ, DH), U32),
            pltpu.VMEM((32, DP), F32),
            pltpu.VMEM((XC, D, XR), BF),
            pltpu.VMEM((32, DH), F32),
            pltpu.VMEM((32, DH), F32),
            pltpu.VMEM((16, 2 * DH), F32),
            pltpu.VMEM((32, DH), F32),
            pltpu.VMEM((32, 128), F32),
            pltpu.VMEM((D // 2, 128), U32),
            pltpu.SMEM((C,), jnp.int32),
            pltpu.SemaphoreType.DMA((XC,)),
            pltpu.SemaphoreType.DMA((4 * HKV,)),
            pltpu.SemaphoreType.DMA((3,)),
            pltpu.SemaphoreType.DMA((XC,)),
        ],
        compiler_params=pltpu.CompilerParams(vmem_limit_bytes=100 * 1024 * 1024,
                                             disable_bounds_checks=True),
        name="fused_attn_moe",
    )(xT, k, v, A_wq, woT, wr, B_w_gate, B_w_up, wdT)
    return outT.T.reshape(1, S, D)
```

```python
import functools
import math

import jax
import jax.numpy as jnp
from jax import lax
import jax.experimental.pallas as pl
import jax.experimental.pallas.tpu as pltpu

S = 2048
D = 576
DP = 640
HQ = 32
HKV = 16
DH = 128
F = 4608
C = 8
EPS_BF16 = 1.0013580322265625e-05

TQ = 128
UN = 8
CH = 512
TPH = S // TQ
IPH = TPH // UN
WSL = 5 if UN == 8 else 2
HEAD0_AT = 3
HEAD1_AT = 7
XC = 8
XR = S // XC

BF = jnp.bfloat16
F32 = jnp.float32
U32 = jnp.uint32
QSCALE = (DH ** -0.5) * math.log2(math.e)

SCORE_BOUND = 40.0
V_HI = 2.0 ** 60
V_LO = 2.0 ** -60


def _rb(v):
    return v.astype(BF).astype(F32)


def _pack(v_bf16):
    return pltpu.bitcast(v_bf16, U32)


def _unpack(v_u32):
    return pltpu.bitcast(v_u32, BF)


def _fold(x, op):
    r = x[:, 0:128]
    for j in range(1, x.shape[1] // 128):
        r = op(r, x[:, j * 128:(j + 1) * 128])
    return r


def _sigmoid(v):
    return 0.5 * jnp.tanh(0.5 * v) + 0.5


def _recip(v):
    r = pl.reciprocal(v, approx=True)
    return r * (2.0 - v * r)


def _kernel(xT_hbm, k_hbm, v_hbm, wq_hbm, woT_hbm, wr_ref, wg_hbm, wu_hbm, wdT_hbm,
            outT_hbm,
            xT_v, xnT_p, xn_p, accT, k_v, v_v, wq_v, woT_v, wg_v, wu_v, wdT_v,
            xs_v, outT_v, kst, vst, wst, xnm, rs_v, yT_p, sel_s,
            sem_x, sem_h, sem_m, sem_o):

    def x_copy(c):
        return pltpu.make_async_copy(
            xT_hbm.at[:, pl.ds(c * XR, XR)], xT_v.at[c], sem_x.at[c])

    k_p, v_p = k_hbm.bitcast(U32), v_hbm.bitcast(U32)
    wq_p, woT_p = wq_hbm.bitcast(U32), woT_hbm.bitcast(U32)

    def head_copies(j):
        col = pl.multiple_of(j * (2 * DH), 2 * DH)
        pairs = [
            (wq_p.at[:, pl.ds(col, 2 * DH)], wq_v.at[j, pl.ds(0, D // 2), :]),
            (k_p.at[j], k_v.at[j]),
            (v_p.at[j], v_v.at[j]),
            (woT_p.at[:, pl.ds(col, 2 * DH)], woT_v.at[j]),
        ]
        return [pltpu.make_async_copy(*pairs[w], sem_h.at[4 * j + w]) for w in range(4)]

    def moe_copies():
        return [pltpu.make_async_copy(wg_hbm.bitcast(U32), wg_v, sem_m.at[0]),
                pltpu.make_async_copy(wu_hbm.bitcast(U32), wu_v, sem_m.at[1]),
                pltpu.make_async_copy(wdT_hbm.bitcast(U32), wdT_v, sem_m.at[2])]

    def out_copy(c):
        cols = pl.ds(pl.multiple_of(c * XR, XR), XR)
        return pltpu.make_async_copy(outT_v.at[c], outT_hbm.at[:, cols], sem_o.at[c])

    for c in range(XC):
        x_copy(c).start()

    wq_v[:, D // 2:DP // 2, :] = jnp.zeros((HKV, (DP - D) // 2, 2 * DH), U32)
    xs_v[...] = jnp.zeros(xs_v.shape, F32)

    def ln_chunk(c):
        xf = xT_v[c].astype(F32)
        mean = jnp.sum(xf, axis=0, keepdims=True) / D
        cen = xf - mean
        var = jnp.sum(cen * cen, axis=0, keepdims=True) / D
        mean_b = _rb(mean)
        dlt = _rb(xf - mean_b)
        sd = _rb(jnp.sqrt(_rb(_rb(var) + EPS_BF16)))
        xnT_p[c] = _pack((dlt / sd).astype(BF))
        return D * (var + (mean - mean_b) * (mean - mean_b)) / (sd * sd)

    def tr_chunk(c):
        xpad = jnp.concatenate([_unpack(xnT_p[c]), jnp.zeros((DP - D, XR), BF)], axis=0)
        xn_p[c * XR // 2:(c + 1) * XR // 2, :] = _pack(xpad.T)

    n2max = None
    for c in range(XC):
        x_copy(c).wait()
        n2 = ln_chunk(c)
        n2max = n2 if n2max is None else jnp.maximum(n2max, n2)
        if c > 0:
            tr_chunk(c - 1)
        if c == HEAD0_AT:
            for cp in head_copies(0):
                cp.start()
        if c == HEAD1_AT:
            for cp in head_copies(1):
                cp.start()
    xnm[0:8] = jnp.broadcast_to(_fold(n2max, jnp.maximum), (8, DH))

    def qproj(j, t, scale=QSCALE):
        r2 = pl.multiple_of(t * (TQ // 2), TQ // 2)
        xb = _unpack(xn_p[pl.ds(r2, TQ // 2), :])
        q2 = jnp.dot(xb, _unpack(wq_v[j]), preferred_element_type=F32)
        q2 = (q2 * scale).astype(BF)
        return jnp.concatenate([_pack(q2[:, 0:DH]), _pack(q2[:, DH:2 * DH])], axis=0)

    def oproj(j, t, o2p):
        upd = lax.dot_general(_unpack(woT_v[j]), _unpack(o2p), (((1,), (1,)), ((), ())),
                              preferred_element_type=F32)
        accT[t] = jnp.where(j == 0, upd, accT[t] + upd)

    def attention(j, qp, fast):
        q = _unpack(qp)
        m = l = acc = None
        for c in range(S // CH):
            kc = _unpack(k_v[j, c * CH // 2:(c + 1) * CH // 2, :])
            s = lax.dot_general(q, kc, (((1,), (1,)), ((), ())),
                                preferred_element_type=F32)
            if fast:
                p = jnp.exp2(s)
            else:
                mc = jnp.broadcast_to(
                    jnp.max(_fold(s, jnp.maximum), axis=1, keepdims=True), (2 * TQ, 128))
                m_new = mc if m is None else jnp.maximum(m, mc)
                p = jnp.exp2(s - jnp.tile(m_new, (1, CH // 128)))
            lc = _fold(p, jnp.add)
            pv = jnp.dot(p.astype(BF), _unpack(v_v[j, c * CH // 2:(c + 1) * CH // 2, :]),
                         preferred_element_type=F32)
            if l is None:
                l, acc = lc, pv
            elif fast:
                l, acc = l + lc, acc + pv
            else:
                alpha = jnp.exp2(m - m_new)
                l, acc = l * alpha + lc, acc * alpha + pv
            if not fast:
                m = m_new
        ls = jnp.sum(l, axis=1, keepdims=True)
        o = (acc * _recip(ls)).astype(BF)
        return jnp.concatenate([_pack(o[0:TQ]), _pack(o[TQ:2 * TQ])], axis=1)

    def _absmax_packed(w):
        w = w & jnp.uint32(0x7FFF7FFF)
        hi = lax.bitcast_convert_type(w, F32)
        lo = lax.bitcast_convert_type(w << 16, F32)
        m = jnp.maximum(hi, lo)
        return _fold8(m, jnp.maximum)

    def _fold8(m, op):
        r = m[0:8]
        for i in range(1, m.shape[0] // 8):
            r = op(r, m[i * 8:(i + 1) * 8])
        return r

    def stats_fold(j, st, k0, nk, w0, nw):
        km, vm, ws = st
        km = jnp.maximum(km, _absmax_packed(k_v[j, pl.ds(k0, nk), :]))
        vm = jnp.maximum(vm, _absmax_packed(v_v[j, pl.ds(k0, nk), :]))
        if nw:
            wf = _unpack(wq_v[j, pl.ds(w0, nw), :]).astype(F32)
            ws = ws + _fold8(wf * wf, jnp.add)
        return km, vm, ws

    def stats_flag(st):
        km, vm, ws = st
        wn2 = jnp.sum(ws, axis=0, keepdims=True)
        wn = jnp.sqrt(jnp.maximum(wn2[:, 0:DH], wn2[:, DH:2 * DH]))
        kmx = jnp.max(km, axis=0, keepdims=True)
        xn = jnp.sqrt(jnp.max(xnm[0:1, :], axis=1, keepdims=True))
        bound = jnp.sum(wn * kmx, axis=1, keepdims=True) * xn * (1.05 * QSCALE)
        vmx = jnp.max(jnp.max(vm, axis=0, keepdims=True), axis=1, keepdims=True)
        ok = jnp.logical_and(bound <= SCORE_BOUND,
                             jnp.logical_and(vmx <= V_HI, vmx >= V_LO))
        return jnp.max(jnp.where(ok, 1.0, 0.0)).astype(jnp.int32)

    def stats_zero():
        return (jnp.zeros((8, DH), F32), jnp.zeros((8, DH), F32), jnp.zeros((8, 2 * DH), F32))

    def head_stats(j):
        return stats_flag(stats_fold(j, stats_zero(), 0, S // 2, 0, DP // 2))

    def moe_route():
        wr = jnp.broadcast_to(wr_ref[...], (16, D))
        xnT_all = jnp.concatenate([_unpack(xnT_p[c]) for c in range(XC)], axis=1)
        r = jnp.dot(wr, xnT_all, preferred_element_type=F32)
        r = _rb(r[0:8, :])
        col = lax.broadcasted_iota(jnp.int32, (8, S), 1)
        r = jnp.where(r == r, jnp.clip(r, -3e38, 3e38), -3e38)
        bits = lax.bitcast_convert_type(r, jnp.int32) & jnp.int32(-65536)
        bits = jnp.where(jnp.abs(r) < 2.0 ** -126, jnp.int32(0x00800000), bits)
        low = jnp.where(bits < 0, col, (S - 1) - col)
        key = lax.bitcast_convert_type(bits | low, F32)
        rowg = lax.broadcasted_iota(jnp.int32, (16, 128), 0)
        rsel = jnp.zeros((16, 128), F32)
        for c in range(C):
            mx = jnp.max(key, axis=1, keepdims=True)
            key = jnp.where(key == mx, -jnp.inf, key)
            mb = lax.bitcast_convert_type(mx, jnp.int32)
            lowb = mb & (S - 1)
            idx_v = jnp.where(mb < 0, lowb, (S - 1) - lowb)
            idx = jnp.max(idx_v)
            val = lax.bitcast_convert_type(mb & jnp.int32(-65536), F32)[0:1, :]
            rsel = jnp.where(rowg == c, val, rsel)
            sel_s[c] = idx
            w = xn_p[pl.ds(lax.shift_right_logical(idx, 1), 1), :]
            w = jnp.where((idx & 1) == 0, w << 16, w & jnp.uint32(0xFFFF0000))
            xs_v[c:c + 1, :] = lax.bitcast_convert_type(w, F32)
        rs_v[0:16] = rsel

    def moe_ffn():
        for cp in moe_copies():
            cp.wait()
        xs = xs_v[0:16, 0:D].astype(BF)
        g = _rb(jnp.dot(xs, _unpack(wg_v[...]), preferred_element_type=F32))
        uu = _rb(jnp.dot(xs, _unpack(wu_v[...]), preferred_element_type=F32))
        h = (_rb(g * _rb(_sigmoid(g))) * uu).astype(BF)
        y = _rb(lax.dot_general(h, _unpack(wdT_v[...]), (((1,), (1,)), ((), ())),
                                preferred_element_type=F32))
        y = _rb(y * _rb(_sigmoid(rs_v[0:16, 0:1])))
        ypad = jnp.concatenate([y, jnp.zeros((112, D), F32)], axis=0)
        ypad = jnp.concatenate([ypad, jnp.zeros((128, DP - D), F32)], axis=1)
        yT_p[...] = _pack(ypad.T[0:D, :].astype(BF))

    def final(c):
        row = lax.broadcasted_iota(jnp.int32, (16, XR), 0)
        tok = lax.broadcasted_iota(jnp.int32, (16, XR), 1) + c * XR
        onehot = jnp.zeros((16, XR), F32)
        for k in range(C):
            onehot = jnp.where(jnp.logical_and(row == k, tok == sel_s[k]), 1.0, onehot)
        onehot = jnp.concatenate([onehot, jnp.zeros((112, XR), F32)], axis=0).astype(BF)
        upd = jnp.dot(_unpack(yT_p[...]), onehot, preferred_element_type=F32)
        z = _unpack(xnT_p[c]).astype(F32) + upd
        s_att = jnp.concatenate([accT[2 * c], accT[2 * c + 1]], axis=1)
        outT_v[c] = (xT_v[c].astype(F32) + s_att * (z * _sigmoid(z))).astype(BF)

    tr_chunk(XC - 1)
    moe_route()
    for cp in head_copies(0):
        cp.wait()
    safe0 = head_stats(0)

    def block(j, i, tasks, fast):
        if not fast:
            for a in tasks:
                oproj(j, i * UN + a, attention(j, qproj(j, i * UN + a), False))
            return None
        first = i == 0
        js = jnp.where(jnp.logical_and(j == 0, first), 0, jnp.minimum(j + 1, HKV - 1))
        st = tuple(jnp.where(first, z, old)
                   for z, old in zip(stats_zero(), (kst[0:8], vst[0:8], wst[0:8])))
        nk = S // 2 // TPH
        nw = DP // 2 // IPH // WSL
        qs = []
        for a in tasks:
            k0 = pl.multiple_of((i * UN + a) * nk, nk)
            w0 = pl.multiple_of((i * WSL + a) * nw, 8)
            st = stats_fold(js, st, k0, nk, w0, nw if a < WSL else 0)
            zero = jnp.minimum(jnp.minimum(st[0][0:1, :], st[1][0:1, :]), 0.0)
            scale = QSCALE + jnp.minimum(jnp.concatenate([zero, zero], axis=1), st[2][0:1, :])
            qs.append(qproj(j, i * UN + a, scale))
        kst[0:8], vst[0:8], wst[0:8] = st
        outs = [attention(j, q, True) for q in qs]
        for a, op in zip(tasks, outs):
            oproj(j, i * UN + a, op)
        return stats_flag(st)

    def finish(c0, n):
        def fin(k, carry):
            for c in (c0 + 2 * k, c0 + 2 * k + 1):
                final(c)
                out_copy(c).start()
            return carry
        lax.fori_loop(0, n // 2, fin, 0)

    def head_body(j, safe):
        @pl.when(jnp.logical_and(j > 0, j + 1 < HKV))
        def _():
            for cp in head_copies(j + 1):
                cp.wait()

        @pl.when(j + 2 < HKV)
        def _():
            for cp in head_copies(j + 2):
                cp.start()

        @pl.when(j == 1)
        def _():
            for cp in moe_copies():
                cp.start()

        @pl.when(j == HKV - 1)
        def _():
            moe_ffn()

        js = jnp.minimum(j + 1, HKV - 1)

        def fast_head():
            def it(i, c):
                flag = block(j, i, range(UN), True)

                @pl.when(jnp.logical_and(j == 0, i == 0))
                def _():
                    for cp in head_copies(1):
                        cp.wait()
                    kst[0:8], vst[0:8], wst[0:8] = stats_fold(
                        1, stats_zero(), 0, S // 2 // IPH, 0, DP // 2 // IPH)

                @pl.when(j == HKV - 1)
                def _():
                    finish(i * (UN // 2), UN // 2)
                return flag
            return lax.fori_loop(0, IPH, it, 0)

        def slow_head():
            @pl.when(j == 0)
            def _():
                for cp in head_copies(1):
                    cp.wait()

            def it(t, c):
                block(j, t // UN, [t % UN], False)
                return c
            lax.fori_loop(0, TPH, it, 0)

            @pl.when(j == HKV - 1)
            def _():
                finish(0, XC)
            return head_stats(js)

        return lax.cond(safe > 0, fast_head, slow_head)

    lax.fori_loop(0, HKV, head_body, safe0)
    for c in range(XC):
        out_copy(c).wait()


@jax.jit
def pallas_recurrent_scan__gqa_block_cached__moe_arch_mod__prompt_kernel(
    A_x: jax.Array,
    A_k_cache: jax.Array,
    A_v_cache: jax.Array,
    A_wq: jax.Array,
    A_wo: jax.Array,
    B_x: jax.Array,
    B_w_r: jax.Array,
    B_w_gate: jax.Array,
    B_w_up: jax.Array,
    B_w_down: jax.Array,
):
    del B_x
    xT = A_x.reshape(S, D).T
    woT = A_wo.T
    wdT = B_w_down.T
    k = A_k_cache.reshape(HKV, S, DH)
    v = A_v_cache.reshape(HKV, S, DH)
    wr = B_w_r.reshape(1, D)

    hbm = pl.BlockSpec(memory_space=pltpu.HBM)
    vmem = pl.BlockSpec(memory_space=pltpu.VMEM)
    outT = pl.pallas_call(
        _kernel,
        out_shape=jax.ShapeDtypeStruct((D, S), BF),
        in_specs=[hbm, hbm, hbm, hbm, hbm, vmem, hbm, hbm, hbm],
        out_specs=hbm,
        scratch_shapes=[
            pltpu.VMEM((XC, D, XR), BF),
            pltpu.VMEM((XC, D // 2, XR), U32),
            pltpu.VMEM((S // 2, DP), U32),
            pltpu.VMEM((S // TQ, D, TQ), F32),
            pltpu.VMEM((HKV, S // 2, DH), U32),
            pltpu.VMEM((HKV, S // 2, DH), U32),
            pltpu.VMEM((HKV, DP // 2, 2 * DH), U32),
            pltpu.VMEM((HKV, D // 2, 2 * DH), U32),
            pltpu.VMEM((D // 2, F), U32),
            pltpu.VMEM((D // 2, F), U32),
            pltpu.VMEM((D // 2, F), U32),
            pltpu.VMEM((32, DP), F32),
            pltpu.VMEM((XC, D, XR), BF),
            pltpu.VMEM((32, DH), F32),
            pltpu.VMEM((32, DH), F32),
            pltpu.VMEM((16, 2 * DH), F32),
            pltpu.VMEM((32, DH), F32),
            pltpu.VMEM((32, 128), F32),
            pltpu.VMEM((D // 2, 128), U32),
            pltpu.SMEM((C,), jnp.int32),
            pltpu.SemaphoreType.DMA((XC,)),
            pltpu.SemaphoreType.DMA((4 * HKV,)),
            pltpu.SemaphoreType.DMA((3,)),
            pltpu.SemaphoreType.DMA((XC,)),
        ],
        compiler_params=pltpu.CompilerParams(vmem_limit_bytes=100 * 1024 * 1024,
                                             disable_bounds_checks=True,
                                             disable_semaphore_checks=True),
        name="fused_attn_moe",
    )(xT, k, v, A_wq, woT, wr, B_w_gate, B_w_up, wdT)
    return outT.T.reshape(1, S, D)
```

```python
import functools
import math

import jax
import jax.numpy as jnp
from jax import lax
import jax.experimental.pallas as pl
import jax.experimental.pallas.tpu as pltpu

S = 2048
D = 576
DP = 640
HQ = 32
HKV = 16
DH = 128
F = 4608
C = 8
EPS_BF16 = 1.0013580322265625e-05

TQ = 128
UN = 8
CH = 512
TPH = S // TQ
IPH = TPH // UN
WSL = 5 if UN == 8 else 2
HEAD0_AT = 3
HEAD1_AT = 7
XC = 8
XR = S // XC

BF = jnp.bfloat16
F32 = jnp.float32
U32 = jnp.uint32
QSCALE = (DH ** -0.5) * math.log2(math.e)

SCORE_BOUND = 40.0
V_HI = 2.0 ** 60
V_LO = 2.0 ** -60


def _rb(v):
    return v.astype(BF).astype(F32)


def _pack(v_bf16):
    return pltpu.bitcast(v_bf16, U32)


def _unpack(v_u32):
    return pltpu.bitcast(v_u32, BF)


def _fold(x, op):
    r = x[:, 0:128]
    for j in range(1, x.shape[1] // 128):
        r = op(r, x[:, j * 128:(j + 1) * 128])
    return r


def _sigmoid(v):
    return 0.5 * jnp.tanh(0.5 * v) + 0.5


def _recip(v):
    r = pl.reciprocal(v, approx=True)
    return r * (2.0 - v * r)


def _kernel(xT_hbm, k_hbm, v_hbm, wq_hbm, woT_hbm, wr_ref, wg_hbm, wu_hbm, wdT_hbm,
            outT_hbm,
            xT_v, xnT_p, xn_p, accT, k_v, v_v, wq_v, woT_v, wg_v, wu_v, wdT_v,
            xs_v, outT_v, kst, vst, wst, xnm, rs_v, yT_p, sel_s,
            sem_x, sem_h, sem_m, sem_o):

    def x_copy(c):
        return pltpu.make_async_copy(
            xT_hbm.at[:, pl.ds(c * XR, XR)], xT_v.at[c], sem_x.at[c])

    k_p, v_p = k_hbm.bitcast(U32), v_hbm.bitcast(U32)
    wq_p, woT_p = wq_hbm.bitcast(U32), woT_hbm.bitcast(U32)

    def head_copies(j):
        col = pl.multiple_of(j * (2 * DH), 2 * DH)
        pairs = [
            (wq_p.at[:, pl.ds(col, 2 * DH)], wq_v.at[j, pl.ds(0, D // 2), :]),
            (k_p.at[j], k_v.at[j]),
            (v_p.at[j], v_v.at[j]),
            (woT_p.at[:, pl.ds(col, 2 * DH)], woT_v.at[j]),
        ]
        return [pltpu.make_async_copy(*pairs[w], sem_h.at[4 * j + w]) for w in range(4)]

    def moe_copies():
        return [pltpu.make_async_copy(wg_hbm.bitcast(U32), wg_v, sem_m.at[0]),
                pltpu.make_async_copy(wu_hbm.bitcast(U32), wu_v, sem_m.at[1]),
                pltpu.make_async_copy(wdT_hbm.bitcast(U32), wdT_v, sem_m.at[2])]

    def out_copy(c):
        cols = pl.ds(pl.multiple_of(c * XR, XR), XR)
        return pltpu.make_async_copy(outT_v.at[c], outT_hbm.at[:, cols], sem_o.at[c])

    for c in range(XC):
        x_copy(c).start()

    wq_v[:, D // 2:DP // 2, :] = jnp.zeros((HKV, (DP - D) // 2, 2 * DH), U32)
    xs_v[...] = jnp.zeros(xs_v.shape, F32)

    def ln_chunk(c):
        xf = xT_v[c].astype(F32)
        mean = jnp.sum(xf, axis=0, keepdims=True) / D
        cen = xf - mean
        var = jnp.sum(cen * cen, axis=0, keepdims=True) / D
        mean_b = _rb(mean)
        dlt = _rb(xf - mean_b)
        sd = _rb(jnp.sqrt(_rb(_rb(var) + EPS_BF16)))
        xnT_p[c] = _pack((dlt / sd).astype(BF))
        return D * (var + (mean - mean_b) * (mean - mean_b)) / (sd * sd)

    def tr_chunk(c):
        xpad = jnp.concatenate([_unpack(xnT_p[c]), jnp.zeros((DP - D, XR), BF)], axis=0)
        xn_p[c * XR // 2:(c + 1) * XR // 2, :] = _pack(xpad.T)

    n2max = None
    for c in range(XC):
        x_copy(c).wait()
        n2 = ln_chunk(c)
        n2max = n2 if n2max is None else jnp.maximum(n2max, n2)
        if c > 0:
            tr_chunk(c - 1)
        if c == HEAD0_AT:
            for cp in head_copies(0):
                cp.start()
        if c == HEAD1_AT:
            for cp in head_copies(1):
                cp.start()
    xnm[0:8] = jnp.broadcast_to(_fold(n2max, jnp.maximum), (8, DH))

    def qproj(j, t, scale=QSCALE):
        r2 = pl.multiple_of(t * (TQ // 2), TQ // 2)
        xb = _unpack(xn_p[pl.ds(r2, TQ // 2), :])
        q2 = jnp.dot(xb, _unpack(wq_v[j]), preferred_element_type=F32)
        q2 = (q2 * scale).astype(BF)
        return jnp.concatenate([_pack(q2[:, 0:DH]), _pack(q2[:, DH:2 * DH])], axis=0)

    def oproj(j, t, o2p):
        upd = lax.dot_general(_unpack(woT_v[j]), _unpack(o2p), (((1,), (1,)), ((), ())),
                              preferred_element_type=F32)
        accT[t] = jnp.where(j == 0, upd, accT[t] + upd)

    def attention(j, qp, fast):
        q = _unpack(qp)
        m = l = acc = None
        for c in range(S // CH):
            kc = _unpack(k_v[j, c * CH // 2:(c + 1) * CH // 2, :])
            s = lax.dot_general(q, kc, (((1,), (1,)), ((), ())),
                                preferred_element_type=F32)
            if fast:
                p = jnp.exp2(s)
            else:
                mc = jnp.broadcast_to(
                    jnp.max(_fold(s, jnp.maximum), axis=1, keepdims=True), (2 * TQ, 128))
                m_new = mc if m is None else jnp.maximum(m, mc)
                p = jnp.exp2(s - jnp.tile(m_new, (1, CH // 128)))
            lc = _fold(p, jnp.add)
            pv = jnp.dot(p.astype(BF), _unpack(v_v[j, c * CH // 2:(c + 1) * CH // 2, :]),
                         preferred_element_type=F32)
            if l is None:
                l, acc = lc, pv
            elif fast:
                l, acc = l + lc, acc + pv
            else:
                alpha = jnp.exp2(m - m_new)
                l, acc = l * alpha + lc, acc * alpha + pv
            if not fast:
                m = m_new
        ls = jnp.sum(l, axis=1, keepdims=True)
        o = (acc * _recip(ls)).astype(BF)
        return jnp.concatenate([_pack(o[0:TQ]), _pack(o[TQ:2 * TQ])], axis=1)

    def _absmax_packed(w):
        w = w & jnp.uint32(0x7FFF7FFF)
        hi = lax.bitcast_convert_type(w, F32)
        lo = lax.bitcast_convert_type(w << 16, F32)
        m = jnp.maximum(hi, lo)
        return _fold8(m, jnp.maximum)

    def _fold8(m, op):
        r = m[0:8]
        for i in range(1, m.shape[0] // 8):
            r = op(r, m[i * 8:(i + 1) * 8])
        return r

    def stats_fold(j, st, k0, nk, w0, nw):
        km, vm, ws = st
        km = jnp.maximum(km, _absmax_packed(k_v[j, pl.ds(k0, nk), :]))
        vm = jnp.maximum(vm, _absmax_packed(v_v[j, pl.ds(k0, nk), :]))
        if nw:
            wf = _unpack(wq_v[j, pl.ds(w0, nw), :]).astype(F32)
            ws = ws + _fold8(wf * wf, jnp.add)
        return km, vm, ws

    def stats_flag(st):
        km, vm, ws = st
        wn2 = jnp.sum(ws, axis=0, keepdims=True)
        wn = jnp.sqrt(jnp.maximum(wn2[:, 0:DH], wn2[:, DH:2 * DH]))
        kmx = jnp.max(km, axis=0, keepdims=True)
        xn = jnp.sqrt(jnp.max(xnm[0:1, :], axis=1, keepdims=True))
        bound = jnp.sum(wn * kmx, axis=1, keepdims=True) * xn * (1.05 * QSCALE)
        vmx = jnp.max(jnp.max(vm, axis=0, keepdims=True), axis=1, keepdims=True)
        ok = jnp.logical_and(bound <= SCORE_BOUND,
                             jnp.logical_and(vmx <= V_HI, vmx >= V_LO))
        return jnp.max(jnp.where(ok, 1.0, 0.0)).astype(jnp.int32)

    def stats_zero():
        return (jnp.zeros((8, DH), F32), jnp.zeros((8, DH), F32), jnp.zeros((8, 2 * DH), F32))

    def head_stats(j):
        return stats_flag(stats_fold(j, stats_zero(), 0, S // 2, 0, DP // 2))

    def moe_route():
        wr = jnp.broadcast_to(wr_ref[...], (16, D))
        xnT_all = jnp.concatenate([_unpack(xnT_p[c]) for c in range(XC)], axis=1)
        r = jnp.dot(wr, xnT_all, preferred_element_type=F32)
        r = _rb(r[0:8, :])
        col = lax.broadcasted_iota(jnp.int32, (8, S), 1)
        r = jnp.where(r == r, jnp.clip(r, -3e38, 3e38), -3e38)
        bits = lax.bitcast_convert_type(r, jnp.int32) & jnp.int32(-65536)
        bits = jnp.where(jnp.abs(r) < 2.0 ** -126, jnp.int32(0x00800000), bits)
        low = jnp.where(bits < 0, col, (S - 1) - col)
        key = lax.bitcast_convert_type(bits | low, F32)
        rowg = lax.broadcasted_iota(jnp.int32, (16, 128), 0)
        rsel = jnp.zeros((16, 128), F32)
        for c in range(C):
            mx = jnp.max(key, axis=1, keepdims=True)
            key = jnp.where(key == mx, -jnp.inf, key)
            mb = lax.bitcast_convert_type(mx, jnp.int32)
            lowb = mb & (S - 1)
            idx_v = jnp.where(mb < 0, lowb, (S - 1) - lowb)
            idx = jnp.max(idx_v)
            val = lax.bitcast_convert_type(mb & jnp.int32(-65536), F32)[0:1, :]
            rsel = jnp.where(rowg == c, val, rsel)
            sel_s[c] = idx
            w = xn_p[pl.ds(lax.shift_right_logical(idx, 1), 1), :]
            w = jnp.where((idx & 1) == 0, w << 16, w & jnp.uint32(0xFFFF0000))
            xs_v[c:c + 1, :] = lax.bitcast_convert_type(w, F32)
        rs_v[0:16] = rsel

    def moe_ffn():
        for cp in moe_copies():
            cp.wait()
        xs = xs_v[0:16, 0:D].astype(BF)
        g = _rb(jnp.dot(xs, _unpack(wg_v[...]), preferred_element_type=F32))
        uu = _rb(jnp.dot(xs, _unpack(wu_v[...]), preferred_element_type=F32))
        h = (_rb(g * _rb(_sigmoid(g))) * uu).astype(BF)
        y = _rb(lax.dot_general(h, _unpack(wdT_v[...]), (((1,), (1,)), ((), ())),
                                preferred_element_type=F32))
        y = _rb(y * _rb(_sigmoid(rs_v[0:16, 0:1])))
        ypad = jnp.concatenate([y, jnp.zeros((112, D), F32)], axis=0)
        ypad = jnp.concatenate([ypad, jnp.zeros((128, DP - D), F32)], axis=1)
        yT_p[...] = _pack(ypad.T[0:D, :].astype(BF))

    def final(c):
        row = lax.broadcasted_iota(jnp.int32, (16, XR), 0)
        tok = lax.broadcasted_iota(jnp.int32, (16, XR), 1) + c * XR
        onehot = jnp.zeros((16, XR), F32)
        for k in range(C):
            onehot = jnp.where(jnp.logical_and(row == k, tok == sel_s[k]), 1.0, onehot)
        onehot = jnp.concatenate([onehot, jnp.zeros((112, XR), F32)], axis=0).astype(BF)
        upd = jnp.dot(_unpack(yT_p[...]), onehot, preferred_element_type=F32)
        z = _unpack(xnT_p[c]).astype(F32) + upd
        s_att = jnp.concatenate([accT[2 * c], accT[2 * c + 1]], axis=1)
        outT_v[c] = (xT_v[c].astype(F32) + s_att * (z * _sigmoid(z))).astype(BF)

    tr_chunk(XC - 1)
    moe_route()
    for cp in head_copies(0):
        cp.wait()
    safe0 = head_stats(0)

    def block(j, i, tasks, fast):
        if not fast:
            for a in tasks:
                oproj(j, i * UN + a, attention(j, qproj(j, i * UN + a), False))
            return None
        first = i == 0
        js = jnp.where(jnp.logical_and(j == 0, first), 0, jnp.minimum(j + 1, HKV - 1))
        st = tuple(jnp.where(first, z, old)
                   for z, old in zip(stats_zero(), (kst[0:8], vst[0:8], wst[0:8])))
        nk = S // 2 // TPH
        nw = DP // 2 // IPH // WSL
        qs = []
        for a in tasks:
            k0 = pl.multiple_of((i * UN + a) * nk, nk)
            w0 = pl.multiple_of((i * WSL + a) * nw, 8)
            st = stats_fold(js, st, k0, nk, w0, nw if a < WSL else 0)
            zero = jnp.minimum(jnp.minimum(st[0][0:1, :], st[1][0:1, :]), 0.0)
            scale = QSCALE + jnp.minimum(jnp.concatenate([zero, zero], axis=1), st[2][0:1, :])
            qs.append(qproj(j, i * UN + a, scale))
        kst[0:8], vst[0:8], wst[0:8] = st
        outs = [attention(j, q, True) for q in qs]
        for a, op in zip(tasks, outs):
            oproj(j, i * UN + a, op)
        return stats_flag(st)

    def finish(c0, n):
        def fin(k, carry):
            for c in (c0 + 2 * k, c0 + 2 * k + 1):
                final(c)
                out_copy(c).start()
            return carry
        lax.fori_loop(0, n // 2, fin, 0)

    def head_body(j, safe):
        @pl.when(jnp.logical_and(j > 0, j + 1 < HKV))
        def _():
            for cp in head_copies(j + 1):
                cp.wait()

        @pl.when(j + 2 < HKV)
        def _():
            for cp in head_copies(j + 2):
                cp.start()

        @pl.when(j == HKV - 1)
        def _():
            moe_ffn()

        def fast_head():
            def it(i, c):
                flag = block(j, i, range(UN), True)

                @pl.when(jnp.logical_and(j == 0, i == 0))
                def _():
                    for cp in head_copies(1):
                        cp.wait()
                    for cp in moe_copies():
                        cp.start()
                    kst[0:8], vst[0:8], wst[0:8] = stats_fold(
                        1, stats_zero(), 0, S // 2 // IPH, 0, DP // 2 // IPH)

                @pl.when(j == HKV - 1)
                def _():
                    finish(i * (UN // 2), UN // 2)
                return flag
            return lax.fori_loop(0, IPH, it, 0)

        def slow_head():
            @pl.when(j == 0)
            def _():
                for cp in head_copies(1):
                    cp.wait()
                for cp in moe_copies():
                    cp.start()

            def it(t, c):
                block(j, t // UN, [t % UN], False)
                return c
            lax.fori_loop(0, TPH, it, 0)

            @pl.when(j == HKV - 1)
            def _():
                finish(0, XC)
            return head_stats(jnp.minimum(j + 1, HKV - 1))

        return lax.cond(safe > 0, fast_head, slow_head)

    lax.fori_loop(0, HKV, head_body, safe0)
    for c in range(XC):
        out_copy(c).wait()


@jax.jit
def pallas_recurrent_scan__gqa_block_cached__moe_arch_mod__prompt_kernel(
    A_x: jax.Array,
    A_k_cache: jax.Array,
    A_v_cache: jax.Array,
    A_wq: jax.Array,
    A_wo: jax.Array,
    B_x: jax.Array,
    B_w_r: jax.Array,
    B_w_gate: jax.Array,
    B_w_up: jax.Array,
    B_w_down: jax.Array,
):
    del B_x
    xT = A_x.reshape(S, D).T
    woT = A_wo.T
    wdT = B_w_down.T
    k = A_k_cache.reshape(HKV, S, DH)
    v = A_v_cache.reshape(HKV, S, DH)
    wr = B_w_r.reshape(1, D)

    hbm = pl.BlockSpec(memory_space=pltpu.HBM)
    vmem = pl.BlockSpec(memory_space=pltpu.VMEM)
    outT = pl.pallas_call(
        _kernel,
        out_shape=jax.ShapeDtypeStruct((D, S), BF),
        in_specs=[hbm, hbm, hbm, hbm, hbm, vmem, hbm, hbm, hbm],
        out_specs=hbm,
        scratch_shapes=[
            pltpu.VMEM((XC, D, XR), BF),
            pltpu.VMEM((XC, D // 2, XR), U32),
            pltpu.VMEM((S // 2, DP), U32),
            pltpu.VMEM((S // TQ, D, TQ), F32),
            pltpu.VMEM((HKV, S // 2, DH), U32),
            pltpu.VMEM((HKV, S // 2, DH), U32),
            pltpu.VMEM((HKV, DP // 2, 2 * DH), U32),
            pltpu.VMEM((HKV, D // 2, 2 * DH), U32),
            pltpu.VMEM((D // 2, F), U32),
            pltpu.VMEM((D // 2, F), U32),
            pltpu.VMEM((D // 2, F), U32),
            pltpu.VMEM((32, DP), F32),
            pltpu.VMEM((XC, D, XR), BF),
            pltpu.VMEM((32, DH), F32),
            pltpu.VMEM((32, DH), F32),
            pltpu.VMEM((16, 2 * DH), F32),
            pltpu.VMEM((32, DH), F32),
            pltpu.VMEM((32, 128), F32),
            pltpu.VMEM((D // 2, 128), U32),
            pltpu.SMEM((C,), jnp.int32),
            pltpu.SemaphoreType.DMA((XC,)),
            pltpu.SemaphoreType.DMA((4 * HKV,)),
            pltpu.SemaphoreType.DMA((3,)),
            pltpu.SemaphoreType.DMA((XC,)),
        ],
        compiler_params=pltpu.CompilerParams(vmem_limit_bytes=100 * 1024 * 1024,
                                             disable_bounds_checks=True,
                                             disable_semaphore_checks=True),
        name="fused_attn_moe",
    )(xT, k, v, A_wq, woT, wr, B_w_gate, B_w_up, wdT)
    return outT.T.reshape(1, S, D)
```

```python
import functools
import math

import jax
import jax.numpy as jnp
from jax import lax
import jax.experimental.pallas as pl
import jax.experimental.pallas.tpu as pltpu

S = 2048
D = 576
DP = 640
HQ = 32
HKV = 16
DH = 128
F = 4608
C = 8
EPS_BF16 = 1.0013580322265625e-05

TQ = 128
UN = 8
CH = 512
TPH = S // TQ
IPH = TPH // UN
WSL = 5 if UN == 8 else 2
HEAD0_AT = 3
HEAD1_AT = 7
XC = 8
XR = S // XC

BF = jnp.bfloat16
F32 = jnp.float32
U32 = jnp.uint32
QSCALE = (DH ** -0.5) * math.log2(math.e)

SCORE_BOUND = 40.0
V_HI = 2.0 ** 60
V_LO = 2.0 ** -60


def _rb(v):
    return v.astype(BF).astype(F32)


def _pack(v_bf16):
    return pltpu.bitcast(v_bf16, U32)


def _unpack(v_u32):
    return pltpu.bitcast(v_u32, BF)


def _fold(x, op):
    r = x[:, 0:128]
    for j in range(1, x.shape[1] // 128):
        r = op(r, x[:, j * 128:(j + 1) * 128])
    return r


def _sigmoid(v):
    return 0.5 * jnp.tanh(0.5 * v) + 0.5


def _recip(v):
    r = pl.reciprocal(v, approx=True)
    return r * (2.0 - v * r)


def _kernel(xT_hbm, k_hbm, v_hbm, wq_hbm, woT_hbm, wr_ref, wg_hbm, wu_hbm, wdT_hbm,
            outT_hbm,
            xT_v, xnT_p, xn_p, accT, k_v, v_v, wq_v, woT_v, wg_v, wu_v, wdT_v,
            xs_v, outT_v, kst, vst, wst, xnm, rs_v, yT_p, sel_s,
            sem_x, sem_h, sem_m, sem_o):

    def x_copy(c):
        return pltpu.make_async_copy(
            xT_hbm.at[:, pl.ds(c * XR, XR)], xT_v.at[c], sem_x.at[c])

    def head_copies(j):
        col = pl.multiple_of(j * (2 * DH), 2 * DH)
        pairs = [
            (wq_hbm.at[:, pl.ds(col, 2 * DH)], wq_v.at[j, pl.ds(0, D), :]),
            (k_hbm.at[j], k_v.at[j]),
            (v_hbm.at[j], v_v.at[j]),
            (woT_hbm.at[:, pl.ds(col, 2 * DH)], woT_v.at[j]),
        ]
        return [pltpu.make_async_copy(*pairs[w], sem_h.at[4 * j + w]) for w in range(4)]

    def moe_copies():
        return [pltpu.make_async_copy(wg_hbm, wg_v, sem_m.at[0]),
                pltpu.make_async_copy(wu_hbm, wu_v, sem_m.at[1]),
                pltpu.make_async_copy(wdT_hbm, wdT_v, sem_m.at[2])]

    def out_copy(c):
        cols = pl.ds(pl.multiple_of(c * XR, XR), XR)
        return pltpu.make_async_copy(outT_v.at[c], outT_hbm.at[:, cols], sem_o.at[c])

    for c in range(XC):
        x_copy(c).start()

    wq_v[:, D:DP, :] = jnp.zeros((HKV, DP - D, 2 * DH), BF)
    xs_v[...] = jnp.zeros(xs_v.shape, F32)

    def ln_chunk(c):
        xf = xT_v[c].astype(F32)
        mean = jnp.sum(xf, axis=0, keepdims=True) / D
        cen = xf - mean
        var = jnp.sum(cen * cen, axis=0, keepdims=True) / D
        mean_b = _rb(mean)
        dlt = _rb(xf - mean_b)
        sd = _rb(jnp.sqrt(_rb(_rb(var) + EPS_BF16)))
        xnT_p[c] = _pack((dlt / sd).astype(BF))
        return D * (var + (mean - mean_b) * (mean - mean_b)) / (sd * sd)

    def tr_chunk(c):
        xpad = jnp.concatenate([_unpack(xnT_p[c]), jnp.zeros((DP - D, XR), BF)], axis=0)
        xn_p[c * XR // 2:(c + 1) * XR // 2, :] = _pack(xpad.T)

    n2max = None
    for c in range(XC):
        x_copy(c).wait()
        n2 = ln_chunk(c)
        n2max = n2 if n2max is None else jnp.maximum(n2max, n2)
        if c > 0:
            tr_chunk(c - 1)
        if c == HEAD0_AT:
            for cp in head_copies(0):
                cp.start()
        if c == HEAD1_AT:
            for cp in head_copies(1):
                cp.start()
    xnm[0:8] = jnp.broadcast_to(_fold(n2max, jnp.maximum), (8, DH))

    def qproj(j, t, scale=QSCALE):
        r2 = pl.multiple_of(t * (TQ // 2), TQ // 2)
        xb = _unpack(xn_p[pl.ds(r2, TQ // 2), :])
        q2 = jnp.dot(xb, wq_v[j], preferred_element_type=F32)
        q2 = (q2 * scale).astype(BF)
        return jnp.concatenate([_pack(q2[:, 0:DH]), _pack(q2[:, DH:2 * DH])], axis=0)

    def oproj(j, t, o2p):
        upd = lax.dot_general(woT_v[j], _unpack(o2p), (((1,), (1,)), ((), ())),
                              preferred_element_type=F32)
        accT[t] = jnp.where(j == 0, upd, accT[t] + upd)

    def attention(j, qp, fast):
        q = _unpack(qp)
        m = l = acc = None
        for c in range(S // CH):
            kc = k_v[j, c * CH:(c + 1) * CH, :]
            s = lax.dot_general(q, kc, (((1,), (1,)), ((), ())),
                                preferred_element_type=F32)
            if fast:
                p = jnp.exp2(s)
            else:
                mc = jnp.broadcast_to(
                    jnp.max(_fold(s, jnp.maximum), axis=1, keepdims=True), (2 * TQ, 128))
                m_new = mc if m is None else jnp.maximum(m, mc)
                p = jnp.exp2(s - jnp.tile(m_new, (1, CH // 128)))
            lc = _fold(p, jnp.add)
            pv = jnp.dot(p.astype(BF), v_v[j, c * CH:(c + 1) * CH, :],
                         preferred_element_type=F32)
            if l is None:
                l, acc = lc, pv
            elif fast:
                l, acc = l + lc, acc + pv
            else:
                alpha = jnp.exp2(m - m_new)
                l, acc = l * alpha + lc, acc * alpha + pv
            if not fast:
                m = m_new
        ls = jnp.sum(l, axis=1, keepdims=True)
        o = (acc * _recip(ls)).astype(BF)
        return jnp.concatenate([_pack(o[0:TQ]), _pack(o[TQ:2 * TQ])], axis=1)

    def _absmax_packed(w):
        w = w & jnp.uint32(0x7FFF7FFF)
        hi = lax.bitcast_convert_type(w, F32)
        lo = lax.bitcast_convert_type(w << 16, F32)
        m = jnp.maximum(hi, lo)
        return _fold8(m, jnp.maximum)

    def _fold8(m, op):
        r = m[0:8]
        for i in range(1, m.shape[0] // 8):
            r = op(r, m[i * 8:(i + 1) * 8])
        return r

    def stats_fold(j, st, k0, nk, w0, nw):
        km, vm, ws = st
        km = jnp.maximum(km, _absmax_packed(_pack(k_v[j, pl.ds(k0, nk), :])))
        vm = jnp.maximum(vm, _absmax_packed(_pack(v_v[j, pl.ds(k0, nk), :])))
        if nw:
            wf = wq_v[j, pl.ds(w0, nw), :].astype(F32)
            ws = ws + _fold8(wf * wf, jnp.add)
        return km, vm, ws

    def stats_flag(st):
        km, vm, ws = st
        wn2 = jnp.sum(ws, axis=0, keepdims=True)
        wn = jnp.sqrt(jnp.maximum(wn2[:, 0:DH], wn2[:, DH:2 * DH]))
        kmx = jnp.max(km, axis=0, keepdims=True)
        xn = jnp.sqrt(jnp.max(xnm[0:1, :], axis=1, keepdims=True))
        bound = jnp.sum(wn * kmx, axis=1, keepdims=True) * xn * (1.05 * QSCALE)
        vmx = jnp.max(jnp.max(vm, axis=0, keepdims=True), axis=1, keepdims=True)
        ok = jnp.logical_and(bound <= SCORE_BOUND,
                             jnp.logical_and(vmx <= V_HI, vmx >= V_LO))
        return jnp.max(jnp.where(ok, 1.0, 0.0)).astype(jnp.int32)

    def stats_zero():
        return (jnp.zeros((8, DH), F32), jnp.zeros((8, DH), F32), jnp.zeros((8, 2 * DH), F32))

    def head_stats(j):
        return stats_flag(stats_fold(j, stats_zero(), 0, S, 0, DP))

    def moe_route():
        wr = jnp.broadcast_to(wr_ref[...], (16, D))
        xnT_all = jnp.concatenate([_unpack(xnT_p[c]) for c in range(XC)], axis=1)
        r = jnp.dot(wr, xnT_all, preferred_element_type=F32)
        r = _rb(r[0:8, :])
        col = lax.broadcasted_iota(jnp.int32, (8, S), 1)
        r = jnp.where(r == r, jnp.clip(r, -3e38, 3e38), -3e38)
        bits = lax.bitcast_convert_type(r, jnp.int32) & jnp.int32(-65536)
        bits = jnp.where(jnp.abs(r) < 2.0 ** -126, jnp.int32(0x00800000), bits)
        low = jnp.where(bits < 0, col, (S - 1) - col)
        key = lax.bitcast_convert_type(bits | low, F32)
        rowg = lax.broadcasted_iota(jnp.int32, (16, 128), 0)
        rsel = jnp.zeros((16, 128), F32)
        for c in range(C):
            mx = jnp.max(key, axis=1, keepdims=True)
            key = jnp.where(key == mx, -jnp.inf, key)
            mb = lax.bitcast_convert_type(mx, jnp.int32)
            lowb = mb & (S - 1)
            idx_v = jnp.where(mb < 0, lowb, (S - 1) - lowb)
            idx = jnp.max(idx_v)
            val = lax.bitcast_convert_type(mb & jnp.int32(-65536), F32)[0:1, :]
            rsel = jnp.where(rowg == c, val, rsel)
            sel_s[c] = idx
            w = xn_p[pl.ds(lax.shift_right_logical(idx, 1), 1), :]
            w = jnp.where((idx & 1) == 0, w << 16, w & jnp.uint32(0xFFFF0000))
            xs_v[c:c + 1, :] = lax.bitcast_convert_type(w, F32)
        rs_v[0:16] = rsel

    def moe_ffn():
        for cp in moe_copies():
            cp.wait()
        xs = xs_v[0:16, 0:D].astype(BF)
        g = _rb(jnp.dot(xs, wg_v[...], preferred_element_type=F32))
        uu = _rb(jnp.dot(xs, wu_v[...], preferred_element_type=F32))
        h = (_rb(g * _rb(_sigmoid(g))) * uu).astype(BF)
        y = _rb(lax.dot_general(h, wdT_v[...], (((1,), (1,)), ((), ())),
                                preferred_element_type=F32))
        y = _rb(y * _rb(_sigmoid(rs_v[0:16, 0:1])))
        ypad = jnp.concatenate([y, jnp.zeros((112, D), F32)], axis=0)
        ypad = jnp.concatenate([ypad, jnp.zeros((128, DP - D), F32)], axis=1)
        yT_p[...] = _pack(ypad.T[0:D, :].astype(BF))

    def final(c):
        row = lax.broadcasted_iota(jnp.int32, (16, XR), 0)
        tok = lax.broadcasted_iota(jnp.int32, (16, XR), 1) + c * XR
        onehot = jnp.zeros((16, XR), F32)
        for k in range(C):
            onehot = jnp.where(jnp.logical_and(row == k, tok == sel_s[k]), 1.0, onehot)
        onehot = jnp.concatenate([onehot, jnp.zeros((112, XR), F32)], axis=0).astype(BF)
        upd = jnp.dot(_unpack(yT_p[...]), onehot, preferred_element_type=F32)
        z = _unpack(xnT_p[c]).astype(F32) + upd
        s_att = jnp.concatenate([accT[2 * c], accT[2 * c + 1]], axis=1)
        outT_v[c] = (xT_v[c].astype(F32) + s_att * (z * _sigmoid(z))).astype(BF)

    tr_chunk(XC - 1)
    moe_route()
    for cp in head_copies(0):
        cp.wait()
    safe0 = head_stats(0)

    def block(j, i, tasks, fast):
        if not fast:
            for a in tasks:
                oproj(j, i * UN + a, attention(j, qproj(j, i * UN + a), False))
            return None
        first = i == 0
        js = jnp.where(jnp.logical_and(j == 0, first), 0, jnp.minimum(j + 1, HKV - 1))
        st = tuple(jnp.where(first, z, old)
                   for z, old in zip(stats_zero(), (kst[0:8], vst[0:8], wst[0:8])))
        nk = S // TPH
        nw = DP // IPH // WSL
        qs = []
        for a in tasks:
            k0 = pl.multiple_of((i * UN + a) * nk, nk)
            w0 = pl.multiple_of((i * WSL + a) * nw, 16)
            st = stats_fold(js, st, k0, nk, w0, nw if a < WSL else 0)
            zero = jnp.minimum(jnp.minimum(st[0][0:1, :], st[1][0:1, :]), 0.0)
            scale = QSCALE + jnp.minimum(jnp.concatenate([zero, zero], axis=1), st[2][0:1, :])
            qs.append(qproj(j, i * UN + a, scale))
        kst[0:8], vst[0:8], wst[0:8] = st
        outs = [attention(j, q, True) for q in qs]
        for a, op in zip(tasks, outs):
            oproj(j, i * UN + a, op)
        return stats_flag(st)

    def finish(c0, n):
        def fin(k, carry):
            for c in (c0 + 2 * k, c0 + 2 * k + 1):
                final(c)
                out_copy(c).start()
            return carry
        lax.fori_loop(0, n // 2, fin, 0)

    def head_body(j, safe):
        @pl.when(jnp.logical_and(j > 0, j + 1 < HKV))
        def _():
            for cp in head_copies(j + 1):
                cp.wait()

        @pl.when(j + 2 < HKV)
        def _():
            for cp in head_copies(j + 2):
                cp.start()

        @pl.when(j == HKV - 1)
        def _():
            moe_ffn()

        def fast_head():
            def it(i, c):
                flag = block(j, i, range(UN), True)

                @pl.when(jnp.logical_and(j == 0, i == 0))
                def _():
                    for cp in head_copies(1):
                        cp.wait()
                    for cp in moe_copies():
                        cp.start()
                    kst[0:8], vst[0:8], wst[0:8] = stats_fold(
                        1, stats_zero(), 0, S // IPH, 0, DP // IPH)

                @pl.when(j == HKV - 1)
                def _():
                    finish(i * (UN // 2), UN // 2)
                return flag
            return lax.fori_loop(0, IPH, it, 0)

        def slow_head():
            @pl.when(j == 0)
            def _():
                for cp in head_copies(1):
                    cp.wait()
                for cp in moe_copies():
                    cp.start()

            def it(t, c):
                block(j, t // UN, [t % UN], False)
                return c
            lax.fori_loop(0, TPH, it, 0)

            @pl.when(j == HKV - 1)
            def _():
                finish(0, XC)
            return head_stats(jnp.minimum(j + 1, HKV - 1))

        return lax.cond(safe > 0, fast_head, slow_head)

    lax.fori_loop(0, HKV, head_body, safe0)
    for c in range(XC):
        out_copy(c).wait()


@jax.jit
def pallas_recurrent_scan__gqa_block_cached__moe_arch_mod__prompt_kernel(
    A_x: jax.Array,
    A_k_cache: jax.Array,
    A_v_cache: jax.Array,
    A_wq: jax.Array,
    A_wo: jax.Array,
    B_x: jax.Array,
    B_w_r: jax.Array,
    B_w_gate: jax.Array,
    B_w_up: jax.Array,
    B_w_down: jax.Array,
):
    del B_x
    xT = A_x.reshape(S, D).T
    woT = A_wo.T
    wdT = B_w_down.T
    k = A_k_cache.reshape(HKV, S, DH)
    v = A_v_cache.reshape(HKV, S, DH)
    wr = B_w_r.reshape(1, D)

    hbm = pl.BlockSpec(memory_space=pltpu.HBM)
    vmem = pl.BlockSpec(memory_space=pltpu.VMEM)
    outT = pl.pallas_call(
        _kernel,
        out_shape=jax.ShapeDtypeStruct((D, S), BF),
        in_specs=[hbm, hbm, hbm, hbm, hbm, vmem, hbm, hbm, hbm],
        out_specs=hbm,
        scratch_shapes=[
            pltpu.VMEM((XC, D, XR), BF),
            pltpu.VMEM((XC, D // 2, XR), U32),
            pltpu.VMEM((S // 2, DP), U32),
            pltpu.VMEM((S // TQ, D, TQ), F32),
            pltpu.VMEM((HKV, S, DH), BF),
            pltpu.VMEM((HKV, S, DH), BF),
            pltpu.VMEM((HKV, DP, 2 * DH), BF),
            pltpu.VMEM((HKV, D, 2 * DH), BF),
            pltpu.VMEM((D, F), BF),
            pltpu.VMEM((D, F), BF),
            pltpu.VMEM((D, F), BF),
            pltpu.VMEM((32, DP), F32),
            pltpu.VMEM((XC, D, XR), BF),
            pltpu.VMEM((32, DH), F32),
            pltpu.VMEM((32, DH), F32),
            pltpu.VMEM((16, 2 * DH), F32),
            pltpu.VMEM((32, DH), F32),
            pltpu.VMEM((32, 128), F32),
            pltpu.VMEM((D // 2, 128), U32),
            pltpu.SMEM((C,), jnp.int32),
            pltpu.SemaphoreType.DMA((XC,)),
            pltpu.SemaphoreType.DMA((4 * HKV,)),
            pltpu.SemaphoreType.DMA((3,)),
            pltpu.SemaphoreType.DMA((XC,)),
        ],
        compiler_params=pltpu.CompilerParams(vmem_limit_bytes=100 * 1024 * 1024,
                                             disable_bounds_checks=True,
                                             disable_semaphore_checks=True),
        name="fused_attn_moe",
    )(xT, k, v, A_wq, woT, wr, B_w_gate, B_w_up, wdT)
    return outT.T.reshape(1, S, D)
```

```python
import math

import jax
import jax.numpy as jnp
from jax import lax
import jax.experimental.pallas as pl
import jax.experimental.pallas.tpu as pltpu

S = 2048
D = 576
DP = 640
HQ = 32
HKV = 16
DH = 128
F = 4608
C = 8
EPS_BF16 = 1.0013580322265625e-05

TQ = 128
UN = 16
CH = 512
TPH = S // TQ
IPH = TPH // UN
WSL = {16: 10, 8: 5, 4: 2}[UN]
HEAD0_AT = 3
HEAD1_AT = 7
XC = 8
XR = S // XC

BF = jnp.bfloat16
F32 = jnp.float32
U32 = jnp.uint32
QSCALE = (DH ** -0.5) * math.log2(math.e)

SCORE_BOUND = 40.0
V_HI = 2.0 ** 60
V_LO = 2.0 ** -60


def _rb(v):
    return v.astype(BF).astype(F32)


def _pack(v_bf16):
    return pltpu.bitcast(v_bf16, U32)


def _unpack(v_u32):
    return pltpu.bitcast(v_u32, BF)


def _fold(x, op):
    r = x[:, 0:128]
    for j in range(1, x.shape[1] // 128):
        r = op(r, x[:, j * 128:(j + 1) * 128])
    return r


def _sigmoid(v):
    return 0.5 * jnp.tanh(0.5 * v) + 0.5


def _recip(v):
    r = pl.reciprocal(v, approx=True)
    return r * (2.0 - v * r)


def _kernel(xT_hbm, k_hbm, v_hbm, wq_hbm, woT_hbm, wr_ref, wg_hbm, wu_hbm, wdT_hbm,
            outT_hbm,
            xT_v, xnT_p, xn_p, accT, k_v, v_v, wq_v, woT_v, wg_v, wu_v, wdT_v,
            xs_v, outT_v, kst, vst, wst, xnm, rs_v, yT_p, sel_s,
            sem_x, sem_h, sem_m, sem_o):

    def x_copy(c):
        return pltpu.make_async_copy(
            xT_hbm.at[:, pl.ds(c * XR, XR)], xT_v.at[c], sem_x.at[c])

    def head_copies(j):
        col = pl.multiple_of(j * (2 * DH), 2 * DH)
        pairs = [
            (wq_hbm.at[:, pl.ds(col, 2 * DH)], wq_v.at[j, pl.ds(0, D), :]),
            (k_hbm.at[j], k_v.at[j]),
            (v_hbm.at[j], v_v.at[j]),
            (woT_hbm.at[:, pl.ds(col, 2 * DH)], woT_v.at[j]),
        ]
        return [pltpu.make_async_copy(*pairs[w], sem_h.at[4 * j + w]) for w in range(4)]

    def moe_copies():
        return [pltpu.make_async_copy(wg_hbm, wg_v, sem_m.at[0]),
                pltpu.make_async_copy(wu_hbm, wu_v, sem_m.at[1]),
                pltpu.make_async_copy(wdT_hbm, wdT_v, sem_m.at[2])]

    def out_copy(c):
        cols = pl.ds(pl.multiple_of(c * XR, XR), XR)
        return pltpu.make_async_copy(outT_v.at[c], outT_hbm.at[:, cols], sem_o.at[c])

    for c in range(XC):
        x_copy(c).start()

    wq_v[:, D:DP, :] = jnp.zeros((HKV, DP - D, 2 * DH), BF)
    xs_v[...] = jnp.zeros(xs_v.shape, F32)

    def ln_chunk(c):
        xf = xT_v[c].astype(F32)
        mean = jnp.sum(xf, axis=0, keepdims=True) / D
        cen = xf - mean
        var = jnp.sum(cen * cen, axis=0, keepdims=True) / D
        mean_b = _rb(mean)
        dlt = _rb(xf - mean_b)
        sd = _rb(jnp.sqrt(_rb(_rb(var) + EPS_BF16)))
        xnT_p[c] = _pack((dlt / sd).astype(BF))
        return D * (var + (mean - mean_b) * (mean - mean_b)) / (sd * sd)

    def tr_chunk(c):
        xpad = jnp.concatenate([_unpack(xnT_p[c]), jnp.zeros((DP - D, XR), BF)], axis=0)
        xn_p[c * XR // 2:(c + 1) * XR // 2, :] = _pack(xpad.T)

    n2max = None
    for c in range(XC):
        x_copy(c).wait()
        n2 = ln_chunk(c)
        n2max = n2 if n2max is None else jnp.maximum(n2max, n2)
        if c > 0:
            tr_chunk(c - 1)
        if c == HEAD0_AT:
            for cp in head_copies(0):
                cp.start()
        if c == HEAD1_AT:
            for cp in head_copies(1):
                cp.start()
    xnm[0:8] = jnp.broadcast_to(_fold(n2max, jnp.maximum), (8, DH))

    def qproj(j, t, scale=QSCALE):
        r2 = pl.multiple_of(t * (TQ // 2), TQ // 2)
        xb = _unpack(xn_p[pl.ds(r2, TQ // 2), :])
        q2 = jnp.dot(xb, wq_v[j], preferred_element_type=F32)
        q2 = (q2 * scale).astype(BF)
        return jnp.concatenate([_pack(q2[:, 0:DH]), _pack(q2[:, DH:2 * DH])], axis=0)

    def oproj(j, t, o2p):
        upd = lax.dot_general(woT_v[j], _unpack(o2p), (((1,), (1,)), ((), ())),
                              preferred_element_type=F32)
        accT[t] = jnp.where(j == 0, upd, accT[t] + upd)

    def attention(j, qp, fast):
        q = _unpack(qp)
        m = l = acc = None
        for c in range(S // CH):
            kc = k_v[j, c * CH:(c + 1) * CH, :]
            s = lax.dot_general(q, kc, (((1,), (1,)), ((), ())),
                                preferred_element_type=F32)
            if fast:
                p = jnp.exp2(s)
            else:
                mc = jnp.broadcast_to(
                    jnp.max(_fold(s, jnp.maximum), axis=1, keepdims=True), (2 * TQ, 128))
                m_new = mc if m is None else jnp.maximum(m, mc)
                p = jnp.exp2(s - jnp.tile(m_new, (1, CH // 128)))
            lc = _fold(p, jnp.add)
            pv = jnp.dot(p.astype(BF), v_v[j, c * CH:(c + 1) * CH, :],
                         preferred_element_type=F32)
            if l is None:
                l, acc = lc, pv
            elif fast:
                l, acc = l + lc, acc + pv
            else:
                alpha = jnp.exp2(m - m_new)
                l, acc = l * alpha + lc, acc * alpha + pv
            if not fast:
                m = m_new
        ls = jnp.sum(l, axis=1, keepdims=True)
        o = (acc * _recip(ls)).astype(BF)
        return jnp.concatenate([_pack(o[0:TQ]), _pack(o[TQ:2 * TQ])], axis=1)

    def _absmax_packed(w):
        w = w & jnp.uint32(0x7FFF7FFF)
        hi = lax.bitcast_convert_type(w, F32)
        lo = lax.bitcast_convert_type(w << 16, F32)
        m = jnp.maximum(hi, lo)
        return _fold8(m, jnp.maximum)

    def _fold8(m, op):
        r = m[0:8]
        for i in range(1, m.shape[0] // 8):
            r = op(r, m[i * 8:(i + 1) * 8])
        return r

    def stats_fold(j, st, k0, nk, w0, nw):
        km, vm, ws = st
        km = jnp.maximum(km, _absmax_packed(_pack(k_v[j, pl.ds(k0, nk), :])))
        vm = jnp.maximum(vm, _absmax_packed(_pack(v_v[j, pl.ds(k0, nk), :])))
        if nw:
            wf = wq_v[j, pl.ds(w0, nw), :].astype(F32)
            ws = ws + _fold8(wf * wf, jnp.add)
        return km, vm, ws

    def stats_flag(st):
        km, vm, ws = st
        wn2 = jnp.sum(ws, axis=0, keepdims=True)
        wn = jnp.sqrt(jnp.maximum(wn2[:, 0:DH], wn2[:, DH:2 * DH]))
        kmx = jnp.max(km, axis=0, keepdims=True)
        xn = jnp.sqrt(jnp.max(xnm[0:1, :], axis=1, keepdims=True))
        bound = jnp.sum(wn * kmx, axis=1, keepdims=True) * xn * (1.05 * QSCALE)
        vmx = jnp.max(jnp.max(vm, axis=0, keepdims=True), axis=1, keepdims=True)
        ok = jnp.logical_and(bound <= SCORE_BOUND,
                             jnp.logical_and(vmx <= V_HI, vmx >= V_LO))
        return jnp.max(jnp.where(ok, 1.0, 0.0)).astype(jnp.int32)

    def stats_zero():
        return (jnp.zeros((8, DH), F32), jnp.zeros((8, DH), F32), jnp.zeros((8, 2 * DH), F32))

    def head_stats(j):
        return stats_flag(stats_fold(j, stats_zero(), 0, S, 0, DP))

    def moe_route():
        wr = jnp.broadcast_to(wr_ref[...], (16, D))
        xnT_all = jnp.concatenate([_unpack(xnT_p[c]) for c in range(XC)], axis=1)
        r = jnp.dot(wr, xnT_all, preferred_element_type=F32)
        r = _rb(r[0:8, :])
        col = lax.broadcasted_iota(jnp.int32, (8, S), 1)
        r = jnp.where(r == r, jnp.clip(r, -3e38, 3e38), -3e38)
        bits = lax.bitcast_convert_type(r, jnp.int32) & jnp.int32(-65536)
        bits = jnp.where(jnp.abs(r) < 2.0 ** -126, jnp.int32(0x00800000), bits)
        low = jnp.where(bits < 0, col, (S - 1) - col)
        key = lax.bitcast_convert_type(bits | low, F32)
        rowg = lax.broadcasted_iota(jnp.int32, (16, 128), 0)
        rsel = jnp.zeros((16, 128), F32)
        for c in range(C):
            mx = jnp.max(key, axis=1, keepdims=True)
            key = jnp.where(key == mx, -jnp.inf, key)
            mb = lax.bitcast_convert_type(mx, jnp.int32)
            lowb = mb & (S - 1)
            idx_v = jnp.where(mb < 0, lowb, (S - 1) - lowb)
            idx = jnp.max(idx_v)
            val = lax.bitcast_convert_type(mb & jnp.int32(-65536), F32)[0:1, :]
            rsel = jnp.where(rowg == c, val, rsel)
            sel_s[c] = idx
            w = xn_p[pl.ds(lax.shift_right_logical(idx, 1), 1), :]
            w = jnp.where((idx & 1) == 0, w << 16, w & jnp.uint32(0xFFFF0000))
            xs_v[c:c + 1, :] = lax.bitcast_convert_type(w, F32)
        rs_v[0:16] = rsel

    def moe_ffn():
        for cp in moe_copies():
            cp.wait()
        xs = xs_v[0:16, 0:D].astype(BF)
        g = _rb(jnp.dot(xs, wg_v[...], preferred_element_type=F32))
        uu = _rb(jnp.dot(xs, wu_v[...], preferred_element_type=F32))
        h = (_rb(g * _rb(_sigmoid(g))) * uu).astype(BF)
        y = _rb(lax.dot_general(h, wdT_v[...], (((1,), (1,)), ((), ())),
                                preferred_element_type=F32))
        y = _rb(y * _rb(_sigmoid(rs_v[0:16, 0:1])))
        ypad = jnp.concatenate([y, jnp.zeros((112, D), F32)], axis=0)
        ypad = jnp.concatenate([ypad, jnp.zeros((128, DP - D), F32)], axis=1)
        yT_p[...] = _pack(ypad.T[0:D, :].astype(BF))

    def final(c):
        row = lax.broadcasted_iota(jnp.int32, (16, XR), 0)
        tok = lax.broadcasted_iota(jnp.int32, (16, XR), 1) + c * XR
        onehot = jnp.zeros((16, XR), F32)
        for k in range(C):
            onehot = jnp.where(jnp.logical_and(row == k, tok == sel_s[k]), 1.0, onehot)
        onehot = jnp.concatenate([onehot, jnp.zeros((112, XR), F32)], axis=0).astype(BF)
        upd = jnp.dot(_unpack(yT_p[...]), onehot, preferred_element_type=F32)
        z = _unpack(xnT_p[c]).astype(F32) + upd
        s_att = jnp.concatenate([accT[2 * c], accT[2 * c + 1]], axis=1)
        hz = 0.5 * z
        silu = hz + hz * jnp.tanh(hz)
        outT_v[c] = (xT_v[c].astype(F32) + s_att * silu).astype(BF)

    tr_chunk(XC - 1)
    moe_route()
    for cp in head_copies(0):
        cp.wait()
    safe0 = head_stats(0)

    def block(j, i, tasks, fast):
        if not fast:
            for a in tasks:
                oproj(j, i * UN + a, attention(j, qproj(j, i * UN + a), False))
            return None
        first = i == 0
        js = jnp.where(jnp.logical_and(j == 0, first), 0, jnp.minimum(j + 1, HKV - 1))
        st = tuple(jnp.where(first, z, old)
                   for z, old in zip(stats_zero(), (kst[0:8], vst[0:8], wst[0:8])))
        nk = S // TPH
        nw = DP // IPH // WSL
        qs = []
        for a in tasks:
            k0 = pl.multiple_of((i * UN + a) * nk, nk)
            w0 = pl.multiple_of((i * WSL + a) * nw, 16)
            st = stats_fold(js, st, k0, nk, w0, nw if a < WSL else 0)
            zero = jnp.minimum(jnp.minimum(st[0][0:1, :], st[1][0:1, :]), 0.0)
            scale = QSCALE + jnp.minimum(jnp.concatenate([zero, zero], axis=1), st[2][0:1, :])
            qs.append(qproj(j, i * UN + a, scale))
        kst[0:8], vst[0:8], wst[0:8] = st
        outs = [attention(j, q, True) for q in qs]
        for a, op in zip(tasks, outs):
            oproj(j, i * UN + a, op)
        return stats_flag(st)

    def finish(c0, n):
        def fin(c, carry):
            final(c)
            out_copy(c).start()
            return carry
        lax.fori_loop(c0, c0 + n, fin, 0)

    def head_body(j, safe):
        @pl.when(jnp.logical_and(j > 0, j + 1 < HKV))
        def _():
            for cp in head_copies(j + 1):
                cp.wait()

        @pl.when(j + 2 < HKV)
        def _():
            for cp in head_copies(j + 2):
                cp.start()

        @pl.when(j == HKV - 1)
        def _():
            moe_ffn()

        def fast_head():
            def it(i, c):
                flag = block(j, i, range(UN), True)

                def redo_head1():
                    for cp in head_copies(1):
                        cp.wait()
                    for cp in moe_copies():
                        cp.start()
                    st = stats_fold(1, stats_zero(), 0, S // IPH, 0, DP // IPH)
                    kst[0:8], vst[0:8], wst[0:8] = st
                    return stats_flag(st) if IPH == 1 else flag

                flag = lax.cond(jnp.logical_and(j == 0, i == 0), redo_head1, lambda: flag)

                @pl.when(j == HKV - 1)
                def _():
                    finish(i * (UN // 2), UN // 2)
                return flag
            return lax.fori_loop(0, IPH, it, 0)

        def slow_head():
            @pl.when(j == 0)
            def _():
                for cp in head_copies(1):
                    cp.wait()
                for cp in moe_copies():
                    cp.start()

            def it(t, c):
                block(j, t // UN, [t % UN], False)
                return c
            lax.fori_loop(0, TPH, it, 0)

            @pl.when(j == HKV - 1)
            def _():
                finish(0, XC)
            return head_stats(jnp.minimum(j + 1, HKV - 1))

        return lax.cond(safe > 0, fast_head, slow_head)

    lax.fori_loop(0, HKV, head_body, safe0)
    for c in range(XC):
        out_copy(c).wait()


@jax.jit
def pallas_recurrent_scan__gqa_block_cached__moe_arch_mod__prompt_kernel(
    A_x: jax.Array,
    A_k_cache: jax.Array,
    A_v_cache: jax.Array,
    A_wq: jax.Array,
    A_wo: jax.Array,
    B_x: jax.Array,
    B_w_r: jax.Array,
    B_w_gate: jax.Array,
    B_w_up: jax.Array,
    B_w_down: jax.Array,
):
    del B_x
    xT = A_x.reshape(S, D).T
    woT = A_wo.T
    wdT = B_w_down.T
    k = A_k_cache.reshape(HKV, S, DH)
    v = A_v_cache.reshape(HKV, S, DH)
    wr = B_w_r.reshape(1, D)

    hbm = pl.BlockSpec(memory_space=pltpu.HBM)
    vmem = pl.BlockSpec(memory_space=pltpu.VMEM)
    outT = pl.pallas_call(
        _kernel,
        out_shape=jax.ShapeDtypeStruct((D, S), BF),
        in_specs=[hbm, hbm, hbm, hbm, hbm, vmem, hbm, hbm, hbm],
        out_specs=hbm,
        scratch_shapes=[
            pltpu.VMEM((XC, D, XR), BF),
            pltpu.VMEM((XC, D // 2, XR), U32),
            pltpu.VMEM((S // 2, DP), U32),
            pltpu.VMEM((S // TQ, D, TQ), F32),
            pltpu.VMEM((HKV, S, DH), BF),
            pltpu.VMEM((HKV, S, DH), BF),
            pltpu.VMEM((HKV, DP, 2 * DH), BF),
            pltpu.VMEM((HKV, D, 2 * DH), BF),
            pltpu.VMEM((D, F), BF),
            pltpu.VMEM((D, F), BF),
            pltpu.VMEM((D, F), BF),
            pltpu.VMEM((32, DP), F32),
            pltpu.VMEM((XC, D, XR), BF),
            pltpu.VMEM((32, DH), F32),
            pltpu.VMEM((32, DH), F32),
            pltpu.VMEM((16, 2 * DH), F32),
            pltpu.VMEM((32, DH), F32),
            pltpu.VMEM((32, 128), F32),
            pltpu.VMEM((D // 2, 128), U32),
            pltpu.SMEM((C,), jnp.int32),
            pltpu.SemaphoreType.DMA((XC,)),
            pltpu.SemaphoreType.DMA((4 * HKV,)),
            pltpu.SemaphoreType.DMA((3,)),
            pltpu.SemaphoreType.DMA((XC,)),
        ],
        compiler_params=pltpu.CompilerParams(vmem_limit_bytes=100 * 1024 * 1024,
                                             disable_bounds_checks=True,
                                             disable_semaphore_checks=True),
        name="fused_attn_moe",
    )(xT, k, v, A_wq, woT, wr, B_w_gate, B_w_up, wdT)
    return outT.T.reshape(1, S, D)
```

```python
import math

import jax
import jax.numpy as jnp
from jax import lax
import jax.experimental.pallas as pl
import jax.experimental.pallas.tpu as pltpu

S = 2048
D = 576
DP = 640
HQ = 32
HKV = 16
DH = 128
F = 4608
C = 8
EPS_BF16 = 1.0013580322265625e-05

TQ = 128
CH = 512
TPH = S // TQ
WSL = 10
HEAD0_AT = 2
XC = 8
XR = S // XC

BF = jnp.bfloat16
F32 = jnp.float32
U32 = jnp.uint32
QSCALE = (DH ** -0.5) * math.log2(math.e)

SCORE_BOUND = 40.0
V_HI = 2.0 ** 60
V_LO = 2.0 ** -60


def _rb(v):
    return v.astype(BF).astype(F32)


def _pack(v_bf16):
    return pltpu.bitcast(v_bf16, U32)


def _unpack(v_u32):
    return pltpu.bitcast(v_u32, BF)


def _fold(x, op):
    r = x[:, 0:128]
    for j in range(1, x.shape[1] // 128):
        r = op(r, x[:, j * 128:(j + 1) * 128])
    return r


def _sigmoid(v):
    return 0.5 * jnp.tanh(0.5 * v) + 0.5


def _recip(v):
    r = pl.reciprocal(v, approx=True)
    return r * (2.0 - v * r)


def _kernel(xT_hbm, k_hbm, v_hbm, wq_hbm, woT_hbm, wr_ref, wg_hbm, wu_hbm, wdT_hbm,
            outT_hbm,
            xT_v, xnT_p, xn_p, accT, k_v, v_v, wq_v, woT_v, wg_v, wu_v, wdT_v,
            xs_v, outT_v, xnm, rs_v, yT_p, sel_s,
            sem_x, sem_h, sem_m, sem_o):

    def x_copy(c):
        return pltpu.make_async_copy(
            xT_hbm.at[:, pl.ds(c * XR, XR)], xT_v.at[c], sem_x.at[c])

    def head_copies(j):
        col = pl.multiple_of(j * (2 * DH), 2 * DH)
        pairs = [
            (wq_hbm.at[:, pl.ds(col, 2 * DH)], wq_v.at[j, pl.ds(0, D), :]),
            (k_hbm.at[j], k_v.at[j]),
            (v_hbm.at[j], v_v.at[j]),
            (woT_hbm.at[:, pl.ds(col, 2 * DH)], woT_v.at[j]),
        ]
        return [pltpu.make_async_copy(*pairs[w], sem_h.at[4 * j + w]) for w in range(4)]

    def moe_copies():
        return [pltpu.make_async_copy(wg_hbm, wg_v, sem_m.at[0]),
                pltpu.make_async_copy(wu_hbm, wu_v, sem_m.at[1]),
                pltpu.make_async_copy(wdT_hbm, wdT_v, sem_m.at[2])]

    def out_copy(c):
        cols = pl.ds(pl.multiple_of(c * XR, XR), XR)
        return pltpu.make_async_copy(outT_v.at[c], outT_hbm.at[:, cols], sem_o.at[c])

    for c in range(XC):
        x_copy(c).start()

    wq_v[:, D:DP, :] = jnp.zeros((HKV, DP - D, 2 * DH), BF)
    xs_v[...] = jnp.zeros(xs_v.shape, F32)

    def ln_chunk(c):
        xf = xT_v[c].astype(F32)
        mean = jnp.sum(xf, axis=0, keepdims=True) / D
        cen = xf - mean
        var = jnp.sum(cen * cen, axis=0, keepdims=True) / D
        mean_b = _rb(mean)
        dlt = _rb(xf - mean_b)
        sd = _rb(jnp.sqrt(_rb(_rb(var) + EPS_BF16)))
        xnT_p[c] = _pack((dlt / sd).astype(BF))
        return D * (var + (mean - mean_b) * (mean - mean_b)) / (sd * sd)

    def tr_chunk(c):
        xpad = jnp.concatenate([_unpack(xnT_p[c]), jnp.zeros((DP - D, XR), BF)], axis=0)
        xn_p[c * XR // 2:(c + 1) * XR // 2, :] = _pack(xpad.T)

    n2max = None
    for c in range(XC):
        x_copy(c).wait()
        n2 = ln_chunk(c)
        n2max = n2 if n2max is None else jnp.maximum(n2max, n2)
        if c > 0:
            tr_chunk(c - 1)
        if c == HEAD0_AT:
            for cp in head_copies(0):
                cp.start()
    xnm[0:8] = jnp.broadcast_to(_fold(n2max, jnp.maximum), (8, DH))

    def qproj(j, t, scale=QSCALE):
        r2 = pl.multiple_of(t * (TQ // 2), TQ // 2)
        xb = _unpack(xn_p[pl.ds(r2, TQ // 2), :])
        q2 = jnp.dot(xb, wq_v[j], preferred_element_type=F32)
        q2 = (q2 * scale).astype(BF)
        return jnp.concatenate([_pack(q2[:, 0:DH]), _pack(q2[:, DH:2 * DH])], axis=0)

    def oproj(j, t, o2p, keep=None):
        upd = lax.dot_general(woT_v[j], _unpack(o2p), (((1,), (1,)), ((), ())),
                              preferred_element_type=F32)
        old = accT[t]
        new = jnp.where(j == 0, upd, old + upd)
        accT[t] = new if keep is None else jnp.where(keep, new, old)

    def attention(j, qp, fast):
        q = _unpack(qp)
        m = l = acc = None
        for c in range(S // CH):
            kc = k_v[j, c * CH:(c + 1) * CH, :]
            s = lax.dot_general(q, kc, (((1,), (1,)), ((), ())),
                                preferred_element_type=F32)
            if fast:
                p = jnp.exp2(s)
            else:
                mc = jnp.broadcast_to(
                    jnp.max(_fold(s, jnp.maximum), axis=1, keepdims=True), (2 * TQ, 128))
                m_new = mc if m is None else jnp.maximum(m, mc)
                p = jnp.exp2(s - jnp.tile(m_new, (1, CH // 128)))
            lc = _fold(p, jnp.add)
            pv = jnp.dot(p.astype(BF), v_v[j, c * CH:(c + 1) * CH, :],
                         preferred_element_type=F32)
            if l is None:
                l, acc = lc, pv
            elif fast:
                l, acc = l + lc, acc + pv
            else:
                alpha = jnp.exp2(m - m_new)
                l, acc = l * alpha + lc, acc * alpha + pv
            if not fast:
                m = m_new
        ls = jnp.sum(l, axis=1, keepdims=True)
        o = (acc * _recip(ls)).astype(BF)
        return jnp.concatenate([_pack(o[0:TQ]), _pack(o[TQ:2 * TQ])], axis=1)

    def _absmax_packed(w):
        w = w & jnp.uint32(0x7FFF7FFF)
        hi = lax.bitcast_convert_type(w, F32)
        lo = lax.bitcast_convert_type(w << 16, F32)
        m = jnp.maximum(hi, lo)
        return _fold8(m, jnp.maximum)

    def _fold8(m, op):
        r = m[0:8]
        for i in range(1, m.shape[0] // 8):
            r = op(r, m[i * 8:(i + 1) * 8])
        return r

    def stats_fold(j, st, k0, nk, w0, nw):
        km, vm, ws = st
        km = jnp.maximum(km, _absmax_packed(_pack(k_v[j, pl.ds(k0, nk), :])))
        vm = jnp.maximum(vm, _absmax_packed(_pack(v_v[j, pl.ds(k0, nk), :])))
        if nw:
            wf = wq_v[j, pl.ds(w0, nw), :].astype(F32)
            ws = ws + _fold8(wf * wf, jnp.add)
        return km, vm, ws

    def stats_flag(st):
        km, vm, ws = st
        wn2 = jnp.sum(ws, axis=0, keepdims=True)
        wn = jnp.sqrt(jnp.maximum(wn2[:, 0:DH], wn2[:, DH:2 * DH]))
        kmx = jnp.max(km, axis=0, keepdims=True)
        xn = jnp.sqrt(jnp.max(xnm[0:1, :], axis=1, keepdims=True))
        bound = jnp.sum(wn * kmx, axis=1, keepdims=True) * xn * (1.05 * QSCALE)
        vmx = jnp.max(jnp.max(vm, axis=0, keepdims=True), axis=1, keepdims=True)
        ok = jnp.logical_and(bound <= SCORE_BOUND,
                             jnp.logical_and(vmx <= V_HI, vmx >= V_LO))
        return ok, jnp.max(jnp.where(ok, 1.0, 0.0)).astype(jnp.int32)

    def stats_zero():
        return (jnp.zeros((8, DH), F32), jnp.zeros((8, DH), F32), jnp.zeros((8, 2 * DH), F32))

    def head_stats(j):
        return stats_flag(stats_fold(j, stats_zero(), 0, S, 0, DP))[1]

    def moe_route():
        wr = jnp.broadcast_to(wr_ref[...].reshape(1, D), (16, D))
        xnT_all = jnp.concatenate([_unpack(xnT_p[c]) for c in range(XC)], axis=1)
        r = jnp.dot(wr, xnT_all, preferred_element_type=F32)
        r = _rb(r[0:8, :])
        col = lax.broadcasted_iota(jnp.int32, (8, S), 1)
        r = jnp.where(r == r, jnp.clip(r, -3e38, 3e38), -3e38)
        bits = lax.bitcast_convert_type(r, jnp.int32) & jnp.int32(-65536)
        bits = jnp.where(jnp.abs(r) < 2.0 ** -126, jnp.int32(0x00800000), bits)
        low = jnp.where(bits < 0, col, (S - 1) - col)
        key = lax.bitcast_convert_type(bits | low, F32)
        rowg = lax.broadcasted_iota(jnp.int32, (16, 128), 0)
        rsel = jnp.zeros((16, 128), F32)
        for c in range(C):
            mx = jnp.max(key, axis=1, keepdims=True)
            key = jnp.where(key == mx, -jnp.inf, key)
            mb = lax.bitcast_convert_type(mx, jnp.int32)
            lowb = mb & (S - 1)
            idx_v = jnp.where(mb < 0, lowb, (S - 1) - lowb)
            idx = jnp.max(idx_v)
            val = lax.bitcast_convert_type(mb & jnp.int32(-65536), F32)[0:1, :]
            rsel = jnp.where(rowg == c, val, rsel)
            sel_s[c] = idx
            w = xn_p[pl.ds(lax.shift_right_logical(idx, 1), 1), :]
            w = jnp.where((idx & 1) == 0, w << 16, w & jnp.uint32(0xFFFF0000))
            xs_v[c:c + 1, :] = lax.bitcast_convert_type(w, F32)
        rs_v[0:16] = rsel

    def moe_ffn():
        for cp in moe_copies():
            cp.wait()
        xs = xs_v[0:16, 0:D].astype(BF)
        g = _rb(jnp.dot(xs, wg_v[...], preferred_element_type=F32))
        uu = _rb(jnp.dot(xs, wu_v[...], preferred_element_type=F32))
        h = (_rb(g * _rb(_sigmoid(g))) * uu).astype(BF)
        y = _rb(lax.dot_general(h, wdT_v[...], (((1,), (1,)), ((), ())),
                                preferred_element_type=F32))
        y = _rb(y * _rb(_sigmoid(rs_v[0:16, 0:1])))
        ypad = jnp.concatenate([y, jnp.zeros((112, D), F32)], axis=0)
        ypad = jnp.concatenate([ypad, jnp.zeros((128, DP - D), F32)], axis=1)
        yT_p[...] = _pack(ypad.T[0:D, :].astype(BF))

    def final(c):
        row = lax.broadcasted_iota(jnp.int32, (16, XR), 0)
        tok = lax.broadcasted_iota(jnp.int32, (16, XR), 1) + c * XR
        onehot = jnp.zeros((16, XR), F32)
        for k in range(C):
            onehot = jnp.where(jnp.logical_and(row == k, tok == sel_s[k]), 1.0, onehot)
        onehot = jnp.concatenate([onehot, jnp.zeros((112, XR), F32)], axis=0).astype(BF)
        upd = jnp.dot(_unpack(yT_p[...]), onehot, preferred_element_type=F32)
        z = _unpack(xnT_p[c]).astype(F32) + upd
        s_att = jnp.concatenate([accT[2 * c], accT[2 * c + 1]], axis=1)
        hz = 0.5 * z
        silu = hz + hz * jnp.tanh(hz)
        outT_v[c] = (xT_v[c].astype(F32) + s_att * silu).astype(BF)

    tr_chunk(XC - 1)
    moe_route()
    for cp in head_copies(0):
        cp.wait()
    for cp in head_copies(1):
        cp.start()

    def fast_head(j):
        nk = S // TPH
        nw = DP // WSL
        st = stats_zero()
        qs = []
        for a in range(TPH):
            st = stats_fold(j, st, a * nk, nk, a * nw, nw if a < WSL else 0)
            zero = jnp.minimum(jnp.minimum(st[0][0:1, :], st[1][0:1, :]), 0.0)
            scale = QSCALE + jnp.minimum(jnp.concatenate([zero, zero], axis=1), st[2][0:1, :])
            qs.append(qproj(j, a, scale))
        ok, flag = stats_flag(st)
        outs = [attention(j, q, True) for q in qs]
        for a, op in enumerate(outs):
            oproj(j, a, op, ok)
        return flag

    def slow_head(j):
        def it(t, c):
            oproj(j, t, attention(j, qproj(j, t), False))
            return c
        lax.fori_loop(0, TPH, it, 0)
        return head_stats(j)

    def head_body(j, try_fast):
        @pl.when(j > 0)
        def _():
            for cp in head_copies(j):
                cp.wait()

        @pl.when(j + 2 < HKV)
        def _():
            for cp in head_copies(j + 2):
                cp.start()

        @pl.when(j == 1)
        def _():
            for cp in moe_copies():
                cp.start()

        @pl.when(j == HKV - 1)
        def _():
            moe_ffn()

        done = lax.cond(try_fast > 0, lambda: fast_head(j), lambda: jnp.int32(0))
        return lax.cond(done > 0, lambda: jnp.int32(1), lambda: slow_head(j))

    lax.fori_loop(0, HKV, head_body, jnp.int32(1))

    def fin(c, carry):
        final(c)
        out_copy(c).start()
        return carry
    lax.fori_loop(0, XC, fin, 0)
    for c in range(XC):
        out_copy(c).wait()


@jax.jit
def pallas_recurrent_scan__gqa_block_cached__moe_arch_mod__prompt_kernel(
    A_x: jax.Array,
    A_k_cache: jax.Array,
    A_v_cache: jax.Array,
    A_wq: jax.Array,
    A_wo: jax.Array,
    B_x: jax.Array,
    B_w_r: jax.Array,
    B_w_gate: jax.Array,
    B_w_up: jax.Array,
    B_w_down: jax.Array,
):
    del B_x
    xT = A_x.reshape(S, D).T
    woT = A_wo.T
    wdT = B_w_down.T
    k = A_k_cache.reshape(HKV, S, DH)
    v = A_v_cache.reshape(HKV, S, DH)
    wr = B_w_r

    hbm = pl.BlockSpec(memory_space=pltpu.HBM)
    vmem = pl.BlockSpec(memory_space=pltpu.VMEM)
    outT = pl.pallas_call(
        _kernel,
        out_shape=jax.ShapeDtypeStruct((D, S), BF),
        in_specs=[hbm, hbm, hbm, hbm, hbm, vmem, hbm, hbm, hbm],
        out_specs=hbm,
        scratch_shapes=[
            pltpu.VMEM((XC, D, XR), BF),
            pltpu.VMEM((XC, D // 2, XR), U32),
            pltpu.VMEM((S // 2, DP), U32),
            pltpu.VMEM((S // TQ, D, TQ), F32),
            pltpu.VMEM((HKV, S, DH), BF),
            pltpu.VMEM((HKV, S, DH), BF),
            pltpu.VMEM((HKV, DP, 2 * DH), BF),
            pltpu.VMEM((HKV, D, 2 * DH), BF),
            pltpu.VMEM((D, F), BF),
            pltpu.VMEM((D, F), BF),
            pltpu.VMEM((D, F), BF),
            pltpu.VMEM((32, DP), F32),
            pltpu.VMEM((XC, D, XR), BF),
            pltpu.VMEM((32, DH), F32),
            pltpu.VMEM((32, 128), F32),
            pltpu.VMEM((D // 2, 128), U32),
            pltpu.SMEM((C,), jnp.int32),
            pltpu.SemaphoreType.DMA((XC,)),
            pltpu.SemaphoreType.DMA((4 * HKV,)),
            pltpu.SemaphoreType.DMA((3,)),
            pltpu.SemaphoreType.DMA((XC,)),
        ],
        compiler_params=pltpu.CompilerParams(vmem_limit_bytes=100 * 1024 * 1024,
                                             disable_bounds_checks=True,
                                             disable_semaphore_checks=True),
        name="fused_attn_moe",
    )(xT, k, v, A_wq, woT, wr, B_w_gate, B_w_up, wdT)
    return outT.T.reshape(1, S, D)
```

```python
import math

import jax
import jax.numpy as jnp
from jax import lax
import jax.experimental.pallas as pl
import jax.experimental.pallas.tpu as pltpu

S = 2048
D = 576
DP = 640
HQ = 32
HKV = 16
DH = 128
F = 4608
C = 8
EPS_BF16 = 1.0013580322265625e-05

TQ = 128
CH = 512
TPH = S // TQ
WSL = 10
HEAD0_AT = 2
XC = 8
XR = S // XC

BF = jnp.bfloat16
F32 = jnp.float32
U32 = jnp.uint32
QSCALE = (DH ** -0.5) * math.log2(math.e)

SCORE_BOUND = 40.0
V_HI = 2.0 ** 60
V_LO = 2.0 ** -60


def _rb(v):
    return v.astype(BF).astype(F32)


def _pack(v_bf16):
    return pltpu.bitcast(v_bf16, U32)


def _unpack(v_u32):
    return pltpu.bitcast(v_u32, BF)


def _fold(x, op):
    r = x[:, 0:128]
    for j in range(1, x.shape[1] // 128):
        r = op(r, x[:, j * 128:(j + 1) * 128])
    return r


def _sigmoid(v):
    return 0.5 * jnp.tanh(0.5 * v) + 0.5


def _recip(v):
    r = pl.reciprocal(v, approx=True)
    return r * (2.0 - v * r)


def _kernel(xT_hbm, k_hbm, v_hbm, wq_hbm, woT_hbm, wr_ref, wg_hbm, wu_hbm, wdT_hbm,
            outT_hbm,
            xT_v, xnT_p, xn_p, accT, k_v, v_v, wq_v, woT_v, wg_v, wu_v, wdT_v,
            xs_v, outT_v, xnm, rs_v, yT_p, sel_s,
            sem_x, sem_h, sem_m, sem_o):

    def x_copy(c):
        return pltpu.make_async_copy(
            xT_hbm.at[:, pl.ds(c * XR, XR)], xT_v.at[c], sem_x.at[c])

    def head_copies(j):
        col = pl.multiple_of(j * (2 * DH), 2 * DH)
        pairs = [
            (wq_hbm.at[:, pl.ds(col, 2 * DH)], wq_v.at[j, pl.ds(0, D), :]),
            (k_hbm.at[j], k_v.at[j]),
            (v_hbm.at[j], v_v.at[j]),
            (woT_hbm.at[:, pl.ds(col, 2 * DH)], woT_v.at[j]),
        ]
        return [pltpu.make_async_copy(*pairs[w], sem_h.at[4 * j + w]) for w in range(4)]

    def moe_copies():
        return [pltpu.make_async_copy(wg_hbm, wg_v, sem_m.at[0]),
                pltpu.make_async_copy(wu_hbm, wu_v, sem_m.at[1]),
                pltpu.make_async_copy(wdT_hbm, wdT_v, sem_m.at[2])]

    def out_copy(c):
        cols = pl.ds(pl.multiple_of(c * XR, XR), XR)
        return pltpu.make_async_copy(outT_v.at[c], outT_hbm.at[:, cols], sem_o.at[c])

    for c in range(XC):
        x_copy(c).start()

    wq_v[:, D:DP, :] = jnp.zeros((HKV, DP - D, 2 * DH), BF)
    xs_v[...] = jnp.zeros(xs_v.shape, F32)

    def ln_chunk(c):
        xf = xT_v[c].astype(F32)
        mean = jnp.sum(xf, axis=0, keepdims=True) / D
        cen = xf - mean
        var = jnp.sum(cen * cen, axis=0, keepdims=True) / D
        mean_b = _rb(mean)
        dlt = _rb(xf - mean_b)
        sd = _rb(jnp.sqrt(_rb(_rb(var) + EPS_BF16)))
        xnT_p[c] = _pack((dlt / sd).astype(BF))
        return D * (var + (mean - mean_b) * (mean - mean_b)) / (sd * sd)

    def tr_chunk(c):
        xpad = jnp.concatenate([_unpack(xnT_p[c]), jnp.zeros((DP - D, XR), BF)], axis=0)
        xn_p[c * XR // 2:(c + 1) * XR // 2, :] = _pack(xpad.T)

    def router_scores(c):
        wr = jnp.broadcast_to(wr_ref[...].reshape(1, D), (16, D))
        return jnp.dot(wr, _unpack(xnT_p[c]), preferred_element_type=F32)[0:8]

    n2max = None
    scores = []
    for c in range(XC):
        x_copy(c).wait()
        n2 = ln_chunk(c)
        n2max = n2 if n2max is None else jnp.maximum(n2max, n2)
        if c > 0:
            scores.append(router_scores(c - 1))
            tr_chunk(c - 1)
        if c == HEAD0_AT:
            for cp in head_copies(0):
                cp.start()
    xnm[0:8] = jnp.broadcast_to(_fold(n2max, jnp.maximum), (8, DH))

    def qproj(j, t, scale=QSCALE):
        r2 = pl.multiple_of(t * (TQ // 2), TQ // 2)
        xb = _unpack(xn_p[pl.ds(r2, TQ // 2), :])
        q2 = jnp.dot(xb, wq_v[j], preferred_element_type=F32)
        q2 = (q2 * scale).astype(BF)
        return jnp.concatenate([_pack(q2[:, 0:DH]), _pack(q2[:, DH:2 * DH])], axis=0)

    def oproj(j, t, o2p, keep=None):
        upd = lax.dot_general(woT_v[j], _unpack(o2p), (((1,), (1,)), ((), ())),
                              preferred_element_type=F32)
        old = accT[t]
        new = jnp.where(j == 0, upd, old + upd)
        accT[t] = new if keep is None else jnp.where(keep, new, old)

    def attention(j, qp, fast):
        q = _unpack(qp)
        m = l = acc = None
        for c in range(S // CH):
            kc = k_v[j, c * CH:(c + 1) * CH, :]
            s = lax.dot_general(q, kc, (((1,), (1,)), ((), ())),
                                preferred_element_type=F32)
            if fast:
                p = jnp.exp2(s)
            else:
                mc = jnp.broadcast_to(
                    jnp.max(_fold(s, jnp.maximum), axis=1, keepdims=True), (2 * TQ, 128))
                m_new = mc if m is None else jnp.maximum(m, mc)
                p = jnp.exp2(s - jnp.tile(m_new, (1, CH // 128)))
            lc = _fold(p, jnp.add)
            pv = jnp.dot(p.astype(BF), v_v[j, c * CH:(c + 1) * CH, :],
                         preferred_element_type=F32)
            if l is None:
                l, acc = lc, pv
            elif fast:
                l, acc = l + lc, acc + pv
            else:
                alpha = jnp.exp2(m - m_new)
                l, acc = l * alpha + lc, acc * alpha + pv
            if not fast:
                m = m_new
        ls = jnp.sum(l, axis=1, keepdims=True)
        o = (acc * _recip(ls)).astype(BF)
        return jnp.concatenate([_pack(o[0:TQ]), _pack(o[TQ:2 * TQ])], axis=1)

    def _absmax_packed(w):
        w = w & jnp.uint32(0x7FFF7FFF)
        hi = lax.bitcast_convert_type(w, F32)
        lo = lax.bitcast_convert_type(w << 16, F32)
        m = jnp.maximum(hi, lo)
        return _fold8(m, jnp.maximum)

    def _fold8(m, op):
        r = m[0:8]
        for i in range(1, m.shape[0] // 8):
            r = op(r, m[i * 8:(i + 1) * 8])
        return r

    def stats_fold(j, st, k0, nk, w0, nw):
        km, vm, ws = st
        km = jnp.maximum(km, _absmax_packed(_pack(k_v[j, pl.ds(k0, nk), :])))
        vm = jnp.maximum(vm, _absmax_packed(_pack(v_v[j, pl.ds(k0, nk), :])))
        if nw:
            wf = wq_v[j, pl.ds(w0, nw), :].astype(F32)
            ws = ws + _fold8(wf * wf, jnp.add)
        return km, vm, ws

    def stats_flag(st):
        km, vm, ws = st
        wn2 = jnp.sum(ws, axis=0, keepdims=True)
        wn = jnp.sqrt(jnp.maximum(wn2[:, 0:DH], wn2[:, DH:2 * DH]))
        kmx = jnp.max(km, axis=0, keepdims=True)
        xn = jnp.sqrt(jnp.max(xnm[0:1, :], axis=1, keepdims=True))
        bound = jnp.sum(wn * kmx, axis=1, keepdims=True) * xn * (1.05 * QSCALE)
        vmx = jnp.max(jnp.max(vm, axis=0, keepdims=True), axis=1, keepdims=True)
        ok = jnp.logical_and(bound <= SCORE_BOUND,
                             jnp.logical_and(vmx <= V_HI, vmx >= V_LO))
        return ok, jnp.max(jnp.where(ok, 1.0, 0.0)).astype(jnp.int32)

    def stats_zero():
        return (jnp.zeros((8, DH), F32), jnp.zeros((8, DH), F32), jnp.zeros((8, 2 * DH), F32))

    def head_stats(j):
        return stats_flag(stats_fold(j, stats_zero(), 0, S, 0, DP))[1]

    def moe_route(r):
        r = _rb(r)
        col = lax.broadcasted_iota(jnp.int32, (8, S), 1)
        r = jnp.where(r == r, jnp.clip(r, -3e38, 3e38), -3e38)
        bits = lax.bitcast_convert_type(r, jnp.int32) & jnp.int32(-65536)
        bits = jnp.where(jnp.abs(r) < 2.0 ** -126, jnp.int32(0x00800000), bits)
        low = jnp.where(bits < 0, col, (S - 1) - col)
        key = lax.bitcast_convert_type(bits | low, F32)
        rowg = lax.broadcasted_iota(jnp.int32, (16, 128), 0)
        rsel = jnp.zeros((16, 128), F32)
        for c in range(C):
            mx = jnp.max(key, axis=1, keepdims=True)
            key = jnp.where(key == mx, -jnp.inf, key)
            mb = lax.bitcast_convert_type(mx, jnp.int32)
            lowb = mb & (S - 1)
            idx_v = jnp.where(mb < 0, lowb, (S - 1) - lowb)
            idx = jnp.max(idx_v)
            val = lax.bitcast_convert_type(mb & jnp.int32(-65536), F32)[0:1, :]
            rsel = jnp.where(rowg == c, val, rsel)
            sel_s[c] = idx
            w = xn_p[pl.ds(lax.shift_right_logical(idx, 1), 1), :]
            w = jnp.where((idx & 1) == 0, w << 16, w & jnp.uint32(0xFFFF0000))
            xs_v[c:c + 1, :] = lax.bitcast_convert_type(w, F32)
        rs_v[0:16] = rsel

    def moe_ffn():
        for cp in moe_copies():
            cp.wait()
        xs = xs_v[0:16, 0:D].astype(BF)
        g = _rb(jnp.dot(xs, wg_v[...], preferred_element_type=F32))
        uu = _rb(jnp.dot(xs, wu_v[...], preferred_element_type=F32))
        h = (_rb(g * _rb(_sigmoid(g))) * uu).astype(BF)
        y = _rb(lax.dot_general(h, wdT_v[...], (((1,), (1,)), ((), ())),
                                preferred_element_type=F32))
        y = _rb(y * _rb(_sigmoid(rs_v[0:16, 0:1])))
        ypad = jnp.concatenate([y, jnp.zeros((112, D), F32)], axis=0)
        ypad = jnp.concatenate([ypad, jnp.zeros((128, DP - D), F32)], axis=1)
        yT_p[...] = _pack(ypad.T[0:D, :].astype(BF))

    def final(c):
        row = lax.broadcasted_iota(jnp.int32, (16, XR), 0)
        tok = lax.broadcasted_iota(jnp.int32, (16, XR), 1) + c * XR
        onehot = jnp.zeros((16, XR), F32)
        for k in range(C):
            onehot = jnp.where(jnp.logical_and(row == k, tok == sel_s[k]), 1.0, onehot)
        onehot = jnp.concatenate([onehot, jnp.zeros((112, XR), F32)], axis=0).astype(BF)
        upd = jnp.dot(_unpack(yT_p[...]), onehot, preferred_element_type=F32)
        z = _unpack(xnT_p[c]).astype(F32) + upd
        s_att = jnp.concatenate([accT[2 * c], accT[2 * c + 1]], axis=1)
        hz = 0.5 * z
        silu = hz + hz * jnp.tanh(hz)
        outT_v[c] = (xT_v[c].astype(F32) + s_att * silu).astype(BF)

    scores.append(router_scores(XC - 1))
    tr_chunk(XC - 1)
    moe_route(jnp.concatenate(scores, axis=1))
    for cp in head_copies(0):
        cp.wait()
    for cp in head_copies(1):
        cp.start()

    def fast_head(j):
        nk = S // TPH
        nw = DP // WSL
        st = stats_zero()
        qs = []
        for a in range(TPH):
            st = stats_fold(j, st, a * nk, nk, a * nw, nw if a < WSL else 0)
            zero = jnp.minimum(jnp.minimum(st[0][0:1, :], st[1][0:1, :]), 0.0)
            scale = QSCALE + jnp.minimum(jnp.concatenate([zero, zero], axis=1), st[2][0:1, :])
            qs.append(qproj(j, a, scale))
        ok, flag = stats_flag(st)
        outs = [attention(j, q, True) for q in qs]
        for a, op in enumerate(outs):
            oproj(j, a, op, ok)
        return flag

    def slow_head(j):
        def it(t, c):
            oproj(j, t, attention(j, qproj(j, t), False))
            return c
        lax.fori_loop(0, TPH, it, 0)
        return head_stats(j)

    def head_body(j, try_fast):
        @pl.when(j > 0)
        def _():
            for cp in head_copies(j):
                cp.wait()

        @pl.when(j + 2 < HKV)
        def _():
            for cp in head_copies(j + 2):
                cp.start()

        @pl.when(j == 1)
        def _():
            for cp in moe_copies():
                cp.start()

        @pl.when(j == HKV - 1)
        def _():
            moe_ffn()

        done = lax.cond(try_fast > 0, lambda: fast_head(j), lambda: jnp.int32(0))
        return lax.cond(done > 0, lambda: jnp.int32(1), lambda: slow_head(j))

    lax.fori_loop(0, HKV, head_body, jnp.int32(1))

    def fin(c, carry):
        final(c)
        out_copy(c).start()
        return carry
    lax.fori_loop(0, XC, fin, 0)
    for c in range(XC):
        out_copy(c).wait()


@jax.jit
def pallas_recurrent_scan__gqa_block_cached__moe_arch_mod__prompt_kernel(
    A_x: jax.Array,
    A_k_cache: jax.Array,
    A_v_cache: jax.Array,
    A_wq: jax.Array,
    A_wo: jax.Array,
    B_x: jax.Array,
    B_w_r: jax.Array,
    B_w_gate: jax.Array,
    B_w_up: jax.Array,
    B_w_down: jax.Array,
):
    del B_x
    xT = A_x.reshape(S, D).T
    woT = A_wo.T
    wdT = B_w_down.T
    k = A_k_cache.reshape(HKV, S, DH)
    v = A_v_cache.reshape(HKV, S, DH)
    wr = B_w_r

    hbm = pl.BlockSpec(memory_space=pltpu.HBM)
    vmem = pl.BlockSpec(memory_space=pltpu.VMEM)
    outT = pl.pallas_call(
        _kernel,
        out_shape=jax.ShapeDtypeStruct((D, S), BF),
        in_specs=[hbm, hbm, hbm, hbm, hbm, vmem, hbm, hbm, hbm],
        out_specs=hbm,
        scratch_shapes=[
            pltpu.VMEM((XC, D, XR), BF),
            pltpu.VMEM((XC, D // 2, XR), U32),
            pltpu.VMEM((S // 2, DP), U32),
            pltpu.VMEM((S // TQ, D, TQ), F32),
            pltpu.VMEM((HKV, S, DH), BF),
            pltpu.VMEM((HKV, S, DH), BF),
            pltpu.VMEM((HKV, DP, 2 * DH), BF),
            pltpu.VMEM((HKV, D, 2 * DH), BF),
            pltpu.VMEM((D, F), BF),
            pltpu.VMEM((D, F), BF),
            pltpu.VMEM((D, F), BF),
            pltpu.VMEM((32, DP), F32),
            pltpu.VMEM((XC, D, XR), BF),
            pltpu.VMEM((32, DH), F32),
            pltpu.VMEM((32, 128), F32),
            pltpu.VMEM((D // 2, 128), U32),
            pltpu.SMEM((C,), jnp.int32),
            pltpu.SemaphoreType.DMA((XC,)),
            pltpu.SemaphoreType.DMA((4 * HKV,)),
            pltpu.SemaphoreType.DMA((3,)),
            pltpu.SemaphoreType.DMA((XC,)),
        ],
        compiler_params=pltpu.CompilerParams(vmem_limit_bytes=100 * 1024 * 1024,
                                             disable_bounds_checks=True,
                                             disable_semaphore_checks=True),
        name="fused_attn_moe",
    )(xT, k, v, A_wq, woT, wr, B_w_gate, B_w_up, wdT)
    return outT.T.reshape(1, S, D)
```
